```python
import jax
import jax.numpy as jnp

def _softmax(x, axis=-1):
    return jax.nn.softmax(x, axis=axis)
def _gelu(x):
    return jax.nn.gelu(x, approximate=True)
def _silu(x):
    return jax.nn.silu(x)
def _sigmoid(x):
    return jax.nn.sigmoid(x)
def _layernorm(x, axis=-1, eps=1e-5):
    m = jnp.mean(x, axis=axis, keepdims=True)
    v = jnp.var(x, axis=axis, keepdims=True)
    return (x - m) / jnp.sqrt(v + eps)
def _scatter_add(tgt, idx, src, axis=0):
    return tgt.at[idx].add(src)
def _segment_sum(src, seg, n):
    return jax.ops.segment_sum(src, seg, n)
class _Rng:
    def __init__(self, key):
        self._k = key
    def _next(self):
        self._k, sub = jax.random.split(self._k)
        return sub
    def normal(self, shape):
        return jax.random.normal(self._next(), shape, dtype=jnp.bfloat16)
    def randint(self, lo, hi, shape):
        return jax.random.randint(self._next(), shape, lo, hi, dtype=jnp.int32)
    def uniform(self, shape, lo=0.0, hi=1.0):
        return jax.random.uniform(self._next(), shape, jnp.bfloat16, lo, hi)
    def permutation(self, n):
        return jax.random.permutation(self._next(), n)


kernel_name = 'recurrent_scan__sliding_local_dilated__geglu_ffn__prompt'

def setup_inputs():
    _rng = _Rng(jax.random.key(int.from_bytes(__import__("os").urandom(4), "little")))
    _w = (lambda a: (lambda t: t.astype(jnp.bfloat16) if jnp.issubdtype(t.dtype, jnp.floating) else t)(jnp.asarray(a)))
    def _A_setup():
        B, S, D = 1, 2048, 1024
        return {
            "x": _w((lambda *s: _rng.normal(s) * 0.05)(B, S, D)),
            "wqkv": _w((lambda *s: _rng.normal(s) * 0.05)(D, 3 * D)),
            "wo": _w((lambda *s: _rng.normal(s) * 0.05)(D, D)),
        }
    _A_in = _A_setup()

    def _B_setup():
        B, S, D, F = 1, 2048, 1024, 3584
        return {
            "x": _w((lambda *s: _rng.normal(s) * 0.05)(B, S, D)),
            "w_gate": _w((lambda *s: _rng.normal(s) * 0.05)(D, F)),
            "w_up": _w((lambda *s: _rng.normal(s) * 0.05)(D, F)),
            "w_down": _w((lambda *s: _rng.normal(s) * 0.05)(F, D)),
        }
    _B_in = _B_setup()

    return {
        "A_x": _A_in["x"],
        "A_wqkv": _A_in["wqkv"],
        "A_wo": _A_in["wo"],
        "B_x": _B_in["x"],
        "B_w_gate": _B_in["w_gate"],
        "B_w_up": _B_in["w_up"],
        "B_w_down": _B_in["w_down"],
    }

def reference(A_x, A_wqkv, A_wo, B_x, B_w_gate, B_w_up, B_w_down):
    def _A_ref(x, wqkv, wo):
        B, S, D = x.shape
        H = 32; Dh = D // H
        W, dil = 8, 2
        qkv = (lambda x, *d: x.transpose(*d))((x @ wqkv).reshape(B, S, 3, H, Dh), 2, 0, 3, 1, 4)
        q, k, v = qkv[0], qkv[1], qkv[2]
        scale = Dh ** -0.5
        pos = jnp.arange(S)
        off = jnp.arange(W) * dil
        idx = pos[:, None] - off[None, :]
        mask = idx >= 0
        idx_c = jnp.where(mask, idx, 0).reshape(-1)
        kg = k[:, :, idx_c, :].reshape(B, H, S, W, Dh)
        vg = v[:, :, idx_c, :].reshape(B, H, S, W, Dh)
        logits = jnp.einsum("bhsd,bhswd->bhsw", q, kg) * scale
        logits = jnp.where(mask[None, None, :, :], logits, -1e9)
        attn = _softmax(logits, axis=-1)
        o = jnp.einsum("bhsw,bhswd->bhsd", attn, vg)
        return (lambda x, *d: x.transpose(*d))(o, 0, 2, 1, 3).reshape(B, S, D) @ wo

    def _B_ref(x, w_gate, w_up, w_down):
        return (_gelu(x @ w_gate) * (x @ w_up)) @ w_down

    x = A_x
    xn = _layernorm(x, axis=-1)
    s = _A_ref(xn, A_wqkv, A_wo)
    g = _silu(_B_ref(xn, B_w_gate, B_w_up, B_w_down))
    return x + s * g
```

```python
import functools
import jax
import jax.numpy as jnp
from jax import lax
import jax.experimental.pallas as pl
import jax.experimental.pallas.tpu as pltpu

f32 = jnp.float32
bf16 = jnp.bfloat16
u32 = jnp.uint32

S, D, F = 2048, 1024, 3584
HS, HD = S // 2, D // 2
FC = 256
FH = FC // 2
NF = F // FC
RB = 256
NB = HS // RB
PAD = 16
AR = 80
NW = 8
SCALE = 32 ** -0.5
LOG2E = 1.4426950408889634
NEG = -1e9 / SCALE


def _dot(a, b):
    return jnp.dot(a, b, preferred_element_type=f32)


def _acomb(a11, a12, a21, a22):
    r = lambda v: v.astype(bf16)
    return [r(a11 + a22), r(a21 + a22), r(a11), r(a22), r(a11 + a12), r(a21 - a11), r(a12 - a22)]


def _bcomb(b11, b12, b21, b22):
    r = lambda v: v.astype(bf16)
    return [r(b11 + b22), r(b11), r(b12 - b22), r(b21 - b11), r(b22), r(b11 + b12), r(b21 + b22)]


def _ccomb(m):
    m1, m2, m3, m4, m5, m6, m7 = m
    return m1 + m4 - m5 + m7, m3 + m5, m2 + m4, m1 - m2 + m3 + m6


def _gelu(x):
    c = 0.7978845608028654
    return 0.5 * x * (1.0 + jnp.tanh(c * (x + 0.044715 * (x * x * x))))


def _ln(xb):
    x = xb.astype(f32)
    m = jnp.mean(x, axis=-1, keepdims=True)
    xc = x - m
    v = jnp.mean(xc * xc, axis=-1, keepdims=True)
    return xc * lax.rsqrt(v + 1e-5)


def _kernel(x_hbm, wqkv_hbm, wo_hbm, wg_hbm, wu_hbm, wd_hbm, out_hbm,
            xraw, xa_u, gu_raw, wd_raw, bgu_u, bd_u, acc, wq_raw, bqa_u, bqb_u, qkv, oa_u,
            wo_raw, wo_f, bo_u, obuf,
            sem_x, sem_w, sem_q, sem_o, sem_out):
    xa = xa_u.bitcast(bf16)
    bgu = bgu_u.bitcast(bf16)
    bd = bd_u.bitcast(bf16)
    bqs = (bqa_u.bitcast(bf16), bqb_u.bitcast(bf16))
    oa = oa_u.bitcast(bf16)
    bo = bo_u.bitcast(bf16)

    def x_copy(r):
        return pltpu.make_async_copy(x_hbm.at[:, pl.ds(r * RB, RB), :],
                                     xraw.at[:, pl.ds(r * RB, RB), :], sem_x.at[r])

    def gu_copies(j, slot):
        off = pl.multiple_of(j * FC, FC)
        return (pltpu.make_async_copy(wg_hbm.at[:, pl.ds(off, FC)], gu_raw.at[slot, 0], sem_w.at[slot, 0]),
                pltpu.make_async_copy(wu_hbm.at[:, pl.ds(off, FC)], gu_raw.at[slot, 1], sem_w.at[slot, 1]))

    def wd_copy(j, slot):
        off = pl.multiple_of(j * FC, FC)
        return pltpu.make_async_copy(wd_hbm.at[pl.ds(off, FC), :], wd_raw.at[slot], sem_w.at[slot, 2])

    def wq_copy(t):
        return pltpu.make_async_copy(wqkv_hbm.at[:, pl.ds(t * D, D)], wq_raw.at[t], sem_q.at[t])

    def wo_copy():
        return pltpu.make_async_copy(wo_hbm, wo_raw, sem_o.at[0])

    def out_copy(r0, n, k):
        return pltpu.make_async_copy(obuf.at[:, pl.ds(r0, n), :], out_hbm.at[:, pl.ds(r0, n), :], sem_out.at[k])

    def ln_block(r):
        LC = 16
        for c0 in range(r * RB, (r + 1) * RB, LC):
            lo = _ln(xraw[0, c0:c0 + LC, :])
            hi = _ln(xraw[1, c0:c0 + LC, :])
            cs = _acomb(lo[:, :HD], lo[:, HD:], hi[:, :HD], hi[:, HD:])
            for i in range(7):
                xa[i, c0:c0 + LC, :] = cs[i]

    def prep_gu(slot):
        KC = 32
        for t in range(2):
            for k0 in range(0, HD, KC):
                lo = gu_raw[slot, t, k0:k0 + KC, :].astype(f32)
                hi = gu_raw[slot, t, HD + k0:HD + k0 + KC, :].astype(f32)
                cs = _bcomb(lo[:, :FH], lo[:, FH:], hi[:, :FH], hi[:, FH:])
                for i in range(7):
                    bgu[i, k0:k0 + KC, t * FH:(t + 1) * FH] = cs[i]

    def prep_d(slot):
        KC = 16
        for k0 in range(0, FH, KC):
            for c0 in range(0, HD, 256):
                w = lambda a, b: wd_raw[slot, a + k0:a + k0 + KC, b + c0:b + c0 + 256].astype(f32)
                cs = _bcomb(w(0, 0), w(0, HD), w(FH, 0), w(FH, HD))
                for i in range(7):
                    bd[i, k0:k0 + KC, c0:c0 + 256] = cs[i]

    def ffn_gu(r):
        ms = [_dot(xa[i, r * RB:(r + 1) * RB, :], bgu[i]) for i in range(7)]
        cs = _ccomb(ms)
        return _acomb(*[_gelu(v[:, :FH]) * v[:, FH:] for v in cs])

    def ffn_dn(r, hs, first):
        for i in range(7):
            y = _dot(hs[i], bd[i])
            if first:
                acc[i, r * RB:(r + 1) * RB, :] = y
            else:
                acc[i, r * RB:(r + 1) * RB, :] += y

    lane = lax.broadcasted_iota(jnp.int32, (8, 128), 1)

    def prep_q(t, bq):
        KC = 16
        m0 = [(lane & (1 << b)) == 0 for b in range(3)]
        for k0 in range(0, HD, KC):
            halves = []
            for hk in range(2):
                blk = [pltpu.bitcast(wq_raw[t, hk * HD + k0:hk * HD + k0 + KC, c * 128:(c + 1) * 128], u32)
                       for c in range(8)]
                for b in range(3):
                    s = 1 << b
                    nxt = list(blk)
                    for c in range(8):
                        if c & s == 0:
                            a_, b_ = blk[c], blk[c + s]
                            nxt[c] = jnp.where(m0[b], a_, pltpu.roll(b_, s, 1))
                            nxt[c + s] = jnp.where(m0[b], pltpu.roll(a_, 128 - s, 1), b_)
                    blk = nxt
                halves.append(blk)
            up = lambda v: pltpu.bitcast(v, bf16).astype(f32)
            for n in range(4):
                cs = _bcomb(up(halves[0][n]), up(halves[0][n + 4]), up(halves[1][n]), up(halves[1][n + 4]))
                for i in range(7):
                    bq[i, k0:k0 + KC, n * 128:(n + 1) * 128] = cs[i]

    def qkv_phase(t, bq):
        for r in range(NB):
            for n in range(4):
                ms = [_dot(xa[i, r * RB:(r + 1) * RB, :], bq[i, :, n * 128:(n + 1) * 128]) for i in range(7)]
                c11, c12, c21, c22 = _ccomb(ms)
                r0 = PAD + r * RB
                qkv[t, n, r0:r0 + RB, :] = c11
                qkv[t, n + 4, r0:r0 + RB, :] = c12
                qkv[t, n, HS + r0:HS + r0 + RB, :] = c21
                qkv[t, n + 4, HS + r0:HS + r0 + RB, :] = c22
                if r == 0 and t > 0:
                    qkv[t, n, 0:PAD, :] = jnp.broadcast_to(c11[0:1, :], (PAD, 128))
                    qkv[t, n + 4, 0:PAD, :] = jnp.broadcast_to(c12[0:1, :], (PAD, 128))

    lane16 = lax.broadcasted_iota(jnp.int32, (16, 128), 1)
    row16 = lax.broadcasted_iota(jnp.int32, (16, 128), 0)

    def attn_group(base, row0):
        lg = [None] * NW
        for c in range(8):
            q = qkv[0, c, pl.ds(base, 16), :]
            for s in range(4):
                win = qkv[1, c, pl.ds(base - 8 - 2 * s, 24), :]
                for w, kk in ((s, win[8:24]), (s + 4, win[0:16])):
                    pr = q * kk
                    lg[w] = pr if lg[w] is None else lg[w] + pr
        b4 = (lane16 & 16) != 0
        b3 = (lane16 & 8) != 0
        for w in range(NW):
            l = lg[w]
            l = l + jnp.where(b4, pltpu.roll(l, 16, 1), pltpu.roll(l, 112, 1))
            l = l + jnp.where(b3, pltpu.roll(l, 8, 1), pltpu.roll(l, 120, 1))
            if row0 is not None and w > 0:
                l = jnp.where(row16 + row0 >= 2 * w, l, NEG)
            lg[w] = l
        m = lg[0]
        for w in range(1, NW):
            m = jnp.maximum(m, lg[w])
        p = [jnp.exp2((lg[w] - m) * (SCALE * LOG2E)) for w in range(NW)]
        den = p[0]
        for w in range(1, NW):
            den = den + p[w]
        inv = 1.0 / den
        p = [v * inv for v in p]
        outs = []
        for c in range(8):
            o = None
            for s in range(4):
                win = qkv[2, c, pl.ds(base - 8 - 2 * s, 24), :]
                for w, vv in ((s, win[8:24]), (s + 4, win[0:16])):
                    pr = p[w] * vv
                    o = pr if o is None else o + pr
            outs.append(o)
        return outs

    def attn_pair(r0):
        lo = attn_group(pl.multiple_of(PAD + r0, 16), r0)
        hi = attn_group(pl.multiple_of(PAD + HS + r0, 16), None)
        for n in range(4):
            cs = _acomb(lo[n], lo[n + 4], hi[n], hi[n + 4])
            for i in range(7):
                oa[i, pl.ds(pl.multiple_of(r0, 16), 16), n * 128:(n + 1) * 128] = cs[i]

    def prep_o():
        for n in range(4):
            for k0 in range(0, D, 64):
                for h in range(2):
                    c0 = (n + 4 * h) * 128
                    wo_f[n + 4 * h, k0:k0 + 64, :] = wo_raw[k0:k0 + 64, c0:c0 + 128].astype(f32)
            for b in range(4):
                for g2 in range(8):
                    def ld(h, bb):
                        return jnp.concatenate(
                            [wo_f[n + 4 * h, pl.ds(16 * g2 + bb, 8, stride=128), :],
                             wo_f[n + 4 * h, pl.ds(16 * g2 + 8 + bb, 8, stride=128), :]], axis=0)
                    cs = _bcomb(ld(0, b), ld(1, b), ld(0, b + 4), ld(1, b + 4))
                    k0 = b * 128 + g2 * 16
                    for i in range(7):
                        bo[i, k0:k0 + 16, n * 128:(n + 1) * 128] = cs[i]

    x_copy(0).start()
    for cp in gu_copies(0, 0):
        cp.start()
    x_copy(1).start()
    wd_copy(0, 0).start()
    for r in range(2, NB):
        x_copy(r).start()

    x_copy(0).wait()
    ln_block(0)
    for cp in gu_copies(0, 0):
        cp.wait()
    wq_copy(0).start()
    for cp in gu_copies(1, 1):
        cp.start()
    prep_gu(0)

    hs = [None] * NB
    x_copy(1).wait()
    wd_copy(0, 0).wait()
    prep_d(0)
    ln_block(1)
    hs[0] = ffn_gu(0)
    x_copy(2).wait()
    x_copy(3).wait()
    wq_copy(1).start()
    wq_copy(2).start()
    wo_copy().start()
    wd_copy(1, 1).start()
    ln_block(2)
    hs[1] = ffn_gu(1)
    ffn_dn(0, hs[0], True)
    ln_block(3)
    hs[2] = ffn_gu(2)
    ffn_dn(1, hs[1], True)
    wq_copy(0).wait()
    for cp in gu_copies(1, 1):
        cp.wait()
    prep_q(0, bqs[0])
    hs[3] = ffn_gu(3)
    ffn_dn(2, hs[2], True)
    prep_gu(1)
    ffn_dn(3, hs[3], True)

    wd_copy(2, 0).start()
    for cp in gu_copies(2, 0):
        cp.start()
    for cp in gu_copies(3, 1):
        cp.start()

    wq_copy(1).wait()
    wq_copy(2).wait()
    wo_copy().wait()
    prep_q(1, bqs[1])
    qkv_phase(0, bqs[0])
    prep_q(2, bqs[0])
    qkv_phase(1, bqs[1])
    prep_o()
    qkv_phase(2, bqs[0])

    def p3_body(j, carry):
        sd = j % 2
        sg = 1 - sd
        wd_copy(j, sd).wait()
        for cp in gu_copies(jnp.minimum(j + 1, NF - 1), sg):
            cp.wait()
        prep_d(sd)
        a = jnp.minimum((j - 1) * AR, HS - AR)
        hs = [None] * NB
        ng = AR // 16
        hs[0] = ffn_gu(0)
        attn_pair(a)
        attn_pair(a + 16)
        hs[1] = ffn_gu(1)
        ffn_dn(0, hs[0], False)
        attn_pair(a + 32)
        attn_pair(a + 48)
        hs[2] = ffn_gu(2)
        ffn_dn(1, hs[1], False)
        attn_pair(a + 64)
        hs[3] = ffn_gu(3)
        ffn_dn(2, hs[2], False)
        prep_gu(sg)
        ffn_dn(3, hs[3], False)

        @pl.when(j + 2 < NF)
        def _():
            wd_copy(j + 2, sd).start()

        @pl.when(j + 2 < NF)
        def _():
            for cp in gu_copies(jnp.minimum(j + 3, NF - 1), sg):
                cp.start()
        return carry

    lax.fori_loop(1, NF, p3_body, 0)

    blocks = [(0, 256), (256, 256), (512, 256), (768, 128), (896, 128)]
    for k, (r0, n_) in enumerate(blocks):
        for n in range(4):
            ms = [_dot(oa[i, r0:r0 + n_, :], bo[i, :, n * 128:(n + 1) * 128]) for i in range(7)]
            ss = _ccomb(ms)
            fs = _ccomb([acc[i, r0:r0 + n_, n * 128:(n + 1) * 128] for i in range(7)])
            for q, (h, cb) in enumerate(((0, n), (0, n + 4), (1, n), (1, n + 4))):
                fv = fs[q]
                g = fv * jax.nn.sigmoid(fv)
                xv = xraw[h, r0:r0 + n_, cb * 128:(cb + 1) * 128].astype(f32)
                obuf[h, r0:r0 + n_, cb * 128:(cb + 1) * 128] = (xv + ss[q] * g).astype(bf16)
        out_copy(r0, n_, k).start()
    for k, (r0, n_) in enumerate(blocks):
        out_copy(r0, n_, k).wait()


@jax.jit
def pallas_recurrent_scan__sliding_local_dilated__geglu_ffn__prompt_kernel(
    A_x: jax.Array,
    A_wqkv: jax.Array,
    A_wo: jax.Array,
    B_x: jax.Array,
    B_w_gate: jax.Array,
    B_w_up: jax.Array,
    B_w_down: jax.Array,
):
    x2 = A_x.reshape(2, HS, D)
    any_spec = pl.BlockSpec(memory_space=pl.ANY)
    out = pl.pallas_call(
        _kernel,
        out_shape=jax.ShapeDtypeStruct((2, HS, D), bf16),
        in_specs=[any_spec] * 6,
        out_specs=any_spec,
        scratch_shapes=[
            pltpu.VMEM((2, HS, D), bf16),
            pltpu.VMEM((7, HS // 2, HD), u32),
            pltpu.VMEM((2, 2, D, FC), bf16),
            pltpu.VMEM((2, FC, D), bf16),
            pltpu.VMEM((7, HD // 2, FC), u32),
            pltpu.VMEM((7, FH // 2, HD), u32),
            pltpu.VMEM((7, HS, HD), f32),
            pltpu.VMEM((3, D, D), bf16),
            pltpu.VMEM((7, HD // 2, HD), u32),
            pltpu.VMEM((7, HD // 2, HD), u32),
            pltpu.VMEM((3, 8, PAD + S, 128), f32),
            pltpu.VMEM((7, HS // 2, HD), u32),
            pltpu.VMEM((D, D), bf16),
            pltpu.VMEM((8, D, 128), f32),
            pltpu.VMEM((7, HD // 2, HD), u32),
            pltpu.VMEM((2, HS, D), bf16),
            pltpu.SemaphoreType.DMA((NB,)),
            pltpu.SemaphoreType.DMA((2, 3)),
            pltpu.SemaphoreType.DMA((3,)),
            pltpu.SemaphoreType.DMA((1,)),
            pltpu.SemaphoreType.DMA((8,)),
        ],
        compiler_params=pltpu.CompilerParams(vmem_limit_bytes=120 * 1024 * 1024),
        name="fusedk",
    )(x2, A_wqkv, A_wo, B_w_gate, B_w_up, B_w_down)
    return out.reshape(1, S, D)
```

```python
import jax
import jax.numpy as jnp
from jax import lax
import jax.experimental.pallas as pl
import jax.experimental.pallas.tpu as pltpu

f32 = jnp.float32
bf16 = jnp.bfloat16
u32 = jnp.uint32

S, D, F = 2048, 1024, 3584
HS, HD = S // 2, D // 2
FC = 256
FH = FC // 2
NF = F // FC
RB = 256
NB = HS // RB
PAD = 16
NW = 8
SCALE = 32 ** -0.5
LOG2E = 1.4426950408889634
NEG = -1e9 / SCALE


def _dot(a, b):
    return jnp.dot(a, b, preferred_element_type=f32)


def _acomb(a11, a12, a21, a22):
    r = lambda v: v.astype(bf16)
    return [r(a11 + a22), r(a21 + a22), r(a11), r(a22), r(a11 + a12), r(a21 - a11), r(a12 - a22)]


def _bcomb(b11, b12, b21, b22):
    r = lambda v: v.astype(bf16)
    return [r(b11 + b22), r(b11), r(b12 - b22), r(b21 - b11), r(b22), r(b11 + b12), r(b21 + b22)]


def _ccomb(m):
    m1, m2, m3, m4, m5, m6, m7 = m
    return m1 + m4 - m5 + m7, m3 + m5, m2 + m4, m1 - m2 + m3 + m6


def _gelu(x):
    c = 0.7978845608028654
    return 0.5 * x * (1.0 + jnp.tanh(c * (x + 0.044715 * (x * x * x))))


def _sum8(v):
    return ((v[0] + v[1]) + (v[2] + v[3])) + ((v[4] + v[5]) + (v[6] + v[7]))


def _butterfly(sets, masks, axis, size):
    for b in range(3):
        sh = 1 << b
        out = []
        for blk in sets:
            nxt = list(blk)
            for c in range(8):
                if c & sh == 0:
                    lo, hi = blk[c], blk[c + sh]
                    nxt[c] = jnp.where(masks[b], lo, pltpu.roll(hi, sh, axis))
                    nxt[c + sh] = jnp.where(masks[b], pltpu.roll(lo, size - sh, axis), hi)
            out.append(nxt)
        sets = out
    return sets


def _kernel(x_hbm, wqkv_hbm, wo_hbm, wg_hbm, wu_hbm, wd_hbm, out_hbm,
            xraw, xa_u, gu_raw, wd_raw, bgu_u, bd_u, acc, wq_raw, bq, qkv, oa_u,
            wo_raw, bo, obuf, zbuf, sems):
    xa = xa_u.bitcast(bf16)
    bgu = bgu_u.bitcast(bf16)
    bd = bd_u.bitcast(bf16)
    oa = oa_u.bitcast(bf16)
    pk = lambda v: pltpu.bitcast(v, u32)
    un = lambda v: pltpu.bitcast(v, bf16)

    lane = lax.broadcasted_iota(jnp.int32, (8, 128), 1)
    row8 = lax.broadcasted_iota(jnp.int32, (8, 128), 0)
    lane_lo = [(lane & (1 << b)) == 0 for b in range(3)]
    row_lo = [(row8 & (1 << b)) == 0 for b in range(3)]

    def x_copy(r):
        return pltpu.make_async_copy(x_hbm.at[:, pl.ds(r * RB, RB), :],
                                     xraw.at[:, pl.ds(r * RB, RB), :], sems.at[r])

    def gu_copies(j, slot):
        off = pl.multiple_of(j * FC, FC)
        return (pltpu.make_async_copy(wg_hbm.at[:, pl.ds(off, FC)], gu_raw.at[slot, 0], sems.at[4 + 3 * slot]),
                pltpu.make_async_copy(wu_hbm.at[:, pl.ds(off, FC)], gu_raw.at[slot, 1], sems.at[5 + 3 * slot]))

    def wd_copy(j, slot):
        off = pl.multiple_of(j * FC, FC)
        return pltpu.make_async_copy(wd_hbm.at[pl.ds(off, FC), :], wd_raw.at[slot], sems.at[6 + 3 * slot])

    def wq_copy(t):
        return pltpu.make_async_copy(wqkv_hbm.at[:, pl.ds(t * D, D)], wq_raw.at[t], sems.at[10 + t])

    def wo_copies():
        return [pltpu.make_async_copy(wo_hbm.at[:, pl.ds(c * 128, 128)], wo_raw.at[c], sems.at[24 + c])
                for c in range(8)]

    def z_copy():
        return pltpu.make_async_copy(x_hbm.at[0, pl.ds(0, 16), pl.ds(0, 128)], zbuf, sems.at[22])

    def out_copy(r0, n, k):
        return pltpu.make_async_copy(obuf.at[:, pl.ds(r0, n), :], out_hbm.at[:, pl.ds(r0, n), :],
                                     sems.at[14 + k])

    def true_mask():
        return pk(zbuf[...]) == pk(xraw.at[0][0:16, 0:128])

    def ln_half(h, c0, tm16, a):
        xs = []
        for c in range(4):
            x2 = xraw.at[h][c0:c0 + 16, c * 256:(c + 1) * 256].astype(f32)
            xs += [x2[:, :128], x2[:, 128:]]
        s1 = _sum8(xs)
        if a is not None:
            s1 = jnp.where(tm16, s1, a)
        m = jnp.sum(s1, axis=-1, keepdims=True) * (1.0 / D)
        xc = [x - m for x in xs]
        v = jnp.sum(_sum8([x * x for x in xc]), axis=-1, keepdims=True) * (1.0 / D)
        r = lax.rsqrt(v + 1e-5)
        return [x * r for x in xc]

    def ln_rows(r0, n, anc=None):
        tm16 = None
        if anc is not None:
            tm = true_mask()
            tm16 = jnp.concatenate([tm, tm], axis=0)
            anc = anc[:int(len(anc) * 0.85)]
        nch = n // 16
        for k in range(nch):
            c0 = r0 + 16 * k
            a = [None, None]
            if anc is not None:
                a = [anc[(len(anc) * (2 * k + u)) // (2 * nch)] for u in range(2)]
            lo = ln_half(0, c0, tm16, a[0])
            hi = ln_half(1, c0, tm16, a[1])
            for c in range(4):
                cs = _acomb(lo[c], lo[c + 4], hi[c], hi[c + 4])
                for i in range(7):
                    xa.at[i][c0:c0 + 16, c * 128:(c + 1) * 128] = cs[i]

    def prep_gu(slot):
        KC = 32
        for t in range(2):
            for k0 in range(0, HD, KC):
                lo = gu_raw[slot, t, k0:k0 + KC, :].astype(f32)
                hi = gu_raw[slot, t, HD + k0:HD + k0 + KC, :].astype(f32)
                cs = _bcomb(lo[:, :FH], lo[:, FH:], hi[:, :FH], hi[:, FH:])
                for i in range(7):
                    bgu.at[i][k0:k0 + KC, t * FH:(t + 1) * FH] = cs[i]

    def prep_d(slot):
        KC = 16
        for k0 in range(0, FH, KC):
            for c0 in range(0, HD, 256):
                w = lambda a, b: wd_raw[slot, a + k0:a + k0 + KC, b + c0:b + c0 + 256].astype(f32)
                cs = _bcomb(w(0, 0), w(0, HD), w(FH, 0), w(FH, HD))
                for i in range(7):
                    bd.at[i][k0:k0 + KC, c0:c0 + 256] = cs[i]

    def ffn_gu(r0, n):
        ms = [_dot(xa[i, r0:r0 + n, :], bgu[i]) for i in range(7)]
        anc = [m_[k:k + 16, t * FH:(t + 1) * FH] for m_ in ms for t in range(2) for k in range(0, n, 64)]
        hs = _acomb(*[_gelu(v[:, :FH]) * v[:, FH:] for v in _ccomb(ms)])
        return hs, anc

    def ffn_dn(r0, n, hs, first):
        for i in range(7):
            y = _dot(hs[i], bd[i])
            if first:
                acc[i, r0:r0 + n, :] = y
            else:
                acc[i, r0:r0 + n, :] += y

    upk = lambda v: un(v).astype(f32)

    def prep_q0():
        KC = 16
        ld = lambda r0: [pk(wq_raw[0, r0:r0 + KC, c * 128:(c + 1) * 128]) for c in range(8)]
        for k00 in range(0, HD, 2 * KC):
            ks = (k00, k00 + KC)
            hv = _butterfly([ld(hk * HD + k0) for k0 in ks for hk in range(2)], lane_lo, 1, 128)
            for ki, k0 in enumerate(ks):
                lo, hi = hv[2 * ki], hv[2 * ki + 1]
                for n in range(4):
                    cs = _bcomb(upk(lo[n]), upk(lo[n + 4]), upk(hi[n]), upk(hi[n + 4]))
                    for i in range(7):
                        bq.at[n // 2, i, n % 2][k0 // 2:(k0 + KC) // 2, :] = pk(cs[i])

    def prep_q_half(t, h, dst):
        KC = 16
        sa = (128 - 2) * h
        sb = 2 * (1 - h)
        w = wq_raw.at[t]

        def stage1(r0):
            blk = [pk(w[r0:r0 + KC, c * 128:(c + 1) * 128]) for c in range(8)]
            return [jnp.where(lane_lo[1], pltpu.roll(blk[c], sa, 1), pltpu.roll(blk[c + 2], sb, 1))
                    for c in (0, 1, 4, 5)]

        def stage(sets, jb, b):
            sh = 1 << b
            out = []
            for blk in sets:
                nxt = list(blk)
                for j in range(4):
                    if j & jb == 0:
                        lo, hi = blk[j], blk[j + jb]
                        nxt[j] = jnp.where(lane_lo[b], lo, pltpu.roll(hi, sh, 1))
                        nxt[j + jb] = jnp.where(lane_lo[b], pltpu.roll(lo, 128 - sh, 1), hi)
                out.append(nxt)
            return out

        for k0 in range(0, HD, KC):
            lo, hi = stage(stage([stage1(hk * HD + k0) for hk in range(2)], 1, 0), 2, 2)
            for e in range(2):
                cs = _bcomb(upk(lo[e]), upk(lo[e + 2]), upk(hi[e]), upk(hi[e + 2]))
                for i in range(7):
                    dst.at[i, e][k0 // 2:(k0 + KC) // 2, :] = pk(cs[i])

    def qkv_tiles(t, h, src):
        anc = []
        for e in range(2):
            n = 2 * h + e
            qlo = qkv.at[t, n]
            qhi = qkv.at[t, n + 4]
            for r in range(NB):
                ms = [_dot(xa[i, r * RB:(r + 1) * RB, :], un(src.at[i, e][...])) for i in range(7)]
                c11, c12, c21, c22 = _ccomb(ms)
                anc += [m_[8 * k:8 * k + 8] for m_ in ms for k in range(0, RB // 8, 8)]
                r0 = PAD + r * RB
                qlo[r0:r0 + RB, :] = c11
                qhi[r0:r0 + RB, :] = c12
                qlo[HS + r0:HS + r0 + RB, :] = c21
                qhi[HS + r0:HS + r0 + RB, :] = c22
                if r == 0:
                    qlo[0:PAD, :] = jnp.broadcast_to(c11[0:1, :], (PAD, 128))
                    qhi[0:PAD, :] = jnp.broadcast_to(c12[0:1, :], (PAD, 128))
        return anc

    def prep_o_chunks(idxs, anc):
        tm = true_mask()
        step = (len(anc) - 12) / (4 * len(idxs))
        pc = 0
        for idx in idxs:
            n = idx // 8
            g16 = pl.multiple_of((idx % 8) * 16, 16)
            g8 = pl.multiple_of((idx % 8) * 8, 8)
            res = []
            for h in range(2):
                w = wo_raw.at[n + 4 * h]
                w16 = [w[pl.ds(128 * i + g16, 16), :].astype(f32) for i in range(8)]
                for u in range(2):
                    blk = [v[8 * u:8 * u + 8] for v in w16]
                    blk[0] = jnp.where(tm, blk[0], anc[int(pc * step)])
                    pc += 1
                    res += _butterfly([blk], row_lo, 0, 8)
            cols = [[jnp.concatenate([res[2 * h][j], res[2 * h + 1][j]], axis=0) for j in range(8)]
                    for h in range(2)]
            for b in range(4):
                cs = _bcomb(cols[0][b], cols[1][b], cols[0][b + 4], cols[1][b + 4])
                for i in range(7):
                    bo.at[i, n][pl.ds(b * 64 + g8, 8), :] = pk(cs[i])

    def attn8(base, row0):
        lg = [None] * NW
        for c in range(8):
            q = qkv[0, c, pl.ds(base, 8), :]
            for w in range(NW):
                pr = q * qkv[1, c, pl.ds(base - 2 * w, 8), :]
                lg[w] = pr if lg[w] is None else lg[w] + pr
        for w0 in range(0, NW, 2):
            for w in (w0, w0 + 1):
                lg[w] = lg[w] + pltpu.roll(lg[w], 8, 1)
            for w in (w0, w0 + 1):
                lg[w] = lg[w] + pltpu.roll(lg[w], 16, 1)
        if row0 is not None:
            for w in range(1, NW):
                lg[w] = jnp.where(row8 + row0 >= 2 * w, lg[w], NEG)
        m = lg[0]
        for w in range(1, NW):
            m = jnp.maximum(m, lg[w])
        p = [jnp.exp2((lg[w] - m) * (SCALE * LOG2E)) for w in range(NW)]
        den = p[0]
        for w in range(1, NW):
            den = den + p[w]
        inv = 1.0 / den
        b4 = (lane & 16) != 0
        b3 = (lane & 8) != 0
        outs = [None] * 8
        for w in range(NW):
            pw = p[w] * inv
            pw = jnp.where(b4, pw, pltpu.roll(pw, 112, 1))
            pw = jnp.where(b3, pw, pltpu.roll(pw, 120, 1))
            for c in range(8):
                pr = pw * qkv[2, c, pl.ds(base - 2 * w, 8), :]
                outs[c] = pr if outs[c] is None else outs[c] + pr
        return outs

    def attn_pair(r0):
        parts = [attn8(pl.multiple_of(PAD + h * HS + r0 + 8 * u, 8), (r0 + 8 * u) if h == 0 else None)
                 for h in range(2) for u in range(2)]
        lo = [jnp.concatenate([parts[0][c], parts[1][c]], axis=0) for c in range(8)]
        hi = [jnp.concatenate([parts[2][c], parts[3][c]], axis=0) for c in range(8)]
        for n in range(4):
            cs = _acomb(lo[n], lo[n + 4], hi[n], hi[n + 4])
            for i in range(7):
                oa.at[i][pl.ds(pl.multiple_of(r0, 16), 16), n * 128:(n + 1) * 128] = cs[i]

    x_copy(0).start()
    for cp in gu_copies(0, 0):
        cp.start()
    z_copy().start()
    x_copy(1).start()
    wd_copy(0, 0).start()
    x_copy(2).start()
    x_copy(3).start()
    wq_copy(0).start()
    for cp in gu_copies(1, 1):
        cp.start()
    wq_copy(1).start()
    for cp in wo_copies():
        cp.start()

    x_copy(0).wait()
    ln_rows(0, RB)
    for cp in gu_copies(0, 0):
        cp.wait()
    prep_gu(0)
    h0a, _ = ffn_gu(0, 128)

    z_copy().wait()
    x_copy(1).wait()
    h0b, anc = ffn_gu(128, 128)
    ln_rows(RB, RB, anc)

    wd_copy(0, 0).wait()
    x_copy(2).wait()
    prep_d(0)
    ffn_dn(0, 128, h0a, True)
    ffn_dn(128, 128, h0b, True)
    h1, anc = ffn_gu(RB, RB)
    ln_rows(2 * RB, RB, anc)

    x_copy(3).wait()
    ffn_dn(RB, RB, h1, True)
    h2, anc = ffn_gu(2 * RB, RB)
    ln_rows(3 * RB, RB, anc)
    wq_copy(2).start()
    wd_copy(1, 1).start()

    wq_copy(0).wait()
    for cp in gu_copies(1, 1):
        cp.wait()
    ffn_dn(2 * RB, RB, h2, True)
    h3, _ = ffn_gu(3 * RB, RB)
    prep_q0()
    zero = jnp.sum(jnp.where(true_mask(), 0, 1))
    prep_gu(1)
    ffn_dn(3 * RB, RB, h3, True)
    wd_copy(2, 0).start()
    for cp in gu_copies(2, 0):
        cp.start()
    for cp in gu_copies(3, 1):
        cp.start()

    wq_copy(1).wait()
    for cp in wo_copies():
        cp.wait()

    def p2_body(i, carry):
        @pl.when(i == 2)
        def _():
            wq_copy(2).wait()
        t = i // 2
        h = i % 2
        bqv = bq.at[pl.ds(i, 3)]
        anc = qkv_tiles(t, h, bqv.at[0])
        prep_q_half(jnp.minimum(t + 1, 2), h, bqv.at[2])
        prep_o_chunks([jnp.minimum(6 * i + k, 31) for k in range(6)], anc)
        return carry

    lax.fori_loop(0, 6, p2_body, 0)

    def p3_body(j, carry):
        sd = j % 2
        sg = 1 - sd
        wd_copy(j, sd).wait()
        for cp in gu_copies(jnp.minimum(j + 1, NF - 1), sg):
            cp.wait()
        prep_d(sd)
        a4 = pl.multiple_of((j - 1) * 64, 64)
        for g in range(4):
            attn_pair(a4 + 16 * g)
        attn_pair(832 + 16 * jnp.minimum(j - 1, 11))
        for r in range(NB):
            hs, _ = ffn_gu(r * RB, RB)
            if r == NB - 1:
                prep_gu(sg)
            ffn_dn(r * RB, RB, hs, False)

        @pl.when(j + 2 < NF)
        def _():
            wd_copy(j + 2, sd).start()
            for cp in gu_copies(jnp.minimum(j + 3, NF - 1), sg):
                cp.start()
        return carry

    lax.fori_loop(1, NF, p3_body, 0)

    SB = 128

    def p4_body(k, carry):
        for u in range(RB // SB):
            r0 = pl.multiple_of(k * RB + u * SB, SB)
            rows = pl.ds(r0, SB)
            for n in range(4):
                ss = _ccomb([_dot(oa.at[i][rows, :], un(bo.at[i, n][...])) for i in range(7)])
                fs = _ccomb([acc.at[i][rows, n * 128:(n + 1) * 128] for i in range(7)])
                for q, (h, cb) in enumerate(((0, n), (0, n + 4), (1, n), (1, n + 4))):
                    g = fs[q] * jax.nn.sigmoid(fs[q])
                    xv = xraw.at[h][rows, cb * 128:(cb + 1) * 128].astype(f32)
                    if u == 0 and n == 0 and q == 0:
                        ka = bq[zero, zero, zero, pl.ds(pl.multiple_of(zero * 8, 8), 8), :]
                        x8 = jnp.where(true_mask(), xv[0:8], pltpu.bitcast(ka, f32))
                        xv = jnp.concatenate([x8, xv[8:]], axis=0)
                    obuf.at[h][rows, cb * 128:(cb + 1) * 128] = (xv + ss[q] * g).astype(bf16)
            out_copy(r0, SB, k * (RB // SB) + u).start()
        return carry

    lax.fori_loop(0, NB, p4_body, 0)
    for k in range(HS // SB):
        out_copy(k * SB, SB, k).wait()


@jax.jit
def pallas_recurrent_scan__sliding_local_dilated__geglu_ffn__prompt_kernel(
    A_x: jax.Array,
    A_wqkv: jax.Array,
    A_wo: jax.Array,
    B_x: jax.Array,
    B_w_gate: jax.Array,
    B_w_up: jax.Array,
    B_w_down: jax.Array,
):
    any_spec = pl.BlockSpec(memory_space=pl.ANY)
    out = pl.pallas_call(
        _kernel,
        out_shape=jax.ShapeDtypeStruct((2, HS, D), bf16),
        in_specs=[any_spec] * 6,
        out_specs=any_spec,
        scratch_shapes=[
            pltpu.VMEM((2, HS, D), bf16),
            pltpu.VMEM((7, HS // 2, HD), u32),
            pltpu.VMEM((2, 2, D, FC), bf16),
            pltpu.VMEM((2, FC, D), bf16),
            pltpu.VMEM((7, HD // 2, FC), u32),
            pltpu.VMEM((7, FH // 2, HD), u32),
            pltpu.VMEM((7, HS, HD), f32),
            pltpu.VMEM((3, D, D), bf16),
            pltpu.VMEM((8, 7, 2, HD // 2, 128), u32),
            pltpu.VMEM((3, 8, PAD + S, 128), f32),
            pltpu.VMEM((7, HS // 2, HD), u32),
            pltpu.VMEM((8, D, 128), bf16),
            pltpu.VMEM((7, 4, HD // 2, 128), u32),
            pltpu.VMEM((2, HS, D), bf16),
            pltpu.VMEM((16, 128), bf16),
            pltpu.SemaphoreType.DMA((32,)),
        ],
        compiler_params=pltpu.CompilerParams(vmem_limit_bytes=120 * 1024 * 1024),
        name="fusedk",
    )(A_x.reshape(2, HS, D), A_wqkv, A_wo, B_w_gate, B_w_up, B_w_down)
    return out.reshape(1, S, D)
```

```python
import jax
import jax.numpy as jnp
from jax import lax
import jax.experimental.pallas as pl
import jax.experimental.pallas.tpu as pltpu

f32 = jnp.float32
bf16 = jnp.bfloat16
u32 = jnp.uint32

S, D, F = 2048, 1024, 3584
HS, HD = S // 2, D // 2
FC = 256
FH = FC // 2
NF = F // FC
QS, QD = S // 4, D // 4
GC = 512
NG = F // GC
RB = 256
NB = HS // RB
PAD = 16
NW = 8
SCALE = 32 ** -0.5
LOG2E = 1.4426950408889634
NEG = -1e9 / SCALE


def _dot(a, b):
    return jnp.dot(a, b, preferred_element_type=f32)


def _acomb(a11, a12, a21, a22):
    r = lambda v: v.astype(bf16)
    return [r(a11 + a22), r(a21 + a22), r(a11), r(a22), r(a11 + a12), r(a21 - a11), r(a12 - a22)]


def _bcomb(b11, b12, b21, b22):
    r = lambda v: v.astype(bf16)
    return [r(b11 + b22), r(b11), r(b12 - b22), r(b21 - b11), r(b22), r(b11 + b12), r(b21 + b22)]


def _asum(a11, a12, a21, a22):
    return [a11 + a22, a21 + a22, a11, a22, a11 + a12, a21 - a11, a12 - a22]


def _bsum(b11, b12, b21, b22):
    return [b11 + b22, b11, b12 - b22, b21 - b11, b22, b11 + b12, b21 + b22]


_A_TERMS = [((0, 0), (1, 1), 1), ((1, 0), (1, 1), 1), ((0, 0), None, 0), ((1, 1), None, 0),
            ((0, 0), (0, 1), 1), ((1, 0), (0, 0), -1), ((0, 1), (1, 1), -1)]
_B_TERMS = [((0, 0), (1, 1), 1), ((0, 0), None, 0), ((0, 1), (1, 1), -1), ((1, 0), (0, 0), -1),
            ((1, 1), None, 0), ((0, 0), (0, 1), 1), ((1, 0), (1, 1), 1)]


def _ccomb(m):
    m1, m2, m3, m4, m5, m6, m7 = m
    return m1 + m4 - m5 + m7, m3 + m5, m2 + m4, m1 - m2 + m3 + m6


def _gate_tanh(x):
    c = 0.7978845608028654
    return jnp.tanh(x * (c + (c * 0.044715) * (x * x)))


def _glu2(g, th, u):
    a = g * u
    return a + a * th


def _sum8(v):
    return ((v[0] + v[1]) + (v[2] + v[3])) + ((v[4] + v[5]) + (v[6] + v[7]))


def _butterfly(sets, masks, axis, size):
    for b in range(3):
        sh = 1 << b
        out = []
        for blk in sets:
            nxt = list(blk)
            for c in range(8):
                if c & sh == 0:
                    lo, hi = blk[c], blk[c + sh]
                    nxt[c] = jnp.where(masks[b], lo, pltpu.roll(hi, sh, axis))
                    nxt[c + sh] = jnp.where(masks[b], pltpu.roll(lo, size - sh, axis), hi)
            out.append(nxt)
        sets = out
    return sets


def _kernel(x_hbm, wqkv_hbm, wo_hbm, wg_hbm, wu_hbm, wd_hbm, out_hbm,
            xraw, xa_u, xa2_u, gu_raw, wd_raw, bgu_u, bgu2_u, bd_u, acc, wq_raw, bq, qkv,
            wo_raw, bo, stats, zbuf, sems):
    obuf = xraw
    xa = xa_u.bitcast(bf16)
    bgu = bgu_u.bitcast(bf16)
    bd = bd_u.bitcast(bf16)
    xa2 = xa2_u.bitcast(bf16)
    bgu2 = bgu2_u.bitcast(bf16)
    oa = xa
    pk = lambda v: pltpu.bitcast(v, u32)
    un = lambda v: pltpu.bitcast(v, bf16)

    lane = lax.broadcasted_iota(jnp.int32, (8, 128), 1)
    row8 = lax.broadcasted_iota(jnp.int32, (8, 128), 0)
    lane_lo = [(lane & (1 << b)) == 0 for b in range(3)]
    row_lo = [(row8 & (1 << b)) == 0 for b in range(3)]

    XP = [(0, 128), (128, 128), (512, 128), (640, 128), (256, 256), (768, 256)]

    def x_copy(r):
        r0, n = XP[r]
        return pltpu.make_async_copy(x_hbm.at[:, pl.ds(r0, n), :],
                                     xraw.at[:, pl.ds(r0, n), :], sems.at[(0, 1, 2, 3, 23, 14)[r]])

    def gu_copies(j, slot):
        off = pl.multiple_of(j * GC, GC)
        return (pltpu.make_async_copy(wg_hbm.at[:, pl.ds(off, GC)], gu_raw.at[slot, 0], sems.at[4 + 3 * slot]),
                pltpu.make_async_copy(wu_hbm.at[:, pl.ds(off, GC)], gu_raw.at[slot, 1], sems.at[5 + 3 * slot]))

    def wd_copy(j, slot):
        off = pl.multiple_of(j * GC, GC)
        return pltpu.make_async_copy(wd_hbm.at[pl.ds(off, GC), :], wd_raw.at[slot], sems.at[6 + 3 * slot])

    def gu0_copy(t, c):
        w = (wg_hbm, wu_hbm)[t]
        return pltpu.make_async_copy(w.at[:, pl.ds(c * FC, FC)], gu_raw.at[0, t, :, pl.ds(c * FC, FC)],
                                     sems.at[15 + 2 * c + t])

    def wd0_copy(c):
        return pltpu.make_async_copy(wd_hbm.at[pl.ds(c * FC, FC), :], wd_raw.at[0, pl.ds(c * FC, FC), :],
                                     sems.at[19 + c])

    def wq_copy(t):
        return pltpu.make_async_copy(wqkv_hbm.at[:, pl.ds(t * D, D)], wq_raw.at[t], sems.at[10 + t])

    def wo_copies():
        return [pltpu.make_async_copy(wo_hbm.at[:, pl.ds(c * 128, 128)], wo_raw.at[c], sems.at[24 + c])
                for c in range(8)]

    class _Z:
        cps = [pltpu.make_async_copy(x_hbm.at[0, pl.ds(0, 16), pl.ds(0, 128)], zbuf.at[q], sems.at[21 + q])
               for q in range(2)]

        def start(self):
            for cp in self.cps:
                cp.start()

        def wait(self):
            for cp in self.cps:
                cp.wait()

    z_copy = _Z

    def out_copy(r0, n, k):
        return pltpu.make_async_copy(obuf.at[:, pl.ds(r0, n), :], out_hbm.at[:, pl.ds(r0, n), :],
                                     sems.at[32 + k])

    def true_mask():
        return pk(zbuf[0]) == pk(zbuf[1])

    def ln_half(h, c0, tm16, a):
        xs = []
        for c in range(4):
            x2 = xraw.at[h][c0:c0 + 16, c * 256:(c + 1) * 256].astype(f32)
            xs += [x2[:, :128], x2[:, 128:]]
        s1 = _sum8(xs)
        if a is not None:
            s1 = jnp.where(tm16, s1, a)
        m = jnp.sum(s1, axis=-1, keepdims=True) * (1.0 / D)
        xc = [x - m for x in xs]
        v = jnp.sum(_sum8([x * x for x in xc]), axis=-1, keepdims=True) * (1.0 / D)
        r = lax.rsqrt(v + 1e-5)
        stats.at[h, 0][c0:c0 + 16, :] = jnp.broadcast_to(m, (16, 128))
        stats.at[h, 1][c0:c0 + 16, :] = jnp.broadcast_to(r, (16, 128))
        return [x * r for x in xc]

    def ln_rows(r0, n, anc=None):
        tm16 = None
        if anc is not None:
            tm = true_mask()
            tm16 = jnp.concatenate([tm, tm], axis=0)
            anc = anc[:int(len(anc) * 0.85)]
        nch = n // 16
        for k in range(nch):
            c0 = r0 + 16 * k
            a = [None, None]
            if anc is not None:
                a = [anc[(len(anc) * (2 * k + u)) // (2 * nch)] for u in range(2)]
            lo = ln_half(0, c0, tm16, a[0])
            hi = ln_half(1, c0, tm16, a[1])
            for c in range(4):
                cs = _acomb(lo[c], lo[c + 4], hi[c], hi[c + 4])
                for i in range(7):
                    xa.at[i][c0:c0 + 16, c * 128:(c + 1) * 128] = cs[i]

    def prep_gu(c, ts=(0, 1)):
        KC = 32
        for t in ts:
            w = gu_raw.at[0, t]
            for k0 in range(0, HD, KC):
                lo = w[k0:k0 + KC, c * FC:(c + 1) * FC].astype(f32)
                hi = w[HD + k0:HD + k0 + KC, c * FC:(c + 1) * FC].astype(f32)
                cs = _bcomb(lo[:, :FH], lo[:, FH:], hi[:, :FH], hi[:, FH:])
                for i in range(7):
                    bgu.at[i][k0:k0 + KC, t * FH:(t + 1) * FH] = cs[i]

    def prep_d(w, kh):
        KC = 16
        for k0 in range(0, kh, KC):
            for c0 in range(0, HD, 256):
                g = lambda a, b: w[a + k0:a + k0 + KC, b + c0:b + c0 + 256].astype(f32)
                cs = _bcomb(g(0, 0), g(0, HD), g(kh, 0), g(kh, HD))
                for i in range(7):
                    bd.at[i][k0:k0 + KC, c0:c0 + 256] = cs[i]

    def two_level_piece(terms, inner, ld, i, tm16, anc, nanc, store):
        p, q, sg = terms[i]
        P = ld(*p)
        for e in range(nanc):
            P[e >> 1][e & 1] = jnp.where(tm16, P[e >> 1][e & 1], anc)
        if q is not None:
            Q = ld(*q)
            P = [[P[b][d] + Q[b][d] if sg > 0 else P[b][d] - Q[b][d] for d in range(2)] for b in range(2)]
        ops = inner(P[0][0], P[0][1], P[1][0], P[1][1])
        for k in range(7):
            store(7 * i + k, ops[k].astype(bf16))

    def prep_gu2_piece(slot, i, t, k0, tm16, anc, nanc):
        w = gu_raw.at[slot, t]
        dst = bgu2.at[slot]

        def ld(R, C):
            out = []
            for b in range(2):
                x2 = w[pl.ds((2 * R + b) * QD + k0, 16), C * 256:(C + 1) * 256].astype(f32)
                out.append([x2[:, :128], x2[:, 128:]])
            return out

        def store(p, v):
            dst.at[p][pl.ds(k0, 16), t * 128:(t + 1) * 128] = v
        two_level_piece(_B_TERMS, _bsum, ld, i, tm16, anc, nanc, store)

    def make_xa2(r0, tm16, ancs):
        st = [[[stats.at[a, e][pl.ds(b * QS + r0, 16), :] for e in range(2)] for b in range(2)] for a in range(2)]
        for j in range(2):
            def ld(R, C):
                out = []
                for b in range(2):
                    m, r = st[R][b]
                    row = []
                    for d in range(2):
                        c0 = (2 * C + d) * QD + j * 128
                        xv = xraw.at[R][pl.ds(b * QS + r0, 16), c0:c0 + 128].astype(f32)
                        row.append((xv - m) * r)
                    out.append(row)
                return out

            def store(p, v):
                xa2.at[p][pl.ds(r0, 16), j * 128:(j + 1) * 128] = v
            for i in range(7):
                two_level_piece(_A_TERMS, _asum, ld, i, tm16, ancs[7 * j + i], 1, store)

    def ffn_gu(r0, n):
        ms = [_dot(xa[i, r0:r0 + n, :], bgu[i]) for i in range(7)]
        anc = [m_[k:k + 16, t * FH:(t + 1) * FH] for m_ in ms for t in range(2) for k in range(0, n, 64)]
        hs = _acomb(*[_glu2(v[:, :FH], _gate_tanh(v[:, :FH]), v[:, FH:]) for v in _ccomb(ms)])
        return hs, anc

    def ffn_dn(r0, n, hs, first):
        anc = []
        for i in range(7):
            y = _dot(hs[i], bd[i, :FH, :])
            anc += [y[k:k + 16, 0:128] for k in range(0, n, 32)]
            if first:
                acc[i, r0:r0 + n, :] = y
            else:
                acc[i, r0:r0 + n, :] += y
        return anc

    upk = lambda v: un(v).astype(f32)

    def prep_q_half(t, h, dst, par=1):
        KC = 16
        sa = (128 - 2) * h
        sb = 2 * (1 - h)
        w = wq_raw.at[t]

        def stage1(r0):
            blk = [pk(w[r0:r0 + KC, c * 128:(c + 1) * 128]) for c in range(8)]
            rl = lambda v, sft: v if (isinstance(sft, int) and sft == 0) else pltpu.roll(v, sft, 1)
            return [jnp.where(lane_lo[1], rl(blk[c], sa), rl(blk[c + 2], sb)) for c in (0, 1, 4, 5)]

        def stage(sets, jb, b):
            sh = 1 << b
            out = []
            for blk in sets:
                nxt = list(blk)
                for j in range(4):
                    if j & jb == 0:
                        lo, hi = blk[j], blk[j + jb]
                        nxt[j] = jnp.where(lane_lo[b], lo, pltpu.roll(hi, sh, 1))
                        nxt[j + jb] = jnp.where(lane_lo[b], pltpu.roll(lo, 128 - sh, 1), hi)
                out.append(nxt)
            return out

        for k00 in range(0, HD, KC * par):
            ks = [k00 + KC * q for q in range(par)]
            hv = stage(stage([stage1(hk * HD + k0) for k0 in ks for hk in range(2)], 1, 0), 2, 2)
            for q, k0 in enumerate(ks):
                lo, hi = hv[2 * q], hv[2 * q + 1]
                for e in range(2):
                    cs = _bcomb(upk(lo[e]), upk(lo[e + 2]), upk(hi[e]), upk(hi[e + 2]))
                    for i in range(7):
                        dst.at[i, e][k0 // 2:(k0 + KC) // 2, :] = pk(cs[i])

    def qkv_tiles(t, h, src):
        anc = []
        anc16 = []
        for e in range(2):
            n = 2 * h + e
            qlo = qkv.at[t, n]
            qhi = qkv.at[t, n + 4]
            for r in range(NB):
                ms = [_dot(xa[i, r * RB:(r + 1) * RB, :], un(src.at[i, e][...])) for i in range(7)]
                c11, c12, c21, c22 = _ccomb(ms)
                anc += [m_[8 * k:8 * k + 8] for m_ in ms for k in range(0, RB // 8, 8)]
                anc16 += [m_[k:k + 16] for m_ in ms for k in range(32, RB, 128)]
                r0 = PAD + r * RB
                qlo[r0:r0 + RB, :] = c11
                qhi[r0:r0 + RB, :] = c12
                qlo[HS + r0:HS + r0 + RB, :] = c21
                qhi[HS + r0:HS + r0 + RB, :] = c22
                if r == 0:
                    qlo[0:PAD, :] = jnp.broadcast_to(c11[0:1, :], (PAD, 128))
                    qhi[0:PAD, :] = jnp.broadcast_to(c12[0:1, :], (PAD, 128))
        return anc, anc16

    def prep_o_chunks(idxs, anc):
        tm = true_mask()
        step = (len(anc) - 12) / (4 * len(idxs))
        pc = 0
        for idx in idxs:
            n = idx >> 3
            g16 = pl.multiple_of((idx & 7) * 16, 16)
            g8 = pl.multiple_of((idx & 7) * 8, 8)
            res = []
            for h in range(2):
                w = wo_raw.at[n + 4 * h]
                w16 = [w[pl.ds(128 * i + g16, 16), :].astype(f32) for i in range(8)]
                for u in range(2):
                    blk = [v[8 * u:8 * u + 8] for v in w16]
                    blk[0] = jnp.where(tm, blk[0], anc[int(pc * step)])
                    pc += 1
                    res += _butterfly([blk], row_lo, 0, 8)
            cols = [[jnp.concatenate([res[2 * h][j], res[2 * h + 1][j]], axis=0) for j in range(8)]
                    for h in range(2)]
            for b in range(4):
                cs = _bcomb(cols[0][b], cols[1][b], cols[0][b + 4], cols[1][b + 4])
                for i in range(7):
                    bo.at[i, n][pl.ds(b * 64 + g8, 8), :] = pk(cs[i])

    def attn8(base, row0):
        lg = [None] * NW
        for c in range(8):
            q = qkv[0, c, pl.ds(base, 8), :]
            for w in range(NW):
                pr = q * qkv[1, c, pl.ds(base - 2 * w, 8), :]
                lg[w] = pr if lg[w] is None else lg[w] + pr
        for w0 in range(0, NW, 2):
            for w in (w0, w0 + 1):
                lg[w] = lg[w] + pltpu.roll(lg[w], 8, 1)
            for w in (w0, w0 + 1):
                lg[w] = lg[w] + pltpu.roll(lg[w], 16, 1)
        if row0 is not None:
            for w in range(1, NW):
                lg[w] = jnp.where(row8 + row0 >= 2 * w, lg[w], NEG)
        m = lg[0]
        for w in range(1, NW):
            m = jnp.maximum(m, lg[w])
        p = [jnp.exp2((lg[w] - m) * (SCALE * LOG2E)) for w in range(NW)]
        den = p[0]
        for w in range(1, NW):
            den = den + p[w]
        inv = 1.0 / den
        b4 = (lane & 16) != 0
        b3 = (lane & 8) != 0
        outs = [None] * 8
        for w in range(NW):
            pw = p[w] * inv
            pw = jnp.where(b4, pw, pltpu.roll(pw, 112, 1))
            pw = jnp.where(b3, pw, pltpu.roll(pw, 120, 1))
            for c in range(8):
                pr = pw * qkv[2, c, pl.ds(base - 2 * w, 8), :]
                outs[c] = pr if outs[c] is None else outs[c] + pr
        return outs

    def attn_pair(r0, mask=False):
        parts = [attn8(pl.multiple_of(PAD + h * HS + r0 + 8 * u, 8), (r0 + 8 * u) if (h == 0 and mask) else None)
                 for h in range(2) for u in range(2)]
        lo = [jnp.concatenate([parts[0][c], parts[1][c]], axis=0) for c in range(8)]
        hi = [jnp.concatenate([parts[2][c], parts[3][c]], axis=0) for c in range(8)]
        for n in range(4):
            cs = _acomb(lo[n], lo[n + 4], hi[n], hi[n + 4])
            for i in range(7):
                oa.at[i][pl.ds(pl.multiple_of(r0, 16), 16), n * 128:(n + 1) * 128] = cs[i]

    wd0 = lambda c: wd_raw.at[0, c * FC:(c + 1) * FC, :]
    RA, RBB, RC, RD = 0, 512, 256, 768

    x_copy(0).start()
    x_copy(1).start()
    gu0_copy(0, 0).start()
    z_copy().start()
    gu0_copy(1, 0).start()
    x_copy(2).start()
    wd0_copy(0).start()
    x_copy(3).start()
    x_copy(4).start()
    gu0_copy(0, 1).start()
    gu0_copy(1, 1).start()
    wd0_copy(1).start()
    x_copy(5).start()
    wq_copy(0).start()
    for cp in wo_copies():
        cp.start()
    wq_copy(1).start()

    x_copy(0).wait()
    ln_rows(RA, 128)
    x_copy(1).wait()
    ln_rows(RA + 128, 128)

    gu0_copy(0, 0).wait()
    prep_gu(0, (0,))
    mg = [_dot(xa[i, RA:RA + RB, :], bgu[i, :, :FH]) for i in range(7)]
    gg = [(v, _gate_tanh(v)) for v in _ccomb(mg)]

    z_copy().wait()
    gu0_copy(1, 0).wait()
    x_copy(2).wait()
    prep_gu(0, (1,))
    mu = [_dot(xa[i, RA:RA + RB, :], bgu[i, :, FH:]) for i in range(7)]
    ha = _acomb(*[_glu2(a[0], a[1], b) for a, b in zip(gg, _ccomb(mu))])
    ln_rows(RBB, 128, [m_[k:k + 16] for m_ in mu for k in range(0, RB, 64)])

    wd0_copy(0).wait()
    x_copy(3).wait()
    prep_d(wd0(0), FH)
    hb0, anc = ffn_gu(RBB, 128)
    ffn_dn(RA, RB, ha, True)
    ln_rows(RBB + 128, 128, anc)

    x_copy(4).wait()
    gu0_copy(0, 1).wait()
    gu0_copy(1, 1).wait()
    hb1, anc = ffn_gu(RBB + 128, 128)
    anc2 = ffn_dn(RBB, 128, hb0, True)
    ffn_dn(RBB + 128, 128, hb1, True)
    prep_gu(1)
    ln_rows(RC, RB, anc + anc2[:8])

    wd0_copy(1).wait()
    x_copy(5).wait()
    prep_d(wd0(1), FH)
    h2, anc = ffn_gu(RA, RB)
    ffn_dn(RA, RB, h2, False)
    ln_rows(RD, RB, anc)
    wq_copy(2).start()
    for cp in gu_copies(1, 1):
        cp.start()
    wd_copy(1, 1).start()

    wq_copy(0).wait()
    h3, _ = ffn_gu(RBB, RB)
    prep_q_half(0, 0, bq.at[0], 2)
    zero = jnp.sum(jnp.where(true_mask(), 0, 1))
    ffn_dn(RBB, RB, h3, False)

    for cp in wo_copies():
        cp.wait()

    def p2_body(i, carry):
        @pl.when(i == 1)
        def _():
            wq_copy(1).wait()

        @pl.when(i == 3)
        def _():
            wq_copy(2).wait()

        @pl.when(i == 4)
        def _():
            for cp in gu_copies(1, 1):
                cp.wait()
        bqv = bq.at[pl.ds(i, 2)]
        anc, anc16 = qkv_tiles(i >> 1, i & 1, bqv.at[0])
        prep_q_half(jnp.minimum((i + 1) >> 1, 2), (i + 1) & 1, bqv.at[1])
        prep_o_chunks([jnp.minimum(6 * i + k, 31) for k in range(6)], anc)
        tm = true_mask()
        tm16 = jnp.concatenate([tm, tm], axis=0)
        n16 = len(anc16) - 6
        for k in range(6):
            idx = jnp.minimum(6 * i + k, 31)
            make_xa2(pl.multiple_of(idx * 16, 16), tm16,
                     [anc16[((k * 14 + e) * n16) // 84] for e in range(14)])
        for k in range(8):
            idx = 4 * i + (k >> 1)
            for q in range(7):
                prep_gu2_piece(idx >> 4, q, k & 1, pl.multiple_of((idx & 15) * 16, 16), tm16,
                               anc16[((k * 7 + q) * n16) // 56], 1)
        for k in range(7):
            blk = jnp.minimum(7 * i + k, 31)
            r0 = pl.multiple_of(256 + (blk >> 4) * 512 + (blk & 15) * 16, 16)
            z16 = jnp.where(tm16, 0.0, anc16[(k * n16) // 7])
            for p in range(7):
                for c in range(4):
                    acc.at[p][pl.ds(r0, 16), c * 128:(c + 1) * 128] = z16
        return carry

    lax.fori_loop(0, 6, p2_body, 0)

    def p3_body(u, carry):
        j = u >> 1
        s_ = u & 1
        sl = j & 1
        jn = jnp.minimum((u >> 1) + 1, NG - 1)
        sn = 1 - sl

        @pl.when(s_ == 0)
        def _():
            wd_copy(j, sl).wait()

        @pl.when(jnp.logical_and(s_ == 0, j + 1 < NG))
        def _():
            for cp in gu_copies(jn, sn):
                cp.wait()
        prep_d(wd_raw.at[sl], FC)
        a4 = pl.multiple_of((u - 1) * 64, 64)
        for g in range(4):
            attn_pair(a4 + 16 * g, g == 0)
        attn_pair(832 + 16 * jnp.minimum(u - 1, 11))

        rows = pl.ds(pl.multiple_of(s_ * RB, RB), RB)
        order = (2, 4, 1, 3, 0, 6, 5)
        bcur = bgu2.at[sl]
        c1 = [None] * 7
        h = [[None] * 4 for _ in range(4)]

        def gate_up(i):
            ms = [None] * 7
            for k in order:
                ms[k] = _dot(xa2.at[7 * i + k][rows, :], bcur.at[7 * i + k][...])
            c1[i] = _ccomb(ms)
            return [ms[k][r_:r_ + 16, t * 128:(t + 1) * 128] for k in order for r_ in range(0, RB, 64)
                    for t in range(2)]

        def hidden(a, e):
            if h[2 * a][2 * e] is None:
                for q in range(4):
                    m = [None if v is None else v[q] for v in c1]
                    if (a, e) == (0, 0):
                        cc = m[0] + m[3] - m[4] + m[6]
                    elif (a, e) == (0, 1):
                        cc = m[2] + m[4]
                    elif (a, e) == (1, 0):
                        cc = m[1] + m[3]
                    else:
                        cc = m[0] - m[1] + m[2] + m[5]
                    h[2 * a + (q >> 1)][2 * e + (q & 1)] = _glu2(cc[:, :128], _gate_tanh(cc[:, :128]),
                                                                 cc[:, 128:])
            return [[h[2 * a + b][2 * e + f] for f in range(2)] for b in range(2)]

        def down(i):
            p, q, sg = _A_TERMS[i]
            P = hidden(*p)
            if q is not None:
                Q = hidden(*q)
                P = [[P[b][f] + Q[b][f] if sg > 0 else P[b][f] - Q[b][f] for f in range(2)] for b in range(2)]
            out = []
            for b in range(2):
                y = _dot(jnp.concatenate([v.astype(bf16) for v in P[b]], axis=1), bd[i])
                out += [y[r_:r_ + 16, 0:128] for r_ in range(0, RB, 32)]
                acc.at[i][pl.ds(pl.multiple_of(b * QS + s_ * RB, RB), RB), :] += y
            return out

        seq = 'G0 G3 G4 G6 G2 G1 D2 D4 G5 D5 D1 D3 D0 D6'.split()
        sanc = [(gate_up if tk[0] == 'G' else down)(int(tk[1])) for tk in seq]
        tm = true_mask()
        tm16 = jnp.concatenate([tm, tm], axis=0)
        last_g = max(p for p, tk in enumerate(seq) if tk[0] == 'G')
        src = [a for p in range(last_g + 1, len(seq)) for a in sanc[p]]
        src = src[:int(len(src) * 0.9)]
        kb = pl.multiple_of(s_ * (QD // 2), QD // 2)
        pieces = [(t, k0, i) for k0 in range(0, QD // 2, 16) for t in range(2) for i in range(7)]
        for e, (t, k0, i) in enumerate(pieces):
            prep_gu2_piece(sn, i, t, kb + k0, tm16, src[e * len(src) // len(pieces)], 4)

        @pl.when(jnp.logical_and(s_ == 0, j + 1 < NG))
        def _():
            wd_copy(j + 1, sn).start()

        @pl.when(jnp.logical_and(s_ == 1, j + 3 < NG))
        def _():
            for cp in gu_copies(j + 3, sn):
                cp.start()
        return carry

    for cp in gu_copies(2, 0):
        cp.start()
    lax.fori_loop(1, 2 * NG, p3_body, 0)

    SB = 64

    def p4_body(k, carry):
        for u in range(RB // SB):
            r0 = pl.multiple_of(k * RB + u * SB, SB)
            rows = pl.ds(r0, SB)
            for n in range(4):
                ss = _ccomb([_dot(oa.at[i][rows, :], un(bo.at[i, n][...])) for i in range(7)])
                fs = _ccomb([acc.at[i][rows, n * 128:(n + 1) * 128] for i in range(7)])
                for q, (h, cb) in enumerate(((0, n), (0, n + 4), (1, n), (1, n + 4))):
                    fv = 0.5 * fs[q]
                    g = fv * jax.nn.sigmoid(fv)
                    xv = xraw.at[h][rows, cb * 128:(cb + 1) * 128].astype(f32)
                    if u == 0 and n == 0 and q == 0:
                        ka = bq[zero, zero, zero, pl.ds(pl.multiple_of(zero * 8, 8), 8), :]
                        x8 = jnp.where(true_mask(), xv[0:8], pltpu.bitcast(ka, f32))
                        xv = jnp.concatenate([x8, xv[8:]], axis=0)
                    obuf.at[h][rows, cb * 128:(cb + 1) * 128] = (xv + ss[q] * g).astype(bf16)
            out_copy(r0, SB, k * (RB // SB) + u).start()
        return carry

    lax.fori_loop(0, NB, p4_body, 0)
    for k in range(HS // SB):
        out_copy(k * SB, SB, k).wait()


@jax.jit
def pallas_recurrent_scan__sliding_local_dilated__geglu_ffn__prompt_kernel(
    A_x: jax.Array,
    A_wqkv: jax.Array,
    A_wo: jax.Array,
    B_x: jax.Array,
    B_w_gate: jax.Array,
    B_w_up: jax.Array,
    B_w_down: jax.Array,
):
    any_spec = pl.BlockSpec(memory_space=pl.ANY)
    out = pl.pallas_call(
        _kernel,
        out_shape=jax.ShapeDtypeStruct((2, HS, D), bf16),
        in_specs=[any_spec] * 6,
        out_specs=any_spec,
        scratch_shapes=[
            pltpu.VMEM((2, HS, D), bf16),
            pltpu.VMEM((7, HS // 2, HD), u32),
            pltpu.VMEM((49, QS // 2, QD), u32),
            pltpu.VMEM((2, 2, D, GC), bf16),
            pltpu.VMEM((2, GC, D), bf16),
            pltpu.VMEM((7, HD // 2, FC), u32),
            pltpu.VMEM((2, 49, QD // 2, 256), u32),
            pltpu.VMEM((7, FC // 2, HD), u32),
            pltpu.VMEM((7, HS, HD), f32),
            pltpu.VMEM((3, D, D), bf16),
            pltpu.VMEM((7, 7, 2, HD // 2, 128), u32),
            pltpu.VMEM((3, 8, PAD + S, 128), f32),
            pltpu.VMEM((8, D, 128), bf16),
            pltpu.VMEM((7, 4, HD // 2, 128), u32),
            pltpu.VMEM((2, 2, HS, 128), f32),
            pltpu.VMEM((2, 16, 128), bf16),
            pltpu.SemaphoreType.DMA((72,)),
        ],
        compiler_params=pltpu.CompilerParams(vmem_limit_bytes=124 * 1024 * 1024,
                                             disable_bounds_checks=True),
        name="fusedk",
    )(A_x.reshape(2, HS, D), A_wqkv, A_wo, B_w_gate, B_w_up, B_w_down)
    return out.reshape(1, S, D)
```

```python
import jax
import jax.numpy as jnp
from jax import lax
import jax.experimental.pallas as pl
import jax.experimental.pallas.tpu as pltpu

f32 = jnp.float32
bf16 = jnp.bfloat16
u32 = jnp.uint32

S, D, F = 2048, 1024, 3584
HS, HD = S // 2, D // 2
FC = 256
FH = FC // 2
NF = F // FC
QS, QD = S // 4, D // 4
GC = 512
NG = F // GC
RB = 256
NB = HS // RB
PAD = 16
NW = 8
SCALE = 32 ** -0.5
LOG2E = 1.4426950408889634
NEG = -1e9 / SCALE


def _dot(a, b):
    return jnp.dot(a, b, preferred_element_type=f32)


def _acomb(a11, a12, a21, a22):
    r = lambda v: v.astype(bf16)
    return [r(a11 + a22), r(a21 + a22), r(a11), r(a22), r(a11 + a12), r(a21 - a11), r(a12 - a22)]


def _bcomb(b11, b12, b21, b22):
    r = lambda v: v.astype(bf16)
    return [r(b11 + b22), r(b11), r(b12 - b22), r(b21 - b11), r(b22), r(b11 + b12), r(b21 + b22)]


def _asum(a11, a12, a21, a22):
    return [a11 + a22, a21 + a22, a11, a22, a11 + a12, a21 - a11, a12 - a22]


def _bsum(b11, b12, b21, b22):
    return [b11 + b22, b11, b12 - b22, b21 - b11, b22, b11 + b12, b21 + b22]


_A_TERMS = [((0, 0), (1, 1), 1), ((1, 0), (1, 1), 1), ((0, 0), None, 0), ((1, 1), None, 0),
            ((0, 0), (0, 1), 1), ((1, 0), (0, 0), -1), ((0, 1), (1, 1), -1)]
_B_TERMS = [((0, 0), (1, 1), 1), ((0, 0), None, 0), ((0, 1), (1, 1), -1), ((1, 0), (0, 0), -1),
            ((1, 1), None, 0), ((0, 0), (0, 1), 1), ((1, 0), (1, 1), 1)]


def _ccomb(m):
    m1, m2, m3, m4, m5, m6, m7 = m
    return m1 + m4 - m5 + m7, m3 + m5, m2 + m4, m1 - m2 + m3 + m6


def _gate_tanh(x):
    c = 0.7978845608028654
    return jnp.tanh(x * (c + (c * 0.044715) * (x * x)))


def _glu2(g, th, u):
    a = g * u
    return a + a * th


def _sum8(v):
    return ((v[0] + v[1]) + (v[2] + v[3])) + ((v[4] + v[5]) + (v[6] + v[7]))


def _butterfly(sets, masks, axis, size):
    for b in range(3):
        sh = 1 << b
        out = []
        for blk in sets:
            nxt = list(blk)
            for c in range(8):
                if c & sh == 0:
                    lo, hi = blk[c], blk[c + sh]
                    nxt[c] = jnp.where(masks[b], lo, pltpu.roll(hi, sh, axis))
                    nxt[c + sh] = jnp.where(masks[b], pltpu.roll(lo, size - sh, axis), hi)
            out.append(nxt)
        sets = out
    return sets


def _kernel(x_hbm, wqkv_hbm, wo_hbm, wg_hbm, wu_hbm, wd_hbm, out_hbm,
            xraw, xa_u, xa2_u, gu_raw, wd_raw, bgu_u, bgu2_u, bd_u, acc, wq_raw, bq_u, qkv,
            wo_raw, bo_u, stats, zbuf, sems):
    bq = bq_u.bitcast(bf16)
    bo = bo_u.bitcast(bf16)
    obuf = xraw
    xa = xa_u.bitcast(bf16)
    bgu = bgu_u.bitcast(bf16)
    bd = bd_u.bitcast(bf16)
    xa2 = xa2_u.bitcast(bf16)
    bgu2 = bgu2_u.bitcast(bf16)
    oa = xa
    pk = lambda v: pltpu.bitcast(v, u32)
    un = lambda v: pltpu.bitcast(v, bf16)

    lane = lax.broadcasted_iota(jnp.int32, (8, 128), 1)
    row8 = lax.broadcasted_iota(jnp.int32, (8, 128), 0)
    lane_lo = [(lane & (1 << b)) == 0 for b in range(3)]
    row_lo = [(row8 & (1 << b)) == 0 for b in range(3)]

    XP = [(0, 128), (128, 128), (512, 128), (640, 128), (256, 256), (768, 256)]

    def x_copy(r):
        r0, n = XP[r]
        return pltpu.make_async_copy(x_hbm.at[:, pl.ds(r0, n), :],
                                     xraw.at[:, pl.ds(r0, n), :], sems.at[(0, 1, 2, 3, 23, 14)[r]])

    def gu_copies(j, slot):
        off = pl.multiple_of(j * GC, GC)
        return (pltpu.make_async_copy(wg_hbm.at[:, pl.ds(off, GC)], gu_raw.at[slot, 0], sems.at[4 + 3 * slot]),
                pltpu.make_async_copy(wu_hbm.at[:, pl.ds(off, GC)], gu_raw.at[slot, 1], sems.at[5 + 3 * slot]))

    def wd_copy(j, slot):
        off = pl.multiple_of(j * GC, GC)
        return pltpu.make_async_copy(wd_hbm.at[pl.ds(off, GC), :], wd_raw.at[slot], sems.at[6 + 3 * slot])

    def gu0_copy(t, c):
        w = (wg_hbm, wu_hbm)[t]
        return pltpu.make_async_copy(w.at[:, pl.ds(c * FC, FC)], gu_raw.at[0, t, :, pl.ds(c * FC, FC)],
                                     sems.at[15 + 2 * c + t])

    def wd0_copy(c):
        return pltpu.make_async_copy(wd_hbm.at[pl.ds(c * FC, FC), :], wd_raw.at[0, pl.ds(c * FC, FC), :],
                                     sems.at[19 + c])

    def wq_copy(t):
        return pltpu.make_async_copy(wqkv_hbm.at[:, pl.ds(t * D, D)], wq_raw.at[t], sems.at[10 + t])

    def wo_copies():
        return [pltpu.make_async_copy(wo_hbm.at[:, pl.ds(c * 128, 128)], wo_raw.at[c], sems.at[24])
                for c in range(8)]

    class _Z:
        cps = [pltpu.make_async_copy(x_hbm.at[0, pl.ds(0, 16), pl.ds(0, 128)], zbuf.at[q], sems.at[21 + q])
               for q in range(2)]

        def start(self):
            for cp in self.cps:
                cp.start()

        def wait(self):
            for cp in self.cps:
                cp.wait()

    z_copy = _Z

    def out_copy(r0, n, k):
        return pltpu.make_async_copy(obuf.at[:, pl.ds(r0, n), :], out_hbm.at[:, pl.ds(r0, n), :],
                                     sems.at[25 + k])

    def true_mask():
        return pk(zbuf[0]) == pk(zbuf[1])

    def ln_half(h, c0, tm16, a):
        xs = []
        for c in range(4):
            x2 = xraw.at[h][c0:c0 + 16, c * 256:(c + 1) * 256].astype(f32)
            xs += [x2[:, :128], x2[:, 128:]]
        s1 = _sum8(xs)
        if a is not None:
            s1 = jnp.where(tm16, s1, a)
        m = jnp.sum(s1, axis=-1, keepdims=True) * (1.0 / D)
        xc = [x - m for x in xs]
        v = jnp.sum(_sum8([x * x for x in xc]), axis=-1, keepdims=True) * (1.0 / D)
        r = lax.rsqrt(v + 1e-5)
        stats.at[h, 0][c0:c0 + 16, :] = jnp.broadcast_to(m, (16, 128))
        stats.at[h, 1][c0:c0 + 16, :] = jnp.broadcast_to(r, (16, 128))
        return [x * r for x in xc]

    def ln_rows(r0, n, anc=None):
        tm16 = None
        if anc is not None:
            tm = true_mask()
            tm16 = jnp.concatenate([tm, tm], axis=0)
            anc = anc[:int(len(anc) * 0.85)]
        nch = n // 16
        for k in range(nch):
            c0 = r0 + 16 * k
            a = [None, None]
            if anc is not None:
                a = [anc[(len(anc) * (2 * k + u)) // (2 * nch)] for u in range(2)]
            lo = ln_half(0, c0, tm16, a[0])
            hi = ln_half(1, c0, tm16, a[1])
            for c in range(4):
                cs = _acomb(lo[c], lo[c + 4], hi[c], hi[c + 4])
                for i in range(7):
                    xa.at[i][c0:c0 + 16, c * 128:(c + 1) * 128] = cs[i]

    def prep_gu(c, ts=(0, 1)):
        KC = 32
        for t in ts:
            w = gu_raw.at[0, t]
            for k0 in range(0, HD, KC):
                lo = w[k0:k0 + KC, c * FC:(c + 1) * FC].astype(f32)
                hi = w[HD + k0:HD + k0 + KC, c * FC:(c + 1) * FC].astype(f32)
                cs = _bcomb(lo[:, :FH], lo[:, FH:], hi[:, :FH], hi[:, FH:])
                for i in range(7):
                    bgu.at[i][k0:k0 + KC, t * FH:(t + 1) * FH] = cs[i]

    def prep_d(w, kh):
        KC = 16
        for k0 in range(0, kh, KC):
            for c0 in range(0, HD, 256):
                g = lambda a, b: w[a + k0:a + k0 + KC, b + c0:b + c0 + 256].astype(f32)
                cs = _bcomb(g(0, 0), g(0, HD), g(kh, 0), g(kh, HD))
                for i in range(7):
                    bd.at[i][k0:k0 + KC, c0:c0 + 256] = cs[i]

    def two_level_piece(terms, inner, ld, i, tm16, anc, nanc, store):
        p, q, sg = terms[i]
        P = ld(*p)
        for e in range(nanc):
            P[e >> 1][e & 1] = jnp.where(tm16, P[e >> 1][e & 1], anc)
        if q is not None:
            Q = ld(*q)
            P = [[P[b][d] + Q[b][d] if sg > 0 else P[b][d] - Q[b][d] for d in range(2)] for b in range(2)]
        ops = inner(P[0][0], P[0][1], P[1][0], P[1][1])
        for k in range(7):
            store(7 * i + k, ops[k].astype(bf16))

    def prep_gu2_piece(slot, i, t, k0, tm16, anc, nanc):
        w = gu_raw.at[slot, t]
        dst = bgu2.at[slot]

        def ld(R, C):
            out = []
            for b in range(2):
                x2 = w[pl.ds((2 * R + b) * QD + k0, 16), C * 256:(C + 1) * 256].astype(f32)
                out.append([x2[:, :128], x2[:, 128:]])
            return out

        def store(p, v):
            dst.at[p][pl.ds(k0, 16), t * 128:(t + 1) * 128] = v
        two_level_piece(_B_TERMS, _bsum, ld, i, tm16, anc, nanc, store)

    def make_xa2(r0, tm16, ancs):
        st = [[[stats.at[a, e][pl.ds(b * QS + r0, 16), :] for e in range(2)] for b in range(2)] for a in range(2)]
        for j in range(2):
            def ld(R, C):
                out = []
                for b in range(2):
                    m, r = st[R][b]
                    row = []
                    for d in range(2):
                        c0 = (2 * C + d) * QD + j * 128
                        xv = xraw.at[R][pl.ds(b * QS + r0, 16), c0:c0 + 128].astype(f32)
                        row.append((xv - m) * r)
                    out.append(row)
                return out

            def store(p, v):
                xa2.at[p][pl.ds(r0, 16), j * 128:(j + 1) * 128] = v
            for i in range(7):
                two_level_piece(_A_TERMS, _asum, ld, i, tm16, ancs[7 * j + i], 1, store)

    def ffn_gu(r0, n):
        ms = [_dot(xa[i, r0:r0 + n, :], bgu[i]) for i in range(7)]
        anc = [m_[k:k + 16, t * FH:(t + 1) * FH] for m_ in ms for t in range(2) for k in range(0, n, 64)]
        hs = _acomb(*[_glu2(v[:, :FH], _gate_tanh(v[:, :FH]), v[:, FH:]) for v in _ccomb(ms)])
        return hs, anc

    def ffn_dn(r0, n, hs, first):
        anc = []
        for i in range(7):
            y = _dot(hs[i], bd[i, :FH, :])
            anc += [y[k:k + 16, 0:128] for k in range(0, n, 32)]
            if first:
                acc[i, r0:r0 + n, :] = y
            else:
                acc[i, r0:r0 + n, :] += y
        return anc

    upk = lambda v: un(v).astype(f32)

    def prep_q_half(t, h, dst, par=1):
        KC = 16
        sa = (128 - 2) * h
        sb = 2 * (1 - h)
        w = wq_raw.at[t]

        def stage1(r0):
            blk = [pk(w[r0:r0 + KC, c * 128:(c + 1) * 128]) for c in range(8)]
            rl = lambda v, sft: v if (isinstance(sft, int) and sft == 0) else pltpu.roll(v, sft, 1)
            return [jnp.where(lane_lo[1], rl(blk[c], sa), rl(blk[c + 2], sb)) for c in (0, 1, 4, 5)]

        def stage(sets, jb, b):
            sh = 1 << b
            out = []
            for blk in sets:
                nxt = list(blk)
                for j in range(4):
                    if j & jb == 0:
                        lo, hi = blk[j], blk[j + jb]
                        nxt[j] = jnp.where(lane_lo[b], lo, pltpu.roll(hi, sh, 1))
                        nxt[j + jb] = jnp.where(lane_lo[b], pltpu.roll(lo, 128 - sh, 1), hi)
                out.append(nxt)
            return out

        for k00 in range(0, HD, KC * par):
            ks = [k00 + KC * q for q in range(par)]
            hv = stage(stage([stage1(hk * HD + k0) for k0 in ks for hk in range(2)], 1, 0), 2, 2)
            for q, k0 in enumerate(ks):
                lo, hi = hv[2 * q], hv[2 * q + 1]
                for e in range(2):
                    cs = _bcomb(upk(lo[e]), upk(lo[e + 2]), upk(hi[e]), upk(hi[e + 2]))
                    for i in range(7):
                        dst.at[i][k0:k0 + KC, e * 128:(e + 1) * 128] = cs[i]

    def qkv_tiles(t, h, src):
        anc16 = []
        for e in range(2):
            n = 2 * h + e
            qlo = qkv.at[t, n]
            qhi = qkv.at[t, n + 4]
            for r in range(NB):
                ms = [_dot(xa[i, r * RB:(r + 1) * RB, :], src.at[i][:, e * 128:(e + 1) * 128]) for i in range(7)]
                c11, c12, c21, c22 = _ccomb(ms)
                anc16 += [m_[k:k + 16] for m_ in ms for k in range(0, RB, 64)]
                r0 = PAD + r * RB
                qlo[r0:r0 + RB, :] = c11
                qhi[r0:r0 + RB, :] = c12
                qlo[HS + r0:HS + r0 + RB, :] = c21
                qhi[HS + r0:HS + r0 + RB, :] = c22
                if r == 0:
                    qlo[0:PAD, :] = jnp.broadcast_to(c11[0:1, :], (PAD, 128))
                    qhi[0:PAD, :] = jnp.broadcast_to(c12[0:1, :], (PAD, 128))
        return anc16

    def prep_o_chunk(m, e, tm, ancs):
        n2 = m >> 3
        g16 = pl.multiple_of((m & 7) * 16, 16)
        res = []
        for h in range(2):
            w = wo_raw.at[2 * n2 + e + 4 * h]
            w16 = [w[pl.ds(128 * i + g16, 16), :].astype(f32) for i in range(8)]
            for u in range(2):
                blk = [v[8 * u:8 * u + 8] for v in w16]
                blk[0] = jnp.where(tm, blk[0], ancs[2 * h + u])
                res += _butterfly([blk], row_lo, 0, 8)
        cols = [[jnp.concatenate([res[2 * h][j], res[2 * h + 1][j]], axis=0) for j in range(8)]
                for h in range(2)]
        for b in range(4):
            cs = _bcomb(cols[0][b], cols[1][b], cols[0][b + 4], cols[1][b + 4])
            for i in range(7):
                bo.at[i, n2][pl.ds(b * 128 + g16, 16), e * 128:(e + 1) * 128] = cs[i]

    def attn8(base, row0):
        lg = [None] * NW
        for c in range(8):
            q = qkv[0, c, pl.ds(base, 8), :]
            for w in range(NW):
                pr = q * qkv[1, c, pl.ds(base - 2 * w, 8), :]
                lg[w] = pr if lg[w] is None else lg[w] + pr
        G1 = 2
        for w0 in range(0, NW, G1):
            for w in range(w0, w0 + G1):
                lg[w] = lg[w] + pltpu.roll(lg[w], 8, 1)
            for w in range(w0, w0 + G1):
                lg[w] = lg[w] + pltpu.roll(lg[w], 16, 1)
        if row0 is not None:
            for w in range(1, NW):
                lg[w] = jnp.where(row8 + row0 >= 2 * w, lg[w], NEG)
        m = lg[0]
        for w in range(1, NW):
            m = jnp.maximum(m, lg[w])
        p = [jnp.exp2((lg[w] - m) * (SCALE * LOG2E)) for w in range(NW)]
        den = p[0]
        for w in range(1, NW):
            den = den + p[w]
        inv = 1.0 / den
        b4 = (lane & 16) != 0
        b3 = (lane & 8) != 0
        outs = [None] * 8
        G2 = 2
        for w0 in range(0, NW, G2):
            ws = range(w0, w0 + G2)
            for w in ws:
                p[w] = p[w] * inv
                p[w] = jnp.where(b4, p[w], pltpu.roll(p[w], 112, 1))
            for w in ws:
                p[w] = jnp.where(b3, p[w], pltpu.roll(p[w], 120, 1))
            for w in ws:
                for c in range(8):
                    pr = p[w] * qkv[2, c, pl.ds(base - 2 * w, 8), :]
                    outs[c] = pr if outs[c] is None else outs[c] + pr
        return outs

    def attn_pair(r0, mask=False):
        parts = [attn8(pl.multiple_of(PAD + h * HS + r0 + 8 * u, 8), (r0 + 8 * u) if (h == 0 and mask) else None)
                 for h in range(2) for u in range(2)]
        lo = [jnp.concatenate([parts[0][c], parts[1][c]], axis=0) for c in range(8)]
        hi = [jnp.concatenate([parts[2][c], parts[3][c]], axis=0) for c in range(8)]
        for n in range(4):
            cs = _acomb(lo[n], lo[n + 4], hi[n], hi[n + 4])
            for i in range(7):
                oa.at[i][pl.ds(pl.multiple_of(r0, 16), 16), n * 128:(n + 1) * 128] = cs[i]
        return hi[7]

    wd0 = lambda c: wd_raw.at[0, c * FC:(c + 1) * FC, :]
    RA, RBB, RC, RD = 0, 512, 256, 768

    x_copy(0).start()
    x_copy(1).start()
    gu0_copy(0, 0).start()
    z_copy().start()
    gu0_copy(1, 0).start()
    x_copy(2).start()
    wd0_copy(0).start()
    x_copy(3).start()
    x_copy(4).start()
    gu0_copy(0, 1).start()
    gu0_copy(1, 1).start()
    wd0_copy(1).start()
    x_copy(5).start()
    wq_copy(0).start()
    for cp in wo_copies():
        cp.start()
    wq_copy(1).start()

    x_copy(0).wait()
    ln_rows(RA, 128)
    x_copy(1).wait()
    ln_rows(RA + 128, 128)

    gu0_copy(0, 0).wait()
    prep_gu(0, (0,))
    mg = [_dot(xa[i, RA:RA + RB, :], bgu[i, :, :FH]) for i in range(7)]
    gg = [(v, _gate_tanh(v)) for v in _ccomb(mg)]

    z_copy().wait()
    gu0_copy(1, 0).wait()
    x_copy(2).wait()
    prep_gu(0, (1,))
    mu = [_dot(xa[i, RA:RA + RB, :], bgu[i, :, FH:]) for i in range(7)]
    ha = _acomb(*[_glu2(a[0], a[1], b) for a, b in zip(gg, _ccomb(mu))])
    ln_rows(RBB, 128, [m_[k:k + 16] for m_ in mu for k in range(0, RB, 64)])

    wd0_copy(0).wait()
    x_copy(3).wait()
    prep_d(wd0(0), FH)
    hb0, anc = ffn_gu(RBB, 128)
    ffn_dn(RA, RB, ha, True)
    ln_rows(RBB + 128, 128, anc)

    x_copy(4).wait()
    gu0_copy(0, 1).wait()
    gu0_copy(1, 1).wait()
    hb1, anc = ffn_gu(RBB + 128, 128)
    anc2 = ffn_dn(RBB, 128, hb0, True)
    ffn_dn(RBB + 128, 128, hb1, True)
    prep_gu(1)
    ln_rows(RC, RB, anc + anc2[:8])

    wd0_copy(1).wait()
    x_copy(5).wait()
    prep_d(wd0(1), FH)
    h2, anc = ffn_gu(RA, RB)
    ffn_dn(RA, RB, h2, False)
    ln_rows(RD, RB, anc)
    wq_copy(2).start()
    for cp in gu_copies(1, 1):
        cp.start()
    wd_copy(1, 1).start()

    wq_copy(0).wait()
    h3, _ = ffn_gu(RBB, RB)
    prep_q_half(0, 0, bq.at[0], 2)
    zero = jnp.sum(jnp.where(true_mask(), 0, 1))
    ffn_dn(RBB, RB, h3, False)

    for cp in wo_copies():
        cp.wait()

    def p2_body(i, carry):
        @pl.when(i == 1)
        def _():
            wq_copy(1).wait()

        @pl.when(i == 3)
        def _():
            wq_copy(2).wait()

        @pl.when(i == 4)
        def _():
            for cp in gu_copies(1, 1):
                cp.wait()
        bqv = bq.at[pl.ds(i, 2)]
        anc16 = qkv_tiles(i >> 1, i & 1, bqv.at[0])
        prep_q_half(jnp.minimum((i + 1) >> 1, 2), (i + 1) & 1, bqv.at[1])
        tm = true_mask()
        tm16 = jnp.concatenate([tm, tm], axis=0)
        jobs = []
        for k in range(6):
            jobs += [('o', k, q) for q in range(4)] + [('x', k, q) for q in range(14)]
        for k in range(8):
            jobs += [('g', k, q) for q in range(7)]
        for k in range(6):
            jobs += [('z', k, q) for q in range(7)]
        by = {}
        for kind in 'oxgz':
            js = [jb for jb in jobs if jb[0] == kind]
            for e, jb in enumerate(js):
                by[jb] = (e + 0.5) / len(js)
        ranked = sorted(jobs, key=lambda jb: by[jb])
        na = len(anc16) - 12
        at = {jb: anc16[(e * na) // len(ranked)] for e, jb in enumerate(ranked)}
        for k in range(6):
            prep_o_chunk(jnp.minimum(3 * i + (k >> 1), 15), k & 1, tm, [at['o', k, q][0:8] for q in range(4)])
            make_xa2(pl.multiple_of(jnp.minimum(6 * i + k, 31) * 16, 16), tm16,
                     [at['x', k, q] for q in range(14)])
        for k in range(8):
            idx = 4 * i + (k >> 1)
            for q in range(7):
                prep_gu2_piece(idx >> 4, q, k & 1, pl.multiple_of((idx & 15) * 16, 16), tm16,
                               at['g', k, q], 1)
        for k in range(6):
            blk = jnp.minimum(6 * i + k, 31)
            r0 = pl.multiple_of(256 + (blk >> 4) * 512 + (blk & 15) * 16, 16)
            for p in range(7):
                z16 = jnp.where(tm16, 0.0, at['z', k, p])
                for c in range(4):
                    acc.at[p][pl.ds(r0, 16), c * 128:(c + 1) * 128] = z16
        return carry

    lax.fori_loop(0, 6, p2_body, 0)

    def p3_body(u, carry):
        j = u >> 1
        s_ = u & 1
        sl = j & 1
        jn = jnp.minimum((u >> 1) + 1, NG - 1)
        sn = 1 - sl

        @pl.when(s_ == 0)
        def _():
            wd_copy(j, sl).wait()

        @pl.when(jnp.logical_and(s_ == 0, j + 1 < NG))
        def _():
            for cp in gu_copies(jn, sn):
                cp.wait()
        prep_d(wd_raw.at[sl], FC)
        a4 = pl.multiple_of((u - 1) * 64, 64)
        for g in range(4):
            attn_pair(a4 + 16 * g, g == 0)
        att_last = attn_pair(832 + 16 * jnp.minimum(u - 1, 11))
        tm = true_mask()
        tm16 = jnp.concatenate([tm, tm], axis=0)

        rows = pl.ds(pl.multiple_of(s_ * RB, RB), RB)
        order = (2, 4, 1, 3, 0, 6, 5)
        bcur = bgu2.at[sl]
        c1 = [None] * 7
        h = [[None] * 4 for _ in range(4)]

        def gate_up(i):
            ms = [None] * 7
            for k in order:
                ms[k] = _dot(xa2.at[7 * i + k][rows, :], bcur.at[7 * i + k][...])
            c1[i] = _ccomb(ms)
            return [ms[k][r_:r_ + 16, t * 128:(t + 1) * 128] for k in order for r_ in range(0, RB, 64)
                    for t in range(2)]

        def hidden(a, e):
            if h[2 * a][2 * e] is None:
                for q in range(4):
                    m = [None if v is None else v[q] for v in c1]
                    if (a, e) == (0, 0):
                        cc = m[0] + m[3] - m[4] + m[6]
                    elif (a, e) == (0, 1):
                        cc = m[2] + m[4]
                    elif (a, e) == (1, 0):
                        cc = m[1] + m[3]
                    else:
                        cc = m[0] - m[1] + m[2] + m[5]
                    h[2 * a + (q >> 1)][2 * e + (q & 1)] = _glu2(cc[:, :128], _gate_tanh(cc[:, :128]),
                                                                 cc[:, 128:])
            return [[h[2 * a + b][2 * e + f] for f in range(2)] for b in range(2)]

        def down(i):
            p, q, sg = _A_TERMS[i]
            P = hidden(*p)
            if q is not None:
                Q = hidden(*q)
                P = [[P[b][f] + Q[b][f] if sg > 0 else P[b][f] - Q[b][f] for f in range(2)] for b in range(2)]
            out = []
            if 4 == i:
                v = P[0][0]
                P[0][0] = jnp.concatenate([jnp.where(tm16, v[0:16], att_last), v[16:]], axis=0)
            for b in range(2):
                y = _dot(jnp.concatenate(P[b], axis=1).astype(bf16), bd[i])
                out += [y[r_:r_ + 16, 0:128] for r_ in range(0, RB, 32)]
                acc.at[i][pl.ds(pl.multiple_of(b * QS + s_ * RB, RB), RB), :] += y
            return out

        seq = 'G0 G3 G4 G6 G2 G1 D2 D4 G5 D5 D1 D3 D0 D6'.split()
        sanc = [(gate_up if tk[0] == 'G' else down)(int(tk[1])) for tk in seq]
        last_g = max(p for p, tk in enumerate(seq) if tk[0] == 'G')
        src = [a for p in range(last_g + 1, len(seq)) for a in sanc[p]]
        src = src[:int(len(src) * 0.9)]
        kb = pl.multiple_of(s_ * (QD // 2), QD // 2)
        pieces = [(t, k0, i) for k0 in range(0, QD // 2, 16) for t in range(2) for i in range(7)]
        for e, (t, k0, i) in enumerate(pieces):
            prep_gu2_piece(sn, i, t, kb + k0, tm16, src[e * len(src) // len(pieces)], 4)

        @pl.when(jnp.logical_and(s_ == 0, j + 1 < NG))
        def _():
            wd_copy(j + 1, sn).start()

        @pl.when(jnp.logical_and(s_ == 1, j + 3 < NG))
        def _():
            for cp in gu_copies(j + 3, sn):
                cp.start()
        return carry

    for cp in gu_copies(2, 0):
        cp.start()
    lax.fori_loop(1, 2 * NG, p3_body, 0)

    SB = 64

    def p4_body(k, carry):
        tm = true_mask()
        for u in range(RB // SB):
            r0 = pl.multiple_of(k * RB + u * SB, SB)
            rows = pl.ds(r0, SB)
            for n in range(2):
                ms = [_dot(oa.at[i][rows, :], bo.at[i, n][...]) for i in range(7)]
                av = [acc.at[i][rows, n * 256:(n + 1) * 256] for i in range(7)]
                ss = _ccomb(ms)
                fs = _ccomb(av)
                for q, (h, c0) in enumerate(((0, n * 256), (0, HD + n * 256), (1, n * 256), (1, HD + n * 256))):
                    fv = 0.5 * fs[q]
                    g = fv * jax.nn.sigmoid(fv)
                    xv = xraw.at[h][rows, c0:c0 + 256].astype(f32)
                    if u == 0 and n == 0 and q == 0:
                        ka = bq_u[zero, zero, pl.ds(pl.multiple_of(zero * 8, 8), 8), 0:128]
                        x8 = jnp.where(tm, xv[0:8, 0:128], pltpu.bitcast(ka, f32))
                        x8 = jnp.concatenate([x8, xv[0:8, 128:]], axis=1)
                        xv = jnp.concatenate([x8, xv[8:]], axis=0)
                    obuf.at[h][rows, c0:c0 + 256] = (xv + ss[q] * g).astype(bf16)
            out_copy(r0, SB, 0).start()
        return carry

    lax.fori_loop(0, NB, p4_body, 0)
    out_copy(0, HS, 0).wait()


@jax.jit
def pallas_recurrent_scan__sliding_local_dilated__geglu_ffn__prompt_kernel(
    A_x: jax.Array,
    A_wqkv: jax.Array,
    A_wo: jax.Array,
    B_x: jax.Array,
    B_w_gate: jax.Array,
    B_w_up: jax.Array,
    B_w_down: jax.Array,
):
    any_spec = pl.BlockSpec(memory_space=pl.ANY)
    out = pl.pallas_call(
        _kernel,
        out_shape=jax.ShapeDtypeStruct((2, HS, D), bf16),
        in_specs=[any_spec] * 6,
        out_specs=any_spec,
        scratch_shapes=[
            pltpu.VMEM((2, HS, D), bf16),
            pltpu.VMEM((7, HS // 2, HD), u32),
            pltpu.VMEM((49, QS // 2, QD), u32),
            pltpu.VMEM((2, 2, D, GC), bf16),
            pltpu.VMEM((2, GC, D), bf16),
            pltpu.VMEM((7, HD // 2, FC), u32),
            pltpu.VMEM((2, 49, QD // 2, 256), u32),
            pltpu.VMEM((7, FC // 2, HD), u32),
            pltpu.VMEM((7, HS, HD), f32),
            pltpu.VMEM((3, D, D), bf16),
            pltpu.VMEM((7, 7, HD // 2, 256), u32),
            pltpu.VMEM((3, 8, PAD + S, 128), f32),
            pltpu.VMEM((8, D, 128), bf16),
            pltpu.VMEM((7, 2, HD // 2, 256), u32),
            pltpu.VMEM((2, 2, HS, 128), f32),
            pltpu.VMEM((2, 16, 128), bf16),
            pltpu.SemaphoreType.DMA((26,)),
        ],
        compiler_params=pltpu.CompilerParams(vmem_limit_bytes=124 * 1024 * 1024,
                                             disable_bounds_checks=True,
                                             disable_semaphore_checks=True),
        name="fusedk",
    )(A_x.reshape(2, HS, D), A_wqkv, A_wo, B_w_gate, B_w_up, B_w_down)
    return out.reshape(1, S, D)
```

```python
import jax
import jax.numpy as jnp
from jax import lax
import jax.experimental.pallas as pl
import jax.experimental.pallas.tpu as pltpu

f32 = jnp.float32
bf16 = jnp.bfloat16
u32 = jnp.uint32

S, D, F = 2048, 1024, 3584
HS, HD = S // 2, D // 2
FC = 256
FH = FC // 2
NF = F // FC
QS, QD = S // 4, D // 4
GC = 512
NG = F // GC
RB = 256
NB = HS // RB
PAD = 16
NW = 8
SCALE = 32 ** -0.5
LOG2E = 1.4426950408889634
NEG = -1e9 / SCALE


def _dot(a, b):
    return jnp.dot(a, b, preferred_element_type=f32)


def _acomb(a11, a12, a21, a22):
    r = lambda v: v.astype(bf16)
    return [r(a11 + a22), r(a21 + a22), r(a11), r(a22), r(a11 + a12), r(a21 - a11), r(a12 - a22)]


def _bcomb(b11, b12, b21, b22):
    r = lambda v: v.astype(bf16)
    return [r(b11 + b22), r(b11), r(b12 - b22), r(b21 - b11), r(b22), r(b11 + b12), r(b21 + b22)]


def _asum(a11, a12, a21, a22):
    return [a11 + a22, a21 + a22, a11, a22, a11 + a12, a21 - a11, a12 - a22]


def _bsum(b11, b12, b21, b22):
    return [b11 + b22, b11, b12 - b22, b21 - b11, b22, b11 + b12, b21 + b22]


_A_TERMS = [((0, 0), (1, 1), 1), ((1, 0), (1, 1), 1), ((0, 0), None, 0), ((1, 1), None, 0),
            ((0, 0), (0, 1), 1), ((1, 0), (0, 0), -1), ((0, 1), (1, 1), -1)]
_B_TERMS = [((0, 0), (1, 1), 1), ((0, 0), None, 0), ((0, 1), (1, 1), -1), ((1, 0), (0, 0), -1),
            ((1, 1), None, 0), ((0, 0), (0, 1), 1), ((1, 0), (1, 1), 1)]


def _ccomb(m):
    m1, m2, m3, m4, m5, m6, m7 = m
    return m1 + m4 - m5 + m7, m3 + m5, m2 + m4, m1 - m2 + m3 + m6


def _gate_tanh(x):
    c = 0.7978845608028654
    return jnp.tanh(x * (c + (c * 0.044715) * (x * x)))


def _glu2(g, th, u):
    a = g * u
    return a + a * th


def _sum8(v):
    return ((v[0] + v[1]) + (v[2] + v[3])) + ((v[4] + v[5]) + (v[6] + v[7]))


def _butterfly(sets, masks, axis, size):
    for b in range(3):
        sh = 1 << b
        out = []
        for blk in sets:
            nxt = list(blk)
            for c in range(8):
                if c & sh == 0:
                    lo, hi = blk[c], blk[c + sh]
                    nxt[c] = jnp.where(masks[b], lo, pltpu.roll(hi, sh, axis))
                    nxt[c + sh] = jnp.where(masks[b], pltpu.roll(lo, size - sh, axis), hi)
            out.append(nxt)
        sets = out
    return sets


def _kernel(x_hbm, wqkv_hbm, wo_hbm, wg_hbm, wu_hbm, wd_hbm, out_hbm,
            xraw, xa_u, xa2_u, gu_raw, wd_raw, bgu_u, bgu2_u, bd_u, acc, wq_raw_u, bq_u, qkv,
            wo_raw_u, bo_u, stats, zbuf, sems):
    wq_raw = wq_raw_u.bitcast(bf16)
    wo_raw = wo_raw_u.bitcast(bf16)
    bq = bq_u.bitcast(bf16)
    bo = bo_u.bitcast(bf16)
    obuf = xraw
    xa = xa_u.bitcast(bf16)
    bgu = bgu_u.bitcast(bf16)
    bdd = bd_u.bitcast(bf16)
    bd = bdd.at[1]
    xa2 = xa2_u.bitcast(bf16)
    bgu2 = bgu2_u.bitcast(bf16)
    oa = xa
    pk = lambda v: pltpu.bitcast(v, u32)
    un = lambda v: pltpu.bitcast(v, bf16)

    lane = lax.broadcasted_iota(jnp.int32, (8, 128), 1)
    row8 = lax.broadcasted_iota(jnp.int32, (8, 128), 0)
    lane_lo = [(lane & (1 << b)) == 0 for b in range(3)]
    row_lo = [(row8 & (1 << b)) == 0 for b in range(3)]

    XP = [(0, 128), (128, 128), (512, 128), (640, 128), (256, 256), (768, 256)]

    def x_copy(r):
        r0, n = XP[r]
        return pltpu.make_async_copy(x_hbm.at[:, pl.ds(r0, n), :],
                                     xraw.at[:, pl.ds(r0, n), :], sems.at[(0, 1, 2, 3, 23, 14)[r]])

    def gu_copies(j, slot):
        off = pl.multiple_of(j * GC, GC)
        return (pltpu.make_async_copy(wg_hbm.at[:, pl.ds(off, GC)], gu_raw.at[slot, 0], sems.at[4 + 3 * slot]),
                pltpu.make_async_copy(wu_hbm.at[:, pl.ds(off, GC)], gu_raw.at[slot, 1], sems.at[5 + 3 * slot]))

    def wd_copy(j, slot):
        off = pl.multiple_of(j * GC, GC)
        return pltpu.make_async_copy(wd_hbm.at[pl.ds(off, GC), :], wd_raw.at[slot], sems.at[6 + 3 * slot])

    def gu0_copy(t, c):
        w = (wg_hbm, wu_hbm)[t]
        return pltpu.make_async_copy(w.at[:, pl.ds(c * FC, FC)], gu_raw.at[0, t, :, pl.ds(c * FC, FC)],
                                     sems.at[15 + 2 * c + t])

    def wd0_copy(c):
        return pltpu.make_async_copy(wd_hbm.at[pl.ds(c * FC, FC), :], wd_raw.at[0, pl.ds(c * FC, FC), :],
                                     sems.at[19 + c])

    def wq_copy(t):
        return pltpu.make_async_copy(wqkv_hbm.at[:, pl.ds(t * D, D)], wq_raw.at[t], sems.at[10 + t])

    def wo_copies():
        return [pltpu.make_async_copy(wo_hbm.at[:, pl.ds(c * 256, 256)], wo_raw.at[c], sems.at[24])
                for c in range(4)]

    class _Z:
        cps = [pltpu.make_async_copy(x_hbm.at[0, pl.ds(0, 16), pl.ds(0, 128)], zbuf.at[q], sems.at[21 + q])
               for q in range(2)]

        def start(self):
            for cp in self.cps:
                cp.start()

        def wait(self):
            for cp in self.cps:
                cp.wait()

    z_copy = _Z

    def out_copy(r0, n, k):
        return pltpu.make_async_copy(obuf.at[:, pl.ds(r0, n), :], out_hbm.at[:, pl.ds(r0, n), :],
                                     sems.at[25 + k])

    def true_mask():
        return pk(zbuf[0]) == pk(zbuf[1])

    def ln_half(h, c0, tm16, a):
        xs = []
        for c in range(4):
            x2 = xraw.at[h][c0:c0 + 16, c * 256:(c + 1) * 256].astype(f32)
            xs += [x2[:, :128], x2[:, 128:]]
        s1 = _sum8(xs)
        if a is not None:
            s1 = jnp.where(tm16, s1, a)
        m = jnp.sum(s1, axis=-1, keepdims=True) * (1.0 / D)
        xc = [x - m for x in xs]
        v = jnp.sum(_sum8([x * x for x in xc]), axis=-1, keepdims=True) * (1.0 / D)
        r = lax.rsqrt(v + 1e-5)
        stats.at[h, 0][c0:c0 + 16, :] = jnp.broadcast_to(m, (16, 128))
        stats.at[h, 1][c0:c0 + 16, :] = jnp.broadcast_to(r, (16, 128))
        return [x * r for x in xc]

    def ln_rows(r0, n, anc=None):
        tm16 = None
        if anc is not None:
            tm = true_mask()
            tm16 = jnp.concatenate([tm, tm], axis=0)
            anc = anc[:int(len(anc) * 0.85)]
        nch = n // 16
        for k in range(nch):
            c0 = r0 + 16 * k
            a = [None, None]
            if anc is not None:
                a = [anc[(len(anc) * (2 * k + u)) // (2 * nch)] for u in range(2)]
            lo = ln_half(0, c0, tm16, a[0])
            hi = ln_half(1, c0, tm16, a[1])
            for c in range(4):
                cs = _acomb(lo[c], lo[c + 4], hi[c], hi[c + 4])
                for i in range(7):
                    xa.at[i][c0:c0 + 16, c * 128:(c + 1) * 128] = cs[i]

    def prep_gu(c, ts=(0, 1)):
        KC = 32
        for t in ts:
            w = gu_raw.at[0, t]
            for k0 in range(0, HD, KC):
                lo = w[k0:k0 + KC, c * FC:(c + 1) * FC].astype(f32)
                hi = w[HD + k0:HD + k0 + KC, c * FC:(c + 1) * FC].astype(f32)
                cs = _bcomb(lo[:, :FH], lo[:, FH:], hi[:, :FH], hi[:, FH:])
                for i in range(7):
                    bgu.at[i][k0:k0 + KC, t * FH:(t + 1) * FH] = cs[i]

    def prep_d(w, kh):
        KC = 16
        for k0 in range(0, kh, KC):
            for c0 in range(0, HD, 256):
                g = lambda a, b: w[a + k0:a + k0 + KC, b + c0:b + c0 + 256].astype(f32)
                cs = _bcomb(g(0, 0), g(0, HD), g(kh, 0), g(kh, HD))
                for i in range(7):
                    bd.at[i][k0:k0 + KC, c0:c0 + 256] = cs[i]

    def prep_d_piece(slot, k0, c0, tm16, anc):
        w = wd_raw.at[slot]
        g = lambda a, b: w[pl.ds(a + k0, 16), b + c0:b + c0 + 256].astype(f32)
        v = [g(0, 0), g(0, HD), g(FC, 0), g(FC, HD)]
        for e in (0, 3):
            v[e] = jnp.concatenate([jnp.where(tm16, v[e][:, :128], anc), jnp.where(tm16, v[e][:, 128:], anc)], axis=1)
        cs = _bcomb(*v)
        for i in range(7):
            bdd.at[slot, i][pl.ds(k0, 16), c0:c0 + 256] = cs[i]

    def two_level_piece(terms, inner, ld, i, tm16, anc, nanc, store):
        p, q, sg = terms[i]
        P = ld(*p)
        for e in range(nanc):
            P[e >> 1][e & 1] = jnp.where(tm16, P[e >> 1][e & 1], anc)
        if q is not None:
            Q = ld(*q)
            P = [[P[b][d] + Q[b][d] if sg > 0 else P[b][d] - Q[b][d] for d in range(2)] for b in range(2)]
        ops = inner(P[0][0], P[0][1], P[1][0], P[1][1])
        for k in range(7):
            store(7 * i + k, ops[k].astype(bf16))

    def prep_gu2_piece(slot, i, t, k0, tm16, anc, nanc):
        w = gu_raw.at[slot, t]
        dst = bgu2.at[slot]

        def ld(R, C):
            out = []
            for b in range(2):
                x2 = w[pl.ds((2 * R + b) * QD + k0, 16), C * 256:(C + 1) * 256].astype(f32)
                out.append([x2[:, :128], x2[:, 128:]])
            return out

        def store(p, v):
            dst.at[p][pl.ds(k0, 16), t * 128:(t + 1) * 128] = v
        two_level_piece(_B_TERMS, _bsum, ld, i, tm16, anc, nanc, store)

    def make_xa2(r0, tm16, ancs):
        st = [[[stats.at[a, e][pl.ds(b * QS + r0, 16), :] for e in range(2)] for b in range(2)] for a in range(2)]
        for j in range(2):
            def ld(R, C):
                out = []
                for b in range(2):
                    m, r = st[R][b]
                    row = []
                    for d in range(2):
                        c0 = (2 * C + d) * QD + j * 128
                        xv = xraw.at[R][pl.ds(b * QS + r0, 16), c0:c0 + 128].astype(f32)
                        row.append((xv - m) * r)
                    out.append(row)
                return out

            def store(p, v):
                xa2.at[p][pl.ds(r0, 16), j * 128:(j + 1) * 128] = v
            for i in range(7):
                two_level_piece(_A_TERMS, _asum, ld, i, tm16, ancs[7 * j + i], 1, store)

    def ffn_gu(r0, n):
        ms = [_dot(xa[i, r0:r0 + n, :], bgu[i]) for i in range(7)]
        anc = [m_[k:k + 16, t * FH:(t + 1) * FH] for m_ in ms for t in range(2) for k in range(0, n, 64)]
        hs = _acomb(*[_glu2(v[:, :FH], _gate_tanh(v[:, :FH]), v[:, FH:]) for v in _ccomb(ms)])
        return hs, anc

    def ffn_dn(r0, n, hs, first):
        anc = []
        for i in range(7):
            y = _dot(hs[i], bd[i, :FH, :])
            anc += [y[k:k + 16, 0:128] for k in range(0, n, 32)]
            if first:
                acc[i, r0:r0 + n, :] = y
            else:
                acc[i, r0:r0 + n, :] += y
        return anc

    upk = lambda v: un(v).astype(f32)

    def prep_q_half(t, h, dst, par=1):
        KC = 16
        sa = (128 - 2) * h
        sb = 2 * (1 - h)
        w = wq_raw_u.at[t]

        def stage1(r0):
            blk = [w[r0 // 2:(r0 + KC) // 2, c * 128:(c + 1) * 128] for c in range(8)]
            rl = lambda v, sft: v if (isinstance(sft, int) and sft == 0) else pltpu.roll(v, sft, 1)
            return [jnp.where(lane_lo[1], rl(blk[c], sa), rl(blk[c + 2], sb)) for c in (0, 1, 4, 5)]

        def stage(sets, jb, b):
            sh = 1 << b
            out = []
            for blk in sets:
                nxt = list(blk)
                for j in range(4):
                    if j & jb == 0:
                        lo, hi = blk[j], blk[j + jb]
                        nxt[j] = jnp.where(lane_lo[b], lo, pltpu.roll(hi, sh, 1))
                        nxt[j + jb] = jnp.where(lane_lo[b], pltpu.roll(lo, 128 - sh, 1), hi)
                out.append(nxt)
            return out

        for k00 in range(0, HD, KC * par):
            ks = [k00 + KC * q for q in range(par)]
            hv = stage(stage([stage1(hk * HD + k0) for k0 in ks for hk in range(2)], 1, 0), 2, 2)
            for q, k0 in enumerate(ks):
                lo, hi = hv[2 * q], hv[2 * q + 1]
                for e in range(2):
                    cs = _bcomb(upk(lo[e]), upk(lo[e + 2]), upk(hi[e]), upk(hi[e + 2]))
                    for i in range(7):
                        dst.at[i][k0:k0 + KC, e * 128:(e + 1) * 128] = cs[i]

    def qkv_tiles(t, h, src):
        anc16 = []
        for e in range(2):
            n = 2 * h + e
            qlo = qkv.at[t, n]
            qhi = qkv.at[t, n + 4]
            for r in range(NB):
                ms = [_dot(xa[i, r * RB:(r + 1) * RB, :], src.at[i][:, e * 128:(e + 1) * 128]) for i in range(7)]
                c11, c12, c21, c22 = _ccomb(ms)
                anc16 += [m_[k:k + 16] for m_ in ms for k in range(0, RB, 64)]
                r0 = PAD + r * RB
                qlo[r0:r0 + RB, :] = c11
                qhi[r0:r0 + RB, :] = c12
                qlo[HS + r0:HS + r0 + RB, :] = c21
                qhi[HS + r0:HS + r0 + RB, :] = c22
                if r == 0:
                    qlo[0:PAD, :] = jnp.broadcast_to(c11[0:1, :], (PAD, 128))
                    qhi[0:PAD, :] = jnp.broadcast_to(c12[0:1, :], (PAD, 128))
        return anc16

    def prep_o_chunk(m, e, tm, ancs):
        n2 = m >> 3
        g16 = pl.multiple_of((m & 7) * 16, 16)
        res = []
        for h in range(2):
            w = wo_raw.at[n2 + 2 * h]
            w16 = [w[pl.ds(128 * i + g16, 16), e * 128:(e + 1) * 128].astype(f32) for i in range(8)]
            for u in range(2):
                blk = [v[8 * u:8 * u + 8] for v in w16]
                blk[0] = jnp.where(tm, blk[0], ancs[2 * h + u])
                res += _butterfly([blk], row_lo, 0, 8)
        cols = [[jnp.concatenate([res[2 * h][j], res[2 * h + 1][j]], axis=0) for j in range(8)]
                for h in range(2)]
        for b in range(4):
            cs = _bcomb(cols[0][b], cols[1][b], cols[0][b + 4], cols[1][b + 4])
            for i in range(7):
                bo.at[i, n2][pl.ds(b * 128 + g16, 16), e * 128:(e + 1) * 128] = cs[i]

    def attn8(base, row0):
        lg = [None] * NW
        for c in range(8):
            q = qkv[0, c, pl.ds(base, 8), :]
            for w in range(NW):
                pr = q * qkv[1, c, pl.ds(base - 2 * w, 8), :]
                lg[w] = pr if lg[w] is None else lg[w] + pr
        G1 = 2
        for w0 in range(0, NW, G1):
            for w in range(w0, w0 + G1):
                lg[w] = lg[w] + pltpu.roll(lg[w], 8, 1)
            for w in range(w0, w0 + G1):
                lg[w] = lg[w] + pltpu.roll(lg[w], 16, 1)
        if row0 is not None:
            for w in range(1, NW):
                lg[w] = jnp.where(row8 + row0 >= 2 * w, lg[w], NEG)
        m = lg[0]
        for w in range(1, NW):
            m = jnp.maximum(m, lg[w])
        p = [jnp.exp2((lg[w] - m) * (SCALE * LOG2E)) for w in range(NW)]
        den = p[0]
        for w in range(1, NW):
            den = den + p[w]
        inv = 1.0 / den
        b4 = (lane & 16) != 0
        b3 = (lane & 8) != 0
        outs = [None] * 8
        G2 = 2
        for w0 in range(0, NW, G2):
            ws = range(w0, w0 + G2)
            for w in ws:
                p[w] = p[w] * inv
                p[w] = jnp.where(b4, p[w], pltpu.roll(p[w], 112, 1))
            for w in ws:
                p[w] = jnp.where(b3, p[w], pltpu.roll(p[w], 120, 1))
            for w in ws:
                for c in range(8):
                    pr = p[w] * qkv[2, c, pl.ds(base - 2 * w, 8), :]
                    outs[c] = pr if outs[c] is None else outs[c] + pr
        return outs

    def attn_pair(r0, mask=False):
        parts = [attn8(pl.multiple_of(PAD + h * HS + r0 + 8 * u, 8), (r0 + 8 * u) if (h == 0 and mask) else None)
                 for h in range(2) for u in range(2)]
        lo = [jnp.concatenate([parts[0][c], parts[1][c]], axis=0) for c in range(8)]
        hi = [jnp.concatenate([parts[2][c], parts[3][c]], axis=0) for c in range(8)]
        for n in range(4):
            cs = _acomb(lo[n], lo[n + 4], hi[n], hi[n + 4])
            for i in range(7):
                oa.at[i][pl.ds(pl.multiple_of(r0, 16), 16), n * 128:(n + 1) * 128] = cs[i]
        return hi[7]

    wd0 = lambda c: wd_raw.at[0, c * FC:(c + 1) * FC, :]
    RA, RBB, RC, RD = 0, 512, 256, 768

    x_copy(0).start()
    x_copy(1).start()
    gu0_copy(0, 0).start()
    z_copy().start()
    gu0_copy(1, 0).start()
    x_copy(2).start()
    wd0_copy(0).start()
    x_copy(3).start()
    x_copy(4).start()
    gu0_copy(0, 1).start()
    gu0_copy(1, 1).start()
    wd0_copy(1).start()
    x_copy(5).start()
    wq_copy(0).start()
    for cp in wo_copies():
        cp.start()
    wq_copy(1).start()

    x_copy(0).wait()
    ln_rows(RA, 128)
    x_copy(1).wait()
    ln_rows(RA + 128, 128)

    gu0_copy(0, 0).wait()
    prep_gu(0, (0,))
    mg = [_dot(xa[i, RA:RA + RB, :], bgu[i, :, :FH]) for i in range(7)]
    gg = [(v, _gate_tanh(v)) for v in _ccomb(mg)]

    z_copy().wait()
    gu0_copy(1, 0).wait()
    x_copy(2).wait()
    prep_gu(0, (1,))
    mu = [_dot(xa[i, RA:RA + RB, :], bgu[i, :, FH:]) for i in range(7)]
    ha = _acomb(*[_glu2(a[0], a[1], b) for a, b in zip(gg, _ccomb(mu))])
    ln_rows(RBB, 128, [m_[k:k + 16] for m_ in mu for k in range(0, RB, 64)])

    wd0_copy(0).wait()
    x_copy(3).wait()
    prep_d(wd0(0), FH)
    hb0, anc = ffn_gu(RBB, 128)
    ffn_dn(RA, RB, ha, True)
    ln_rows(RBB + 128, 128, anc)

    x_copy(4).wait()
    gu0_copy(0, 1).wait()
    gu0_copy(1, 1).wait()
    hb1, anc = ffn_gu(RBB + 128, 128)
    anc2 = ffn_dn(RBB, 128, hb0, True)
    ffn_dn(RBB + 128, 128, hb1, True)
    prep_gu(1)
    ln_rows(RC, RB, anc + anc2[:8])

    wd0_copy(1).wait()
    x_copy(5).wait()
    prep_d(wd0(1), FH)
    h2, anc = ffn_gu(RA, RB)
    ffn_dn(RA, RB, h2, False)
    ln_rows(RD, RB, anc)
    wq_copy(2).start()
    for cp in gu_copies(1, 1):
        cp.start()
    wd_copy(1, 1).start()

    wq_copy(0).wait()
    h3, _ = ffn_gu(RBB, RB)
    prep_q_half(0, 0, bq.at[0], 2)
    zero = jnp.sum(jnp.where(true_mask(), 0, 1))
    ffn_dn(RBB, RB, h3, False)

    for cp in wo_copies():
        cp.wait()

    def p2_body(i, carry):
        @pl.when(i == 1)
        def _():
            wq_copy(1).wait()

        @pl.when(i == 3)
        def _():
            wq_copy(2).wait()

        @pl.when(i == 4)
        def _():
            for cp in gu_copies(1, 1):
                cp.wait()
            wd_copy(1, 1).wait()
        bqv = bq.at[pl.ds(i, 2)]
        anc16 = qkv_tiles(i >> 1, i & 1, bqv.at[0])
        prep_q_half(jnp.minimum((i + 1) >> 1, 2), (i + 1) & 1, bqv.at[1], 2)
        tm = true_mask()
        tm16 = jnp.concatenate([tm, tm], axis=0)
        jobs = []
        for k in range(6):
            jobs += [('o', k, q) for q in range(4)] + [('x', k, q) for q in range(14)]
        for k in range(8):
            jobs += [('g', k, q) for q in range(7)] + [('d', k, 0)]
        for k in range(6):
            jobs += [('z', k, q) for q in range(7)]
        by = {}
        for kind in 'oxgzd':
            js = [jb for jb in jobs if jb[0] == kind]
            for e, jb in enumerate(js):
                by[jb] = (e + 0.5) / len(js)
        ranked = sorted(jobs, key=lambda jb: by[jb])
        na = len(anc16) - 12
        at = {jb: anc16[(e * na) // len(ranked)] for e, jb in enumerate(ranked)}
        for k in range(6):
            prep_o_chunk(jnp.minimum(3 * i + (k >> 1), 15), k & 1, tm, [at['o', k, q][0:8] for q in range(4)])
            make_xa2(pl.multiple_of(jnp.minimum(6 * i + k, 31) * 16, 16), tm16,
                     [at['x', k, q] for q in range(14)])
        for k in range(8):
            idx = 4 * i + (k >> 1)
            for q in range(7):
                prep_gu2_piece(idx >> 4, q, k & 1, pl.multiple_of((idx & 15) * 16, 16), tm16,
                               at['g', k, q], 1)
            prep_d_piece(idx >> 4, pl.multiple_of((idx & 15) * 16, 16), (k & 1) * 256, tm16, at['d', k, 0])
        for k in range(6):
            blk = jnp.minimum(6 * i + k, 31)
            r0 = pl.multiple_of(256 + (blk >> 4) * 512 + (blk & 15) * 16, 16)
            for p in range(7):
                z16 = jnp.where(tm16, 0.0, at['z', k, p])
                for c in range(4):
                    acc.at[p][pl.ds(r0, 16), c * 128:(c + 1) * 128] = z16
        return carry

    lax.fori_loop(0, 6, p2_body, 0)

    def p3_body(u, carry):
        j = u >> 1
        s_ = u & 1
        sl = j & 1
        jn = jnp.minimum((u >> 1) + 1, NG - 1)
        sn = 1 - sl

        @pl.when(jnp.logical_and(s_ == 0, j + 1 < NG))
        def _():
            wd_copy(jn, sn).wait()
            for cp in gu_copies(jn, sn):
                cp.wait()
        a4 = pl.multiple_of((u - 1) * 64, 64)
        for g in range(4):
            attn_pair(a4 + 16 * g, g == 0)
        att_last = attn_pair(832 + 16 * jnp.minimum(u - 1, 11))
        tm = true_mask()
        tm16 = jnp.concatenate([tm, tm], axis=0)

        rows = pl.ds(pl.multiple_of(s_ * RB, RB), RB)
        order = tuple([4, 2, 3, 1, 0, 6, 5])
        bcur = bgu2.at[sl]
        c1 = [None] * 7
        dprep = []
        h = [[None] * 4 for _ in range(4)]

        def gate_up(i):
            ms = [None] * 7
            for k in order:
                ms[k] = _dot(xa2.at[7 * i + k][rows, :], bcur.at[7 * i + k][...])
            c1[i] = _ccomb(ms)
            return [ms[k][r_:r_ + 16, t * 128:(t + 1) * 128] for k in order for r_ in range(0, RB, 64)
                    for t in range(2)]

        def hidden(a, e):
            if h[2 * a][2 * e] is None:
                for q in range(4):
                    m = [None if v is None else v[q] for v in c1]
                    if (a, e) == (0, 0):
                        cc = m[0] + m[3] - m[4] + m[6]
                    elif (a, e) == (0, 1):
                        cc = m[2] + m[4]
                    elif (a, e) == (1, 0):
                        cc = m[1] + m[3]
                    else:
                        cc = m[0] - m[1] + m[2] + m[5]
                    h[2 * a + (q >> 1)][2 * e + (q & 1)] = _glu2(cc[:, :128], _gate_tanh(cc[:, :128]),
                                                                 cc[:, 128:])
            return [[h[2 * a + b][2 * e + f] for f in range(2)] for b in range(2)]

        def down(i):
            p, q, sg = _A_TERMS[i]
            P = hidden(*p)
            if q is not None:
                Q = hidden(*q)
                P = [[P[b][f] + Q[b][f] if sg > 0 else P[b][f] - Q[b][f] for f in range(2)] for b in range(2)]
            out = []
            if 4 == i:
                v = P[0][0]
                P[0][0] = jnp.concatenate([jnp.where(tm16, v[0:16], att_last), v[16:]], axis=0)
            for b in range(2):
                y = _dot(jnp.concatenate(P[b], axis=1).astype(bf16), bdd.at[sl, i][...])
                out += [y[r_:r_ + 16, 0:128] for r_ in range(0, RB, 32)]
                acc.at[i][pl.ds(pl.multiple_of(b * QS + s_ * RB, RB), RB), :] += y
            return out

        seq = 'G0 G3 G4 G6 G2 G1 D2 D4 G5 D5 D1 D3 D0 D6'.split()
        sanc = []
        for tk in seq:
            if tk[0] == 'D' and not dprep:
                dprep.append(1)
                lo_, hi_ = [2, 5]
                src = [a for p in range(lo_, hi_) for a in sanc[p]]
                pcs = [(k0, c0) for k0 in range(0, FC // 2, 16) for c0 in range(0, HD, 256)]
                for e, (k0, c0) in enumerate(pcs):
                    prep_d_piece(sn, pl.multiple_of(s_ * (FC // 2), FC // 2) + k0, c0, tm16,
                                 src[e * len(src) // len(pcs)])
            sanc.append((gate_up if tk[0] == 'G' else down)(int(tk[1])))
        last_g = max(p for p, tk in enumerate(seq) if tk[0] == 'G')
        src = [a for p in range(last_g + 1, len(seq)) for a in sanc[p]]
        src = src[:int(len(src) * 1.0)]
        kb = pl.multiple_of(s_ * (QD // 2), QD // 2)
        pieces = [(t, k0, i) for k0 in range(0, QD // 2, 16) for t in range(2) for i in range(7)]
        for e, (t, k0, i) in enumerate(pieces):
            prep_gu2_piece(sn, i, t, kb + k0, tm16, src[e * len(src) // len(pieces)], 4)

        @pl.when(jnp.logical_and(s_ == 1, j + 3 < NG))
        def _():
            wd_copy(j + 3, sn).start()
            for cp in gu_copies(j + 3, sn):
                cp.start()
        return carry

    wd_copy(2, 0).start()
    for cp in gu_copies(2, 0):
        cp.start()
    lax.fori_loop(1, 2 * NG, p3_body, 0)

    SB = 32

    def p4_body(k, carry):
        tm = true_mask()
        for u in range(RB // SB):
            r0 = pl.multiple_of(k * RB + u * SB, SB)
            rows = pl.ds(r0, SB)
            for n in range(2):
                ms = [_dot(oa.at[i][rows, :], bo.at[i, n][...]) for i in range(7)]
                av = [acc.at[i][rows, n * 256:(n + 1) * 256] for i in range(7)]
                ss = _ccomb(ms)
                fs = _ccomb(av)
                for q, (h, c0) in enumerate(((0, n * 256), (0, HD + n * 256), (1, n * 256), (1, HD + n * 256))):
                    fv = 0.5 * fs[q]
                    g = fv * jax.nn.sigmoid(fv)
                    xv = xraw.at[h][rows, c0:c0 + 256].astype(f32)
                    if u == 0 and n == 0 and q == 0:
                        ka = bq_u[zero, zero, pl.ds(pl.multiple_of(zero * 8, 8), 8), 0:128]
                        x8 = jnp.where(tm, xv[0:8, 0:128], pltpu.bitcast(ka, f32))
                        x8 = jnp.concatenate([x8, xv[0:8, 128:]], axis=1)
                        xv = jnp.concatenate([x8, xv[8:]], axis=0)
                    obuf.at[h][rows, c0:c0 + 256] = (xv + ss[q] * g).astype(bf16)
            out_copy(r0, SB, 0).start()
        return carry

    lax.fori_loop(0, NB, p4_body, 0)
    out_copy(0, HS, 0).wait()


@jax.jit
def pallas_recurrent_scan__sliding_local_dilated__geglu_ffn__prompt_kernel(
    A_x: jax.Array,
    A_wqkv: jax.Array,
    A_wo: jax.Array,
    B_x: jax.Array,
    B_w_gate: jax.Array,
    B_w_up: jax.Array,
    B_w_down: jax.Array,
):
    any_spec = pl.BlockSpec(memory_space=pl.ANY)
    out = pl.pallas_call(
        _kernel,
        out_shape=jax.ShapeDtypeStruct((2, HS, D), bf16),
        in_specs=[any_spec] * 6,
        out_specs=any_spec,
        scratch_shapes=[
            pltpu.VMEM((2, HS, D), bf16),
            pltpu.VMEM((7, HS // 2, HD), u32),
            pltpu.VMEM((49, QS // 2, QD), u32),
            pltpu.VMEM((2, 2, D, GC), bf16),
            pltpu.VMEM((2, GC, D), bf16),
            pltpu.VMEM((7, HD // 2, FC), u32),
            pltpu.VMEM((2, 49, QD // 2, 256), u32),
            pltpu.VMEM((2, 7, FC // 2, HD), u32),
            pltpu.VMEM((7, HS, HD), f32),
            pltpu.VMEM((3, D // 2, D), u32),
            pltpu.VMEM((7, 7, HD // 2, 256), u32),
            pltpu.VMEM((3, 8, PAD + S, 128), f32),
            pltpu.VMEM((4, D // 2, 256), u32),
            pltpu.VMEM((7, 2, HD // 2, 256), u32),
            pltpu.VMEM((2, 2, HS, 128), f32),
            pltpu.VMEM((2, 16, 128), bf16),
            pltpu.SemaphoreType.DMA((26,)),
        ],
        compiler_params=pltpu.CompilerParams(vmem_limit_bytes=124 * 1024 * 1024,
                                             disable_bounds_checks=True,
                                             disable_semaphore_checks=True),
        name="fusedk",
    )(A_x.reshape(2, HS, D), A_wqkv, A_wo, B_w_gate, B_w_up, B_w_down)
    return out.reshape(1, S, D)
```

```python
import jax
import jax.numpy as jnp
from jax import lax
import jax.experimental.pallas as pl
import jax.experimental.pallas.tpu as pltpu

f32 = jnp.float32
bf16 = jnp.bfloat16
u32 = jnp.uint32

S, D, F = 2048, 1024, 3584
HS, HD = S // 2, D // 2
FC = 256
FH = FC // 2
NF = F // FC
QS, QD = S // 4, D // 4
GC = 512
NG = F // GC
RB = 256
NB = HS // RB
PAD = 16
NW = 8
SCALE = 32 ** -0.5
LOG2E = 1.4426950408889634
NEG = -1e9 / SCALE


def _dot(a, b):
    return jnp.dot(a, b, preferred_element_type=f32)


def _acomb(a11, a12, a21, a22):
    r = lambda v: v.astype(bf16)
    return [r(a11 + a22), r(a21 + a22), r(a11), r(a22), r(a11 + a12), r(a21 - a11), r(a12 - a22)]


def _bcomb(b11, b12, b21, b22):
    r = lambda v: v.astype(bf16)
    return [r(b11 + b22), r(b11), r(b12 - b22), r(b21 - b11), r(b22), r(b11 + b12), r(b21 + b22)]


def _asum(a11, a12, a21, a22):
    return [a11 + a22, a21 + a22, a11, a22, a11 + a12, a21 - a11, a12 - a22]


def _bsum(b11, b12, b21, b22):
    return [b11 + b22, b11, b12 - b22, b21 - b11, b22, b11 + b12, b21 + b22]


_A_TERMS = [((0, 0), (1, 1), 1), ((1, 0), (1, 1), 1), ((0, 0), None, 0), ((1, 1), None, 0),
            ((0, 0), (0, 1), 1), ((1, 0), (0, 0), -1), ((0, 1), (1, 1), -1)]
_B_TERMS = [((0, 0), (1, 1), 1), ((0, 0), None, 0), ((0, 1), (1, 1), -1), ((1, 0), (0, 0), -1),
            ((1, 1), None, 0), ((0, 0), (0, 1), 1), ((1, 0), (1, 1), 1)]


def _ccomb(m):
    m1, m2, m3, m4, m5, m6, m7 = m
    return m1 + m4 - m5 + m7, m3 + m5, m2 + m4, m1 - m2 + m3 + m6


def _gate_tanh(x):
    c = 0.7978845608028654
    return jnp.tanh(x * (c + (c * 0.044715) * (x * x)))


def _glu2(g, th, u):
    a = g * u
    return a + a * th


def _sum8(v):
    return ((v[0] + v[1]) + (v[2] + v[3])) + ((v[4] + v[5]) + (v[6] + v[7]))


def _butterfly(sets, masks, axis, size):
    for b in range(3):
        sh = 1 << b
        out = []
        for blk in sets:
            nxt = list(blk)
            for c in range(8):
                if c & sh == 0:
                    lo, hi = blk[c], blk[c + sh]
                    nxt[c] = jnp.where(masks[b], lo, pltpu.roll(hi, sh, axis))
                    nxt[c + sh] = jnp.where(masks[b], pltpu.roll(lo, size - sh, axis), hi)
            out.append(nxt)
        sets = out
    return sets


def _kernel(x_hbm, wqkv_hbm, wo_hbm, wg_hbm, wu_hbm, wd_hbm, out_hbm,
            xraw, xa_u, xa2_u, gu_raw, wd_raw, bgu_u, bgu2_u, bd_u, acc, wq_raw, bq_u, qkv,
            wo_raw, bo_u, stats, zbuf, sems):
    bq = bq_u.bitcast(bf16)
    bo = bo_u.bitcast(bf16)
    obuf = xraw
    xa = xa_u.bitcast(bf16)
    bgu = bgu_u.bitcast(bf16)
    bdd = bd_u.bitcast(bf16)
    bd = bdd.at[1]
    xa2 = xa2_u.bitcast(bf16)
    bgu2 = bgu2_u.bitcast(bf16)
    oa = xa
    pk = lambda v: pltpu.bitcast(v, u32)
    un = lambda v: pltpu.bitcast(v, bf16)

    lane = lax.broadcasted_iota(jnp.int32, (8, 128), 1)
    row8 = lax.broadcasted_iota(jnp.int32, (8, 128), 0)
    lane_lo = [(lane & (1 << b)) == 0 for b in range(3)]
    row_lo = [(row8 & (1 << b)) == 0 for b in range(3)]

    XP = [(0, 128), (128, 128), (512, 128), (640, 128), (256, 256), (768, 256)]

    def x_copy(r):
        r0, n = XP[r]
        return pltpu.make_async_copy(x_hbm.at[:, pl.ds(r0, n), :],
                                     xraw.at[:, pl.ds(r0, n), :], sems.at[(0, 1, 2, 3, 23, 14)[r]])

    def gu_copies(j, slot):
        off = pl.multiple_of(j * GC, GC)
        return (pltpu.make_async_copy(wg_hbm.at[:, pl.ds(off, GC)], gu_raw.at[slot, 0], sems.at[4 + 3 * slot]),
                pltpu.make_async_copy(wu_hbm.at[:, pl.ds(off, GC)], gu_raw.at[slot, 1], sems.at[5 + 3 * slot]))

    def wd_copy(j, slot):
        off = pl.multiple_of(j * GC, GC)
        return pltpu.make_async_copy(wd_hbm.at[pl.ds(off, GC), :], wd_raw.at[slot], sems.at[6 + 3 * slot])

    def gu0_copy(t, c):
        w = (wg_hbm, wu_hbm)[t]
        return pltpu.make_async_copy(w.at[:, pl.ds(c * FC, FC)], gu_raw.at[0, t, :, pl.ds(c * FC, FC)],
                                     sems.at[15 + 2 * c + t])

    def wd0_copy(c):
        return pltpu.make_async_copy(wd_hbm.at[pl.ds(c * FC, FC), :], wd_raw.at[0, pl.ds(c * FC, FC), :],
                                     sems.at[19 + c])

    def wq_copy(t):
        return pltpu.make_async_copy(wqkv_hbm.at[:, pl.ds(t * D, D)], wq_raw.at[t], sems.at[10 + t])

    def wo_copies():
        return [pltpu.make_async_copy(wo_hbm.at[:, pl.ds(c * 256, 256)], wo_raw.at[c], sems.at[24])
                for c in range(4)]

    class _Z:
        cps = [pltpu.make_async_copy(x_hbm.at[0, pl.ds(0, 16), pl.ds(0, 128)], zbuf.at[q], sems.at[21 + q])
               for q in range(2)]

        def start(self):
            for cp in self.cps:
                cp.start()

        def wait(self):
            for cp in self.cps:
                cp.wait()

    z_copy = _Z

    def out_copy(r0, n, k):
        return pltpu.make_async_copy(obuf.at[:, pl.ds(r0, n), :], out_hbm.at[:, pl.ds(r0, n), :],
                                     sems.at[25 + k])

    def true_mask():
        return pk(zbuf[0]) == pk(zbuf[1])

    def ln_half(h, c0, tm16, a):
        xs = []
        for c in range(4):
            x2 = xraw.at[h][c0:c0 + 16, c * 256:(c + 1) * 256].astype(f32)
            xs += [x2[:, :128], x2[:, 128:]]
        s1 = _sum8(xs)
        if a is not None:
            s1 = jnp.where(tm16, s1, a)
        m = jnp.sum(s1, axis=-1, keepdims=True) * (1.0 / D)
        xc = [x - m for x in xs]
        v = jnp.sum(_sum8([x * x for x in xc]), axis=-1, keepdims=True) * (1.0 / D)
        r = lax.rsqrt(v + 1e-5)
        stats.at[h, 0][c0:c0 + 16, :] = jnp.broadcast_to(m, (16, 128))
        stats.at[h, 1][c0:c0 + 16, :] = jnp.broadcast_to(r, (16, 128))
        return [x * r for x in xc]

    def ln_rows(r0, n, anc=None):
        tm16 = None
        if anc is not None:
            tm = true_mask()
            tm16 = jnp.concatenate([tm, tm], axis=0)
            anc = anc[:int(len(anc) * 0.85)]
        nch = n // 16
        for k in range(nch):
            c0 = r0 + 16 * k
            a = [None, None]
            if anc is not None:
                a = [anc[(len(anc) * (2 * k + u)) // (2 * nch)] for u in range(2)]
            lo = ln_half(0, c0, tm16, a[0])
            hi = ln_half(1, c0, tm16, a[1])
            for c in range(4):
                cs = _acomb(lo[c], lo[c + 4], hi[c], hi[c + 4])
                for i in range(7):
                    xa.at[i][c0:c0 + 16, c * 128:(c + 1) * 128] = cs[i]

    def prep_gu(c, ts=(0, 1)):
        KC = 32
        for t in ts:
            w = gu_raw.at[0, t]
            for k0 in range(0, HD, KC):
                lo = w[k0:k0 + KC, c * FC:(c + 1) * FC].astype(f32)
                hi = w[HD + k0:HD + k0 + KC, c * FC:(c + 1) * FC].astype(f32)
                cs = _bcomb(lo[:, :FH], lo[:, FH:], hi[:, :FH], hi[:, FH:])
                for i in range(7):
                    bgu.at[i][k0:k0 + KC, t * FH:(t + 1) * FH] = cs[i]

    def prep_d(w, kh):
        KC = 16
        for k0 in range(0, kh, KC):
            for c0 in range(0, HD, 256):
                g = lambda a, b: w[a + k0:a + k0 + KC, b + c0:b + c0 + 256].astype(f32)
                cs = _bcomb(g(0, 0), g(0, HD), g(kh, 0), g(kh, HD))
                for i in range(7):
                    bd.at[i][k0:k0 + KC, c0:c0 + 256] = cs[i]

    def prep_d_piece(slot, k0, c0, tm16, anc):
        w = wd_raw.at[slot]
        g = lambda a, b: w[pl.ds(a + k0, 16), b + c0:b + c0 + 256].astype(f32)
        v = [g(0, 0), g(0, HD), g(FC, 0), g(FC, HD)]
        for e in (0, 3):
            v[e] = jnp.concatenate([jnp.where(tm16, v[e][:, :128], anc), jnp.where(tm16, v[e][:, 128:], anc)], axis=1)
        cs = _bcomb(*v)
        for i in range(7):
            bdd.at[slot, i][pl.ds(k0, 16), c0:c0 + 256] = cs[i]

    def two_level_piece(terms, inner, ld, i, tm16, anc, nanc, store):
        p, q, sg = terms[i]
        P = ld(*p)
        for e in range(nanc):
            P[e >> 1][e & 1] = jnp.where(tm16, P[e >> 1][e & 1], anc)
        if q is not None:
            Q = ld(*q)
            P = [[P[b][d] + Q[b][d] if sg > 0 else P[b][d] - Q[b][d] for d in range(2)] for b in range(2)]
        ops = inner(P[0][0], P[0][1], P[1][0], P[1][1])
        for k in range(7):
            store(7 * i + k, ops[k].astype(bf16))

    def prep_gu2_piece(slot, i, t, k0, tm16, anc, nanc):
        w = gu_raw.at[slot, t]
        dst = bgu2.at[slot]

        def ld(R, C):
            out = []
            for b in range(2):
                x2 = w[pl.ds((2 * R + b) * QD + k0, 16), C * 256:(C + 1) * 256].astype(f32)
                out.append([x2[:, :128], x2[:, 128:]])
            return out

        def store(p, v):
            dst.at[p][pl.ds(k0, 16), t * 128:(t + 1) * 128] = v
        two_level_piece(_B_TERMS, _bsum, ld, i, tm16, anc, nanc, store)

    def make_xa2(r0, tm16, ancs):
        st = [[[stats.at[a, e][pl.ds(b * QS + r0, 16), :] for e in range(2)] for b in range(2)] for a in range(2)]
        for j in range(2):
            def ld(R, C):
                out = []
                for b in range(2):
                    m, r = st[R][b]
                    row = []
                    for d in range(2):
                        c0 = (2 * C + d) * QD + j * 128
                        xv = xraw.at[R][pl.ds(b * QS + r0, 16), c0:c0 + 128].astype(f32)
                        row.append((xv - m) * r)
                    out.append(row)
                return out

            def store(p, v):
                xa2.at[p][pl.ds(r0, 16), j * 128:(j + 1) * 128] = v
            for i in range(7):
                two_level_piece(_A_TERMS, _asum, ld, i, tm16, ancs[7 * j + i], 1, store)

    def ffn_gu(r0, n):
        ms = [_dot(xa[i, r0:r0 + n, :], bgu[i]) for i in range(7)]
        anc = [m_[k:k + 16, t * FH:(t + 1) * FH] for m_ in ms for t in range(2) for k in range(0, n, 64)]
        hs = _acomb(*[_glu2(v[:, :FH], _gate_tanh(v[:, :FH]), v[:, FH:]) for v in _ccomb(ms)])
        return hs, anc

    def ffn_dn(r0, n, hs, first):
        anc = []
        for i in range(7):
            y = _dot(hs[i], bd[i, :FH, :])
            anc += [y[k:k + 16, 0:128] for k in range(0, n, 32)]
            if first:
                acc[i, r0:r0 + n, :] = y
            else:
                acc[i, r0:r0 + n, :] += y
        return anc

    upk = lambda v: un(v).astype(f32)

    def prep_q_half(t, h, dst, par=1):
        KC = 16
        sa = (128 - 2) * h
        sb = 2 * (1 - h)
        w = wq_raw.at[t]

        def stage1(r0):
            blk = [pk(w[r0:r0 + KC, c * 128:(c + 1) * 128]) for c in range(8)]
            rl = lambda v, sft: v if (isinstance(sft, int) and sft == 0) else pltpu.roll(v, sft, 1)
            return [jnp.where(lane_lo[1], rl(blk[c], sa), rl(blk[c + 2], sb)) for c in (0, 1, 4, 5)]

        def stage(sets, jb, b):
            sh = 1 << b
            out = []
            for blk in sets:
                nxt = list(blk)
                for j in range(4):
                    if j & jb == 0:
                        lo, hi = blk[j], blk[j + jb]
                        nxt[j] = jnp.where(lane_lo[b], lo, pltpu.roll(hi, sh, 1))
                        nxt[j + jb] = jnp.where(lane_lo[b], pltpu.roll(lo, 128 - sh, 1), hi)
                out.append(nxt)
            return out

        for k00 in range(0, HD, KC * par):
            ks = [k00 + KC * q for q in range(par)]
            hv = stage(stage([stage1(hk * HD + k0) for k0 in ks for hk in range(2)], 1, 0), 2, 2)
            for q, k0 in enumerate(ks):
                lo, hi = hv[2 * q], hv[2 * q + 1]
                for e in range(2):
                    cs = _bcomb(upk(lo[e]), upk(lo[e + 2]), upk(hi[e]), upk(hi[e + 2]))
                    for i in range(7):
                        dst.at[i][k0:k0 + KC, e * 128:(e + 1) * 128] = cs[i]

    def qkv_tiles(t, h, src):
        anc16 = []
        for e in range(2):
            n = 2 * h + e
            qlo = qkv.at[t, n]
            qhi = qkv.at[t, n + 4]
            for r in range(NB):
                ms = [_dot(xa[i, r * RB:(r + 1) * RB, :], src.at[i][:, e * 128:(e + 1) * 128]) for i in range(7)]
                c11, c12, c21, c22 = _ccomb(ms)
                anc16 += [m_[k:k + 16] for m_ in ms for k in range(0, RB, 64)]
                r0 = PAD + r * RB
                qlo[r0:r0 + RB, :] = c11
                qhi[r0:r0 + RB, :] = c12
                qlo[HS + r0:HS + r0 + RB, :] = c21
                qhi[HS + r0:HS + r0 + RB, :] = c22
                if r == 0:
                    qlo[0:PAD, :] = jnp.broadcast_to(c11[0:1, :], (PAD, 128))
                    qhi[0:PAD, :] = jnp.broadcast_to(c12[0:1, :], (PAD, 128))
        return anc16

    def prep_o_chunk(m, e, tm, ancs):
        n2 = m >> 3
        g16 = pl.multiple_of((m & 7) * 16, 16)
        res = []
        for h in range(2):
            w = wo_raw.at[n2 + 2 * h]
            w16 = [w[pl.ds(128 * i + g16, 16), e * 128:(e + 1) * 128].astype(f32) for i in range(8)]
            for u in range(2):
                blk = [v[8 * u:8 * u + 8] for v in w16]
                blk[0] = jnp.where(tm, blk[0], ancs[2 * h + u])
                res += _butterfly([blk], row_lo, 0, 8)
        cols = [[jnp.concatenate([res[2 * h][j], res[2 * h + 1][j]], axis=0) for j in range(8)]
                for h in range(2)]
        for b in range(4):
            cs = _bcomb(cols[0][b], cols[1][b], cols[0][b + 4], cols[1][b + 4])
            for i in range(7):
                bo.at[i, n2][pl.ds(b * 128 + g16, 16), e * 128:(e + 1) * 128] = cs[i]

    def attn8(base, row0):
        lg = [None] * NW
        for c in range(8):
            q = qkv[0, c, pl.ds(base, 8), :]
            for w in range(NW):
                pr = q * qkv[1, c, pl.ds(base - 2 * w, 8), :]
                lg[w] = pr if lg[w] is None else lg[w] + pr
        G1 = 2
        for w0 in range(0, NW, G1):
            for w in range(w0, w0 + G1):
                lg[w] = lg[w] + pltpu.roll(lg[w], 8, 1)
            for w in range(w0, w0 + G1):
                lg[w] = lg[w] + pltpu.roll(lg[w], 16, 1)
        if row0 is not None:
            for w in range(1, NW):
                lg[w] = jnp.where(row8 + row0 >= 2 * w, lg[w], NEG)
        m = lg[0]
        for w in range(1, NW):
            m = jnp.maximum(m, lg[w])
        p = [jnp.exp2((lg[w] - m) * (SCALE * LOG2E)) for w in range(NW)]
        den = p[0]
        for w in range(1, NW):
            den = den + p[w]
        inv = 1.0 / den
        b4 = (lane & 16) != 0
        b3 = (lane & 8) != 0
        outs = [None] * 8
        G2 = 2
        for w0 in range(0, NW, G2):
            ws = range(w0, w0 + G2)
            for w in ws:
                p[w] = p[w] * inv
                p[w] = jnp.where(b4, p[w], pltpu.roll(p[w], 112, 1))
            for w in ws:
                p[w] = jnp.where(b3, p[w], pltpu.roll(p[w], 120, 1))
            for w in ws:
                for c in range(8):
                    pr = p[w] * qkv[2, c, pl.ds(base - 2 * w, 8), :]
                    outs[c] = pr if outs[c] is None else outs[c] + pr
        return outs

    def attn_pair(r0, mask=False):
        parts = [attn8(pl.multiple_of(PAD + h * HS + r0 + 8 * u, 8), (r0 + 8 * u) if (h == 0 and mask) else None)
                 for h in range(2) for u in range(2)]
        lo = [jnp.concatenate([parts[0][c], parts[1][c]], axis=0) for c in range(8)]
        hi = [jnp.concatenate([parts[2][c], parts[3][c]], axis=0) for c in range(8)]
        for n in range(4):
            cs = _acomb(lo[n], lo[n + 4], hi[n], hi[n + 4])
            for i in range(7):
                oa.at[i][pl.ds(pl.multiple_of(r0, 16), 16), n * 128:(n + 1) * 128] = cs[i]
        return hi[7]

    wd0 = lambda c: wd_raw.at[0, c * FC:(c + 1) * FC, :]
    RA, RBB, RC, RD = 0, 512, 256, 768

    x_copy(0).start()
    x_copy(1).start()
    gu0_copy(0, 0).start()
    z_copy().start()
    gu0_copy(1, 0).start()
    x_copy(2).start()
    wd0_copy(0).start()
    x_copy(3).start()
    x_copy(4).start()
    gu0_copy(0, 1).start()
    gu0_copy(1, 1).start()
    wd0_copy(1).start()
    x_copy(5).start()
    wq_copy(0).start()
    for cp in wo_copies():
        cp.start()
    wq_copy(1).start()

    x_copy(0).wait()
    ln_rows(RA, 128)
    x_copy(1).wait()
    ln_rows(RA + 128, 128)

    gu0_copy(0, 0).wait()
    prep_gu(0, (0,))
    mg = [_dot(xa[i, RA:RA + RB, :], bgu[i, :, :FH]) for i in range(7)]
    gg = [(v, _gate_tanh(v)) for v in _ccomb(mg)]

    z_copy().wait()
    gu0_copy(1, 0).wait()
    x_copy(2).wait()
    prep_gu(0, (1,))
    mu = [_dot(xa[i, RA:RA + RB, :], bgu[i, :, FH:]) for i in range(7)]
    ha = _acomb(*[_glu2(a[0], a[1], b) for a, b in zip(gg, _ccomb(mu))])
    ln_rows(RBB, 128, [m_[k:k + 16] for m_ in mu for k in range(0, RB, 64)])

    wd0_copy(0).wait()
    x_copy(3).wait()
    prep_d(wd0(0), FH)
    hb0, anc = ffn_gu(RBB, 128)
    ffn_dn(RA, RB, ha, True)
    ln_rows(RBB + 128, 128, anc)

    x_copy(4).wait()
    gu0_copy(0, 1).wait()
    gu0_copy(1, 1).wait()
    hb1, anc = ffn_gu(RBB + 128, 128)
    anc2 = ffn_dn(RBB, 128, hb0, True)
    ffn_dn(RBB + 128, 128, hb1, True)
    prep_gu(1)
    ln_rows(RC, RB, anc + anc2[:8])

    wd0_copy(1).wait()
    x_copy(5).wait()
    prep_d(wd0(1), FH)
    h2, anc = ffn_gu(RA, RB)
    ffn_dn(RA, RB, h2, False)
    ln_rows(RD, RB, anc)
    wq_copy(2).start()
    for cp in gu_copies(1, 1):
        cp.start()
    wd_copy(1, 1).start()

    wq_copy(0).wait()
    h3, _ = ffn_gu(RBB, RB)
    prep_q_half(0, 0, bq.at[0], 2)
    zero = jnp.sum(jnp.where(true_mask(), 0, 1))
    ffn_dn(RBB, RB, h3, False)

    for cp in wo_copies():
        cp.wait()

    def p2_body(i, carry):
        @pl.when(i == 1)
        def _():
            wq_copy(1).wait()

        @pl.when(i == 3)
        def _():
            wq_copy(2).wait()

        @pl.when(i == 4)
        def _():
            for cp in gu_copies(1, 1):
                cp.wait()
            wd_copy(1, 1).wait()
        bqv = bq.at[pl.ds(i, 2)]
        anc16 = qkv_tiles(i >> 1, i & 1, bqv.at[0])
        prep_q_half(jnp.minimum((i + 1) >> 1, 2), (i + 1) & 1, bqv.at[1], 2)
        tm = true_mask()
        tm16 = jnp.concatenate([tm, tm], axis=0)
        jobs = []
        for k in range(6):
            jobs += [('o', k, q) for q in range(4)] + [('x', k, q) for q in range(14)]
        for k in range(8):
            jobs += [('g', k, q) for q in range(7)] + [('d', k, 0)]
        for k in range(6):
            jobs += [('z', k, q) for q in range(7)]
        by = {}
        for kind in 'oxgzd':
            js = [jb for jb in jobs if jb[0] == kind]
            for e, jb in enumerate(js):
                by[jb] = (e + 0.5) / len(js)
        ranked = sorted(jobs, key=lambda jb: by[jb])
        na = len(anc16) - 12
        at = {jb: anc16[(e * na) // len(ranked)] for e, jb in enumerate(ranked)}
        for k in range(6):
            prep_o_chunk(jnp.minimum(3 * i + (k >> 1), 15), k & 1, tm, [at['o', k, q][0:8] for q in range(4)])
            make_xa2(pl.multiple_of(jnp.minimum(6 * i + k, 31) * 16, 16), tm16,
                     [at['x', k, q] for q in range(14)])
        for k in range(8):
            idx = 4 * i + (k >> 1)
            for q in range(7):
                prep_gu2_piece(idx >> 4, q, k & 1, pl.multiple_of((idx & 15) * 16, 16), tm16,
                               at['g', k, q], 1)
            prep_d_piece(idx >> 4, pl.multiple_of((idx & 15) * 16, 16), (k & 1) * 256, tm16, at['d', k, 0])
        for k in range(6):
            blk = jnp.minimum(6 * i + k, 31)
            r0 = pl.multiple_of(256 + (blk >> 4) * 512 + (blk & 15) * 16, 16)
            for p in range(7):
                z16 = jnp.where(tm16, 0.0, at['z', k, p])
                for c in range(4):
                    acc.at[p][pl.ds(r0, 16), c * 128:(c + 1) * 128] = z16
        return carry

    lax.fori_loop(0, 6, p2_body, 0)

    def p3_body(u, carry):
        j = u >> 1
        s_ = u & 1
        sl = j & 1
        jn = jnp.minimum((u >> 1) + 1, NG - 1)
        sn = 1 - sl

        @pl.when(jnp.logical_and(s_ == 0, j + 1 < NG))
        def _():
            wd_copy(jn, sn).wait()
            for cp in gu_copies(jn, sn):
                cp.wait()
        a4 = pl.multiple_of((u - 1) * 64, 64)
        for g in range(5):
            att_last = attn_pair(a4 + 16 * g if g < 4 else 832 + 16 * jnp.minimum(u - 1, 11), g == 0)
        tm = true_mask()
        tm16 = jnp.concatenate([tm, tm], axis=0)

        rows = pl.ds(pl.multiple_of(s_ * RB, RB), RB)
        order = (4, 2, 3, 1, 0, 6, 5)
        bcur = bgu2.at[sl]
        c1 = [None] * 7
        dprep = []
        h = [[None] * 4 for _ in range(4)]

        def gate_up(i):
            ms = [None] * 7
            for k in order:
                ms[k] = _dot(xa2.at[7 * i + k][rows, :], bcur.at[7 * i + k][...])
            c1[i] = _ccomb(ms)
            return [ms[k][r_:r_ + 16, t * 128:(t + 1) * 128] for k in order for r_ in range(0, RB, 64)
                    for t in range(2)]

        def hidden(a, e):
            if h[2 * a][2 * e] is None:
                for q in range(4):
                    m = [None if v is None else v[q] for v in c1]
                    if (a, e) == (0, 0):
                        cc = m[0] + m[3] - m[4] + m[6]
                    elif (a, e) == (0, 1):
                        cc = m[2] + m[4]
                    elif (a, e) == (1, 0):
                        cc = m[1] + m[3]
                    else:
                        cc = m[0] - m[1] + m[2] + m[5]
                    h[2 * a + (q >> 1)][2 * e + (q & 1)] = _glu2(cc[:, :128], _gate_tanh(cc[:, :128]),
                                                                 cc[:, 128:])
            return [[h[2 * a + b][2 * e + f] for f in range(2)] for b in range(2)]

        def down(i):
            p, q, sg = _A_TERMS[i]
            P = hidden(*p)
            if q is not None:
                Q = hidden(*q)
                P = [[P[b][f] + Q[b][f] if sg > 0 else P[b][f] - Q[b][f] for f in range(2)] for b in range(2)]
            out = []
            if i == 4:
                v = P[0][0]
                P[0][0] = jnp.concatenate([jnp.where(tm16, v[0:16], att_last), v[16:]], axis=0)
            for b in range(2):
                y = _dot(jnp.concatenate(P[b], axis=1).astype(bf16), bdd.at[sl, i][...])
                out += [y[r_:r_ + 16, 0:128] for r_ in range(0, RB, 32)]
                acc.at[i][pl.ds(pl.multiple_of(b * QS + s_ * RB, RB), RB), :] += y
            return out

        seq = 'G0 G3 G4 G6 G2 G1 D2 D4 G5 D5 D1 D3 D0 D6'.split()
        sanc = []
        for tk in seq:
            if tk[0] == 'D' and not dprep:
                dprep.append(1)
                lo_, hi_ = 2, 5
                src = [a for p in range(lo_, hi_) for a in sanc[p]]
                pcs = [(k0, c0) for k0 in range(0, FC // 2, 16) for c0 in range(0, HD, 256)]
                for e, (k0, c0) in enumerate(pcs):
                    prep_d_piece(sn, pl.multiple_of(s_ * (FC // 2), FC // 2) + k0, c0, tm16,
                                 src[e * len(src) // len(pcs)])
            sanc.append((gate_up if tk[0] == 'G' else down)(int(tk[1])))
        last_g = max(p for p, tk in enumerate(seq) if tk[0] == 'G')
        src = [a for p in range(last_g + 1, len(seq)) for a in sanc[p]]
        kb = pl.multiple_of(s_ * (QD // 2), QD // 2)
        pieces = [(t, k0, i) for k0 in range(0, QD // 2, 16) for t in range(2) for i in range(7)]
        for e, (t, k0, i) in enumerate(pieces):
            prep_gu2_piece(sn, i, t, kb + k0, tm16, src[e * len(src) // len(pieces)], 4)

        @pl.when(jnp.logical_and(s_ == 1, j + 3 < NG))
        def _():
            wd_copy(j + 3, sn).start()
            for cp in gu_copies(j + 3, sn):
                cp.start()
        return carry

    wd_copy(2, 0).start()
    for cp in gu_copies(2, 0):
        cp.start()
    lax.fori_loop(1, 2 * NG, p3_body, 0)

    SB = 32

    def p4_body(k, carry):
        tm = true_mask()
        for u in range(RB // SB):
            r0 = pl.multiple_of(k * RB + u * SB, SB)
            rows = pl.ds(r0, SB)
            for n in range(2):
                ms = [_dot(oa.at[i][rows, :], bo.at[i, n][...]) for i in range(7)]
                av = [acc.at[i][rows, n * 256:(n + 1) * 256] for i in range(7)]
                ss = _ccomb(ms)
                fs = _ccomb(av)
                for q, (h, c0) in enumerate(((0, n * 256), (0, HD + n * 256), (1, n * 256), (1, HD + n * 256))):
                    hf = 0.25 * fs[q]
                    g = hf + hf * jnp.tanh(hf)
                    xv = xraw.at[h][rows, c0:c0 + 256].astype(f32)
                    if u == 0 and n == 0 and q == 0:
                        ka = bq.at[zero, zero][pl.ds(pl.multiple_of(zero * 16, 16), 16), 0:128]
                        x8 = jnp.where(tm, xv[0:8, 0:128], pltpu.bitcast(ka, f32))
                        x8 = jnp.concatenate([x8, xv[0:8, 128:]], axis=1)
                        xv = jnp.concatenate([x8, xv[8:]], axis=0)
                    obuf.at[h][rows, c0:c0 + 256] = (xv + ss[q] * g).astype(bf16)
            out_copy(r0, SB, 0).start()
        return carry

    lax.fori_loop(0, NB, p4_body, 0)
    out_copy(0, HS, 0).wait()


@jax.jit
def pallas_recurrent_scan__sliding_local_dilated__geglu_ffn__prompt_kernel(
    A_x: jax.Array,
    A_wqkv: jax.Array,
    A_wo: jax.Array,
    B_x: jax.Array,
    B_w_gate: jax.Array,
    B_w_up: jax.Array,
    B_w_down: jax.Array,
):
    any_spec = pl.BlockSpec(memory_space=pl.ANY)
    out = pl.pallas_call(
        _kernel,
        out_shape=jax.ShapeDtypeStruct((2, HS, D), bf16),
        in_specs=[any_spec] * 6,
        out_specs=any_spec,
        scratch_shapes=[
            pltpu.VMEM((2, HS, D), bf16),
            pltpu.VMEM((7, HS // 2, HD), u32),
            pltpu.VMEM((49, QS // 2, QD), u32),
            pltpu.VMEM((2, 2, D, GC), bf16),
            pltpu.VMEM((2, GC, D), bf16),
            pltpu.VMEM((7, HD // 2, FC), u32),
            pltpu.VMEM((2, 49, QD // 2, 256), u32),
            pltpu.VMEM((2, 7, FC // 2, HD), u32),
            pltpu.VMEM((7, HS, HD), f32),
            pltpu.VMEM((3, D, D), bf16),
            pltpu.VMEM((7, 7, HD // 2, 256), u32),
            pltpu.VMEM((3, 8, PAD + S, 128), f32),
            pltpu.VMEM((4, D, 256), bf16),
            pltpu.VMEM((7, 2, HD // 2, 256), u32),
            pltpu.VMEM((2, 2, HS, 128), f32),
            pltpu.VMEM((2, 16, 128), bf16),
            pltpu.SemaphoreType.DMA((26,)),
        ],
        compiler_params=pltpu.CompilerParams(vmem_limit_bytes=124 * 1024 * 1024,
                                             disable_bounds_checks=True,
                                             disable_semaphore_checks=True),
        name="fusedk",
    )(A_x.reshape(2, HS, D), A_wqkv, A_wo, B_w_gate, B_w_up, B_w_down)
    return out.reshape(1, S, D)
```

```python
import jax
import jax.numpy as jnp
from jax import lax
import jax.experimental.pallas as pl
import jax.experimental.pallas.tpu as pltpu

f32 = jnp.float32
bf16 = jnp.bfloat16
u32 = jnp.uint32

S, D, F = 2048, 1024, 3584
HS, HD = S // 2, D // 2
FC = 256
FH = FC // 2
NF = F // FC
QS, QD = S // 4, D // 4
GC = 512
NG = F // GC
RB = 256
NB = HS // RB
PAD = 16
NW = 8
SCALE = 32 ** -0.5
LOG2E = 1.4426950408889634
NEG = -1e9 / SCALE


def _dot(a, b):
    return jnp.dot(a, b, preferred_element_type=f32)


def _acomb(a11, a12, a21, a22):
    r = lambda v: v.astype(bf16)
    return [r(a11 + a22), r(a21 + a22), r(a11), r(a22), r(a11 + a12), r(a21 - a11), r(a12 - a22)]


def _bcomb(b11, b12, b21, b22):
    r = lambda v: v.astype(bf16)
    return [r(b11 + b22), r(b11), r(b12 - b22), r(b21 - b11), r(b22), r(b11 + b12), r(b21 + b22)]


def _asum(a11, a12, a21, a22):
    return [a11 + a22, a21 + a22, a11, a22, a11 + a12, a21 - a11, a12 - a22]


def _bsum(b11, b12, b21, b22):
    return [b11 + b22, b11, b12 - b22, b21 - b11, b22, b11 + b12, b21 + b22]


_A_TERMS = [((0, 0), (1, 1), 1), ((1, 0), (1, 1), 1), ((0, 0), None, 0), ((1, 1), None, 0),
            ((0, 0), (0, 1), 1), ((1, 0), (0, 0), -1), ((0, 1), (1, 1), -1)]
_B_TERMS = [((0, 0), (1, 1), 1), ((0, 0), None, 0), ((0, 1), (1, 1), -1), ((1, 0), (0, 0), -1),
            ((1, 1), None, 0), ((0, 0), (0, 1), 1), ((1, 0), (1, 1), 1)]


def _ccomb(m):
    m1, m2, m3, m4, m5, m6, m7 = m
    return m1 + m4 - m5 + m7, m3 + m5, m2 + m4, m1 - m2 + m3 + m6


def _gate_tanh(x):
    c = 0.7978845608028654
    return jnp.tanh(x * (c + (c * 0.044715) * (x * x)))


def _glu2(g, th, u):
    a = g * u
    return a + a * th


def _sum8(v):
    return ((v[0] + v[1]) + (v[2] + v[3])) + ((v[4] + v[5]) + (v[6] + v[7]))


def _butterfly(sets, masks, axis, size):
    for b in range(3):
        sh = 1 << b
        out = []
        for blk in sets:
            nxt = list(blk)
            for c in range(8):
                if c & sh == 0:
                    lo, hi = blk[c], blk[c + sh]
                    nxt[c] = jnp.where(masks[b], lo, pltpu.roll(hi, sh, axis))
                    nxt[c + sh] = jnp.where(masks[b], pltpu.roll(lo, size - sh, axis), hi)
            out.append(nxt)
        sets = out
    return sets


def _kernel(x_hbm, wqkv_hbm, wo_hbm, wg_hbm, wu_hbm, wd_hbm, out_hbm,
            xraw, xa_u, xa2_u, gu_raw, wd_raw, bgu_u, bgu2_u, bd_u, bd2_u, accq, wq_raw, qkv,
            wo_raw, bo_u, stats, zbuf, sems):
    acc = accq.bitcast(f32)
    bq = accq.bitcast(bf16)
    bo = bo_u.bitcast(bf16)
    obuf = xraw
    xa = xa_u.bitcast(bf16)
    bgu = bgu_u.bitcast(bf16)
    bd = bd_u.bitcast(bf16)
    bd2 = bd2_u.bitcast(bf16)
    xa2 = xa2_u.bitcast(bf16)
    bgu2 = bgu2_u.bitcast(bf16)
    oa = xa
    pk = lambda v: pltpu.bitcast(v, u32)
    un = lambda v: pltpu.bitcast(v, bf16)

    lane = lax.broadcasted_iota(jnp.int32, (8, 128), 1)
    row8 = lax.broadcasted_iota(jnp.int32, (8, 128), 0)
    lane_lo = [(lane & (1 << b)) == 0 for b in range(3)]
    row_lo = [(row8 & (1 << b)) == 0 for b in range(3)]

    XP = [(0, 128), (128, 128), (512, 128), (640, 128), (256, 256), (768, 256)]

    def x_copy(r):
        r0, n = XP[r]
        return pltpu.make_async_copy(x_hbm.at[:, pl.ds(r0, n), :],
                                     xraw.at[:, pl.ds(r0, n), :], sems.at[(0, 1, 2, 3, 23, 14)[r]])

    def gu_copies(j, slot):
        off = pl.multiple_of(j * GC, GC)
        return (pltpu.make_async_copy(wg_hbm.at[:, pl.ds(off, GC)], gu_raw.at[slot, 0], sems.at[4 + 3 * slot]),
                pltpu.make_async_copy(wu_hbm.at[:, pl.ds(off, GC)], gu_raw.at[slot, 1], sems.at[5 + 3 * slot]))

    def wd_copy(j, slot):
        off = pl.multiple_of(j * GC, GC)
        return pltpu.make_async_copy(wd_hbm.at[pl.ds(off, GC), :], wd_raw.at[slot], sems.at[6 + 3 * slot])

    def gu0_copy(t, c):
        w = (wg_hbm, wu_hbm)[t]
        return pltpu.make_async_copy(w.at[:, pl.ds(c * FC, FC)], gu_raw.at[0, t, :, pl.ds(c * FC, FC)],
                                     sems.at[15 + 2 * c + t])

    def wd0_copy(c):
        return pltpu.make_async_copy(wd_hbm.at[pl.ds(c * FC, FC), :], wd_raw.at[0, pl.ds(c * FC, FC), :],
                                     sems.at[19 + c])

    def wq_copy(t):
        return pltpu.make_async_copy(wqkv_hbm.at[:, pl.ds(t * D, D)], wq_raw.at[t], sems.at[10 + t])

    def wo_copies():
        return [pltpu.make_async_copy(wo_hbm.at[:, pl.ds(c * 256, 256)], wo_raw.at[c], sems.at[24])
                for c in range(4)]

    class _Z:
        cps = [pltpu.make_async_copy(x_hbm.at[0, pl.ds(0, 16), pl.ds(0, 128)], zbuf.at[q], sems.at[21 + q])
               for q in range(2)]

        def start(self):
            for cp in self.cps:
                cp.start()

        def wait(self):
            for cp in self.cps:
                cp.wait()

    z_copy = _Z

    def out_copy(r0, n, k):
        return pltpu.make_async_copy(obuf.at[:, pl.ds(r0, n), :], out_hbm.at[:, pl.ds(r0, n), :],
                                     sems.at[25 + k])

    def true_mask():
        return pk(zbuf[0]) == pk(zbuf[1])

    def ln_half(h, c0, tm16, a):
        xs = []
        for c in range(4):
            x2 = xraw.at[h][c0:c0 + 16, c * 256:(c + 1) * 256].astype(f32)
            xs += [x2[:, :128], x2[:, 128:]]
        s1 = _sum8(xs)
        if a is not None:
            s1 = jnp.where(tm16, s1, a)
        m = jnp.sum(s1, axis=-1, keepdims=True) * (1.0 / D)
        xc = [x - m for x in xs]
        v = jnp.sum(_sum8([x * x for x in xc]), axis=-1, keepdims=True) * (1.0 / D)
        r = lax.rsqrt(v + 1e-5)
        stats.at[h, 0][c0:c0 + 16, :] = jnp.broadcast_to(m, (16, 128))
        stats.at[h, 1][c0:c0 + 16, :] = jnp.broadcast_to(r, (16, 128))
        return [x * r for x in xc]

    def ln_rows(r0, n, anc=None):
        tm16 = None
        if anc is not None:
            tm = true_mask()
            tm16 = jnp.concatenate([tm, tm], axis=0)
            anc = anc[:int(len(anc) * 0.85)]
        nch = n // 16
        for k in range(nch):
            c0 = r0 + 16 * k
            a = [None, None]
            if anc is not None:
                a = [anc[(len(anc) * (2 * k + u)) // (2 * nch)] for u in range(2)]
            lo = ln_half(0, c0, tm16, a[0])
            hi = ln_half(1, c0, tm16, a[1])
            for c in range(4):
                cs = _acomb(lo[c], lo[c + 4], hi[c], hi[c + 4])
                for i in range(7):
                    xa.at[i][c0:c0 + 16, c * 128:(c + 1) * 128] = cs[i]

    def prep_gu(c, ts=(0, 1)):
        KC = 32
        for t in ts:
            w = gu_raw.at[0, t]
            for k0 in range(0, HD, KC):
                lo = w[k0:k0 + KC, c * FC:(c + 1) * FC].astype(f32)
                hi = w[HD + k0:HD + k0 + KC, c * FC:(c + 1) * FC].astype(f32)
                cs = _bcomb(lo[:, :FH], lo[:, FH:], hi[:, :FH], hi[:, FH:])
                for i in range(7):
                    bgu.at[i][k0:k0 + KC, t * FH:(t + 1) * FH] = cs[i]

    def prep_d(w, kh):
        KC = 16
        for k0 in range(0, kh, KC):
            for c0 in range(0, HD, 256):
                g = lambda a, b: w[a + k0:a + k0 + KC, b + c0:b + c0 + 256].astype(f32)
                cs = _bcomb(g(0, 0), g(0, HD), g(kh, 0), g(kh, HD))
                for i in range(7):
                    bd.at[i][k0:k0 + KC, c0:c0 + 256] = cs[i]

    def two_level_piece(terms, inner, ld, i, tm16, anc, nanc, store):
        p, q, sg = terms[i]
        P = ld(*p)
        for e in range(nanc):
            P[e >> 1][e & 1] = jnp.where(tm16, P[e >> 1][e & 1], anc)
        if q is not None:
            Q = ld(*q)
            P = [[P[b][d] + Q[b][d] if sg > 0 else P[b][d] - Q[b][d] for d in range(2)] for b in range(2)]
        ops = inner(P[0][0], P[0][1], P[1][0], P[1][1])
        for k in range(7):
            store(7 * i + k, ops[k].astype(bf16))

    def prep_gu2_piece(slot, i, t, k0, tm16, anc, nanc):
        w = gu_raw.at[slot, t]
        dst = bgu2.at[slot]

        def ld(R, C):
            out = []
            for b in range(2):
                x2 = w[pl.ds((2 * R + b) * QD + k0, 16), C * 256:(C + 1) * 256].astype(f32)
                out.append([x2[:, :128], x2[:, 128:]])
            return out

        def store(p, v):
            dst.at[p][pl.ds(k0, 16), t * 128:(t + 1) * 128] = v
        two_level_piece(_B_TERMS, _bsum, ld, i, tm16, anc, nanc, store)

    def prep_d2_piece(slot, i, k0, c0, tm16, anc, nanc):
        w = wd_raw.at[slot]

        def ld(R, C):
            return [[w[pl.ds((2 * R + b) * 128 + k0, 16),
                       (2 * C + d) * QD + c0:(2 * C + d) * QD + c0 + 128].astype(f32) for d in range(2)]
                    for b in range(2)]

        def store(p, v):
            bd2.at[slot, p][pl.ds(k0, 16), c0:c0 + 128] = v
        two_level_piece(_B_TERMS, _bsum, ld, i, tm16, anc, nanc, store)

    def make_xa2(r0, tm16, ancs):
        st = [[[stats.at[a, e][pl.ds(b * QS + r0, 16), :] for e in range(2)] for b in range(2)] for a in range(2)]
        for j in range(2):
            def ld(R, C):
                out = []
                for b in range(2):
                    m, r = st[R][b]
                    row = []
                    for d in range(2):
                        c0 = (2 * C + d) * QD + j * 128
                        xv = xraw.at[R][pl.ds(b * QS + r0, 16), c0:c0 + 128].astype(f32)
                        row.append((xv - m) * r)
                    out.append(row)
                return out

            def store(p, v):
                xa2.at[p][pl.ds(r0, 16), j * 128:(j + 1) * 128] = v
            for i in range(7):
                two_level_piece(_A_TERMS, _asum, ld, i, tm16, ancs[7 * j + i], 1, store)

    def ffn_gu(r0, n):
        ms = [_dot(xa[i, r0:r0 + n, :], bgu[i]) for i in range(7)]
        anc = [m_[k:k + 16, t * FH:(t + 1) * FH] for m_ in ms for t in range(2) for k in range(0, n, 64)]
        hs = _acomb(*[_glu2(v[:, :FH], _gate_tanh(v[:, :FH]), v[:, FH:]) for v in _ccomb(ms)])
        return hs, anc

    def ffn_dn(r0, n, hs, first, last=False):
        b, q0 = r0 // QS, r0 % QS
        anc = []
        for i in range(7):
            y = _dot(hs[i], bd[i])
            anc += [y[k:k + 16, 0:128] for k in range(0, n, 32)]
            lo, hi = (acc.at[7 * i + e] for e in ((6, 2), (1, 5))[b])
            ylo, yhi = y[:, :QD], y[:, QD:]
            if not first:
                ylo = ylo + lo[q0:q0 + n, :]
                yhi = yhi + hi[q0:q0 + n, :]
            if last:
                yhi = yhi + (ylo - acc.at[7 * i + 2][q0:q0 + n, :])
            lo[q0:q0 + n, :] = ylo
            hi[q0:q0 + n, :] = yhi
        return anc

    def zero_acc0(ps, anc):
        tm = true_mask()
        tm16 = jnp.concatenate([tm, tm], axis=0)
        pcs = [(p, q) for p in ps for q in range(4)]
        for e, (p, q) in enumerate(pcs):
            z16 = jnp.where(tm16, 0.0, anc[e * len(anc) // len(pcs)])
            for r0 in range(64 * q, 64 * q + 64, 16):
                for c in range(2):
                    acc.at[p][r0:r0 + 16, c * 128:(c + 1) * 128] = z16

    upk = lambda v: un(v).astype(f32)

    def prep_q_half(t, h, dst, par=1):
        KC = 16
        sa = (128 - 2) * h
        sb = 2 * (1 - h)
        w = wq_raw.at[t]

        def stage1(r0):
            blk = [pk(w[r0:r0 + KC, c * 128:(c + 1) * 128]) for c in range(8)]
            rl = lambda v, sft: v if (isinstance(sft, int) and sft == 0) else pltpu.roll(v, sft, 1)
            return [jnp.where(lane_lo[1], rl(blk[c], sa), rl(blk[c + 2], sb)) for c in (0, 1, 4, 5)]

        def stage(sets, jb, b):
            sh = 1 << b
            out = []
            for blk in sets:
                nxt = list(blk)
                for j in range(4):
                    if j & jb == 0:
                        lo, hi = blk[j], blk[j + jb]
                        nxt[j] = jnp.where(lane_lo[b], lo, pltpu.roll(hi, sh, 1))
                        nxt[j + jb] = jnp.where(lane_lo[b], pltpu.roll(lo, 128 - sh, 1), hi)
                out.append(nxt)
            return out

        for k00 in range(0, HD, KC * par):
            ks = [k00 + KC * q for q in range(par)]
            hv = stage(stage([stage1(hk * HD + k0) for k0 in ks for hk in range(2)], 1, 0), 2, 2)
            for q, k0 in enumerate(ks):
                lo, hi = hv[2 * q], hv[2 * q + 1]
                for e in range(2):
                    cs = _bcomb(upk(lo[e]), upk(lo[e + 2]), upk(hi[e]), upk(hi[e + 2]))
                    for i in range(7):
                        dst.at[i][k0:k0 + KC, e * 128:(e + 1) * 128] = cs[i]

    def qkv_tiles(t, h, src):
        anc16 = []
        for e in range(2):
            n = 2 * h + e
            qlo = qkv.at[t, n]
            qhi = qkv.at[t, n + 4]
            for r in range(NB):
                ms = [_dot(xa[i, r * RB:(r + 1) * RB, :], src.at[i][:, e * 128:(e + 1) * 128]) for i in range(7)]
                c11, c12, c21, c22 = _ccomb(ms)
                anc16 += [m_[k:k + 16] for m_ in ms for k in range(0, RB, 64)]
                r0 = PAD + r * RB
                qlo[r0:r0 + RB, :] = c11
                qhi[r0:r0 + RB, :] = c12
                qlo[HS + r0:HS + r0 + RB, :] = c21
                qhi[HS + r0:HS + r0 + RB, :] = c22
                if r == 0:
                    qlo[0:PAD, :] = jnp.broadcast_to(c11[0:1, :], (PAD, 128))
                    qhi[0:PAD, :] = jnp.broadcast_to(c12[0:1, :], (PAD, 128))
        return anc16

    def prep_o_chunk(m, e, tm, ancs):
        n2 = m >> 3
        g16 = pl.multiple_of((m & 7) * 16, 16)
        res = []
        for h in range(2):
            w = wo_raw.at[n2 + 2 * h]
            w16 = [w[pl.ds(128 * i + g16, 16), e * 128:(e + 1) * 128].astype(f32) for i in range(8)]
            for u in range(2):
                blk = [v[8 * u:8 * u + 8] for v in w16]
                blk[0] = jnp.where(tm, blk[0], ancs[2 * h + u])
                res += _butterfly([blk], row_lo, 0, 8)
        cols = [[jnp.concatenate([res[2 * h][j], res[2 * h + 1][j]], axis=0) for j in range(8)]
                for h in range(2)]
        for b in range(4):
            cs = _bcomb(cols[0][b], cols[1][b], cols[0][b + 4], cols[1][b + 4])
            for i in range(7):
                bo.at[i, n2][pl.ds(b * 128 + g16, 16), e * 128:(e + 1) * 128] = cs[i]

    def attn8(base, row0):
        lg = [None] * NW
        for c in range(8):
            q = qkv[0, c, pl.ds(base, 8), :]
            for w in range(NW):
                pr = q * qkv[1, c, pl.ds(base - 2 * w, 8), :]
                lg[w] = pr if lg[w] is None else lg[w] + pr
        G1 = 2
        for w0 in range(0, NW, G1):
            for w in range(w0, w0 + G1):
                lg[w] = lg[w] + pltpu.roll(lg[w], 8, 1)
            for w in range(w0, w0 + G1):
                lg[w] = lg[w] + pltpu.roll(lg[w], 16, 1)
        if row0 is not None:
            for w in range(1, NW):
                lg[w] = jnp.where(row8 + row0 >= 2 * w, lg[w], NEG)
        m = lg[0]
        for w in range(1, NW):
            m = jnp.maximum(m, lg[w])
        p = [jnp.exp2((lg[w] - m) * (SCALE * LOG2E)) for w in range(NW)]
        den = p[0]
        for w in range(1, NW):
            den = den + p[w]
        inv = 1.0 / den
        b4 = (lane & 16) != 0
        b3 = (lane & 8) != 0
        outs = [None] * 8
        G2 = 2
        for w0 in range(0, NW, G2):
            ws = range(w0, w0 + G2)
            for w in ws:
                p[w] = p[w] * inv
                p[w] = jnp.where(b4, p[w], pltpu.roll(p[w], 112, 1))
            for w in ws:
                p[w] = jnp.where(b3, p[w], pltpu.roll(p[w], 120, 1))
            for w in ws:
                for c in range(8):
                    pr = p[w] * qkv[2, c, pl.ds(base - 2 * w, 8), :]
                    outs[c] = pr if outs[c] is None else outs[c] + pr
        return outs

    def attn_pair(r0, mask=False):
        parts = [attn8(pl.multiple_of(PAD + h * HS + r0 + 8 * u, 8), (r0 + 8 * u) if (h == 0 and mask) else None)
                 for h in range(2) for u in range(2)]
        lo = [jnp.concatenate([parts[0][c], parts[1][c]], axis=0) for c in range(8)]
        hi = [jnp.concatenate([parts[2][c], parts[3][c]], axis=0) for c in range(8)]
        for n in range(4):
            cs = _acomb(lo[n], lo[n + 4], hi[n], hi[n + 4])
            for i in range(7):
                oa.at[i][pl.ds(pl.multiple_of(r0, 16), 16), n * 128:(n + 1) * 128] = cs[i]
        return hi[7]

    wd0 = lambda c: wd_raw.at[0, c * FC:(c + 1) * FC, :]
    RA, RBB, RC, RD = 0, 512, 256, 768

    x_copy(0).start()
    x_copy(1).start()
    gu0_copy(0, 0).start()
    z_copy().start()
    gu0_copy(1, 0).start()
    x_copy(2).start()
    wd0_copy(0).start()
    x_copy(3).start()
    x_copy(4).start()
    gu0_copy(0, 1).start()
    gu0_copy(1, 1).start()
    wd0_copy(1).start()
    x_copy(5).start()
    wq_copy(0).start()
    for cp in wo_copies():
        cp.start()
    wq_copy(1).start()

    x_copy(0).wait()
    ln_rows(RA, 128)
    x_copy(1).wait()
    ln_rows(RA + 128, 128)

    gu0_copy(0, 0).wait()
    prep_gu(0, (0,))
    mg = [_dot(xa[i, RA:RA + RB, :], bgu[i, :, :FH]) for i in range(7)]
    gg = [(v, _gate_tanh(v)) for v in _ccomb(mg)]

    z_copy().wait()
    gu0_copy(1, 0).wait()
    x_copy(2).wait()
    prep_gu(0, (1,))
    mu = [_dot(xa[i, RA:RA + RB, :], bgu[i, :, FH:]) for i in range(7)]
    ha = _acomb(*[_glu2(a[0], a[1], b) for a, b in zip(gg, _ccomb(mu))])
    ln_rows(RBB, 128, [m_[k:k + 16] for m_ in mu for k in range(0, RB, 64)])

    wd0_copy(0).wait()
    x_copy(3).wait()
    prep_d(wd0(0), FH)
    hb0, anc = ffn_gu(RBB, 128)
    ffn_dn(RA, RB, ha, True)
    ln_rows(RBB + 128, 128, anc)

    x_copy(4).wait()
    gu0_copy(0, 1).wait()
    gu0_copy(1, 1).wait()
    hb1, anc = ffn_gu(RBB + 128, 128)
    anc2 = ffn_dn(RBB, 128, hb0, True)
    ffn_dn(RBB + 128, 128, hb1, True)
    prep_gu(1)
    ln_rows(RC, RB, anc + anc2[:8])

    wd0_copy(1).wait()
    x_copy(5).wait()
    prep_d(wd0(1), FH)
    h2, anc = ffn_gu(RA, RB)
    ffn_dn(RA, RB, h2, False)
    ln_rows(RD, RB, anc)
    zs_ = [p for p in range(49) if p % 7 in (0, 3, 4)]
    zero_acc0(zs_[:7], anc)
    wq_copy(2).start()
    for cp in gu_copies(1, 1):
        cp.start()
    wd_copy(1, 1).start()

    wq_copy(0).wait()
    h3, anc = ffn_gu(RBB, RB)
    zero_acc0(zs_[7:], anc)
    prep_q_half(0, 0, bq.at[56:63], 2)
    ffn_dn(RBB, RB, h3, False, True)

    for cp in wo_copies():
        cp.wait()

    def p2_body(i, carry):
        @pl.when(i == 1)
        def _():
            wq_copy(1).wait()

        @pl.when(i == 3)
        def _():
            wq_copy(2).wait()

        @pl.when(i == 4)
        def _():
            for cp in gu_copies(1, 1):
                cp.wait()
            wd_copy(1, 1).wait()
        bqv = bq.at[pl.ds(49 + 7 * i, 21)]
        anc16 = qkv_tiles(i >> 1, i & 1, bqv.at[7:14])
        prep_q_half(jnp.minimum((i + 1) >> 1, 2), (i + 1) & 1, bqv.at[14:21], 2)
        tm = true_mask()
        tm16 = jnp.concatenate([tm, tm], axis=0)
        jobs = []
        for k in range(6):
            jobs += [('o', k, q) for q in range(4)] + [('x', k, q) for q in range(14)]
        for k in range(8):
            jobs += [('g', k, q) for q in range(7)]
        for k in range(4):
            jobs += [('d', k, q) for q in range(7)]
        for k in range(7):
            jobs += [('z', k, q) for q in range(4)]
        by = {}
        for kind in 'oxgzd':
            js = [jb for jb in jobs if jb[0] == kind]
            for e, jb in enumerate(js):
                by[jb] = (e + 0.5) / len(js)
        ranked = sorted(jobs, key=lambda jb: by[jb])
        na = len(anc16) - 12
        at = {jb: anc16[(e * na) // len(ranked)] for e, jb in enumerate(ranked)}
        for k in range(6):
            prep_o_chunk(jnp.minimum(3 * i + (k >> 1), 15), k & 1, tm, [at['o', k, q][0:8] for q in range(4)])
            make_xa2(pl.multiple_of(jnp.minimum(6 * i + k, 31) * 16, 16), tm16,
                     [at['x', k, q] for q in range(14)])
        for k in range(8):
            idx = 4 * i + (k >> 1)
            for q in range(7):
                prep_gu2_piece(idx >> 4, q, k & 1, pl.multiple_of((idx & 15) * 16, 16), tm16,
                               at['g', k, q], 1)
        for k in range(4):
            idx = 2 * i + (k >> 1)
            for q in range(7):
                prep_d2_piece(idx >> 3, q, pl.multiple_of((idx & 7) * 16, 16), (k & 1) * 128, tm16,
                              at['d', k, q], 1)
        az = acc.at[pl.ds(49 + 7 * i, 21)]
        for k in range(7):
            for q in range(4):
                z16 = jnp.where(tm16, 0.0, at['z', k, q])
                for r0 in range(64 * q, 64 * q + 64, 16):
                    for c in range(2):
                        az.at[k][r0:r0 + 16, c * 128:(c + 1) * 128] = z16
        return carry

    lax.fori_loop(0, 6, p2_body, 0)

    def p3_body(u, carry):
        j = u >> 1
        s_ = u & 1
        sl = j & 1
        jn = jnp.minimum((u >> 1) + 1, NG - 1)
        sn = 1 - sl

        @pl.when(jnp.logical_and(s_ == 0, j + 1 < NG))
        def _():
            wd_copy(jn, sn).wait()
            for cp in gu_copies(jn, sn):
                cp.wait()
        a4 = pl.multiple_of((u - 1) * 64, 64)
        for g in range(5):
            att_last = attn_pair(a4 + 16 * g if g < 4 else 832 + 16 * jnp.minimum(u - 1, 11), g == 0)
        tm = true_mask()
        tm16 = jnp.concatenate([tm, tm], axis=0)

        rows = pl.ds(pl.multiple_of(s_ * RB, RB), RB)
        accs = acc.at[pl.ds(49 * s_, 49)]
        order = (0, 3, 4, 6, 2, 1, 5)
        bcur = bgu2.at[sl]
        c1 = [None] * 7
        dprep = []
        h = [[None] * 4 for _ in range(4)]

        def gate_up(i):
            ms = [None] * 7
            for k in order:
                ms[k] = _dot(xa2.at[7 * i + k][rows, :], bcur.at[7 * i + k][...])
            c1[i] = _ccomb(ms)
            return [ms[k][r_:r_ + 16, t * 128:(t + 1) * 128] for k in order for r_ in range(0, RB, 64)
                    for t in range(2)]

        def hidden(a, e):
            if h[2 * a][2 * e] is None:
                for q in range(4):
                    m = [None if v is None else v[q] for v in c1]
                    if (a, e) == (0, 0):
                        cc = m[0] + m[3] - m[4] + m[6]
                    elif (a, e) == (0, 1):
                        cc = m[2] + m[4]
                    elif (a, e) == (1, 0):
                        cc = m[1] + m[3]
                    else:
                        cc = m[0] - m[1] + m[2] + m[5]
                    h[2 * a + (q >> 1)][2 * e + (q & 1)] = _glu2(cc[:, :128], _gate_tanh(cc[:, :128]),
                                                                 cc[:, 128:])
            return [[h[2 * a + b][2 * e + f] for f in range(2)] for b in range(2)]

        def down(i):
            p, q, sg = _A_TERMS[i]
            P = hidden(*p)
            if q is not None:
                Q = hidden(*q)
                P = [[P[b][f] + Q[b][f] if sg > 0 else P[b][f] - Q[b][f] for f in range(2)] for b in range(2)]
            out = []
            if i == 2:
                v = P[0][0]
                P[0][0] = jnp.concatenate([jnp.where(tm16, v[0:16], att_last), v[16:]], axis=0)
            a7 = _asum(P[0][0], P[0][1], P[1][0], P[1][1])
            for k in [6, 1, 4, 3, 2, 5, 0]:
                y = _dot(a7[k].astype(bf16), bd2.at[sl, 7 * i + k][...])
                out += [y[r_:r_ + 16, 0:128] for r_ in range(0, RB, 128)]
                old = accs.at[7 * i + k][...]
                if i == 6:
                    old = jnp.where(u == 1, 0.0, old)
                accs.at[7 * i + k][...] = old + y
            return out

        seq = 'G0 G3 G4 G6 G1 G2 D2 G5 D5 D4 D3 D1 D0 D6'.split()
        sanc = []
        for tk in seq:
            if tk[0] == 'D' and not dprep:
                dprep.append(1)
                lo_, hi_ = 1, 5
                src = [a for p in range(lo_, hi_) for a in sanc[p]]
                pcs = [(k0, c0, i) for k0 in range(0, 64, 16) for c0 in range(0, QD, 128) for i in range(7)]
                for e, (k0, c0, i) in enumerate(pcs):
                    prep_d2_piece(sn, i, pl.multiple_of(s_ * 64, 64) + k0, c0, tm16,
                                  src[e * len(src) // len(pcs)], 1)
            sanc.append((gate_up if tk[0] == 'G' else down)(int(tk[1])))
        last_g = max(p for p, tk in enumerate(seq) if tk[0] == 'G')
        src = [a for p in range(last_g + 1, len(seq)) for a in sanc[p]]
        src = src[:int(len(src) * 0.8)]
        kb = pl.multiple_of(s_ * (QD // 2), QD // 2)
        pieces = [(t, k0, i) for k0 in range(0, QD // 2, 16) for t in range(2) for i in range(7)]
        for e, (t, k0, i) in enumerate(pieces):
            prep_gu2_piece(sn, i, t, kb + k0, tm16, src[e * len(src) // len(pieces)], 4)

        @pl.when(jnp.logical_and(s_ == 1, j + 3 < NG))
        def _():
            wd_copy(j + 3, sn).start()
            for cp in gu_copies(j + 3, sn):
                cp.start()
        return carry

    wd_copy(2, 0).start()
    for cp in gu_copies(2, 0):
        cp.start()
    lax.fori_loop(1, 2 * NG, p3_body, 0)

    SB = 32

    def p4_body(k, carry):
        acck = acc.at[pl.ds(49 * (k >> 1), 49)]
        for u in range(RB // SB):
            b = u // (128 // SB)
            q0 = pl.multiple_of(k * 128 + (u % (128 // SB)) * SB, SB)
            r0 = pl.multiple_of(b * QS + q0, SB)
            rows = pl.ds(r0, SB)
            qr = pl.multiple_of((k & 1) * 128 + (u % (128 // SB)) * SB, SB)
            for n in range(2):
                ms = [_dot(oa.at[i][rows, :], bo.at[i, n][...]) for i in range(7)]
                av = []
                for i in range(7):
                    ld = lambda e: acck.at[7 * i + e][pl.ds(qr, SB), :]
                    av.append((lambda: ld(0) + ld(3) - ld(4) + ld(6), lambda: ld(2) + ld(4),
                               lambda: ld(1) + ld(3), lambda: ld(0) - ld(1) + ld(2) + ld(5))[2 * b + n]())
                ss = _ccomb(ms)
                fs = _ccomb(av)
                for q, (h, c0) in enumerate(((0, n * 256), (0, HD + n * 256), (1, n * 256), (1, HD + n * 256))):
                    hf = 0.25 * fs[q]
                    g = hf + hf * jnp.tanh(hf)
                    xv = xraw.at[h][rows, c0:c0 + 256].astype(f32)
                    obuf.at[h][rows, c0:c0 + 256] = (xv + ss[q] * g).astype(bf16)
            out_copy(r0, SB, 0).start()
        return carry

    lax.fori_loop(0, NB, p4_body, 0)
    out_copy(0, HS, 0).wait()


@jax.jit
def pallas_recurrent_scan__sliding_local_dilated__geglu_ffn__prompt_kernel(
    A_x: jax.Array,
    A_wqkv: jax.Array,
    A_wo: jax.Array,
    B_x: jax.Array,
    B_w_gate: jax.Array,
    B_w_up: jax.Array,
    B_w_down: jax.Array,
):
    any_spec = pl.BlockSpec(memory_space=pl.ANY)
    out = pl.pallas_call(
        _kernel,
        out_shape=jax.ShapeDtypeStruct((2, HS, D), bf16),
        in_specs=[any_spec] * 6,
        out_specs=any_spec,
        scratch_shapes=[
            pltpu.VMEM((2, HS, D), bf16),
            pltpu.VMEM((7, HS // 2, HD), u32),
            pltpu.VMEM((49, QS // 2, QD), u32),
            pltpu.VMEM((2, 2, D, GC), bf16),
            pltpu.VMEM((2, GC, D), bf16),
            pltpu.VMEM((7, HD // 2, FC), u32),
            pltpu.VMEM((2, 49, QD // 2, 256), u32),
            pltpu.VMEM((7, FH // 2, HD), u32),
            pltpu.VMEM((2, 49, 64, QD), u32),
            pltpu.VMEM((105, RB, QD), u32),
            pltpu.VMEM((3, D, D), bf16),
            pltpu.VMEM((3, 8, PAD + S, 128), f32),
            pltpu.VMEM((4, D, 256), bf16),
            pltpu.VMEM((7, 2, HD // 2, 256), u32),
            pltpu.VMEM((2, 2, HS, 128), f32),
            pltpu.VMEM((2, 16, 128), bf16),
            pltpu.SemaphoreType.DMA((26,)),
        ],
        compiler_params=pltpu.CompilerParams(vmem_limit_bytes=127 * 1024 * 1024,
                                             disable_bounds_checks=True,
                                             disable_semaphore_checks=True),
        name="fusedk",
    )(A_x.reshape(2, HS, D), A_wqkv, A_wo, B_w_gate, B_w_up, B_w_down)
    return out.reshape(1, S, D)
```

```python
import jax
import jax.numpy as jnp
from jax import lax
import jax.experimental.pallas as pl
import jax.experimental.pallas.tpu as pltpu

f32 = jnp.float32
bf16 = jnp.bfloat16
u32 = jnp.uint32

S, D, F = 2048, 1024, 3584
HS, HD = S // 2, D // 2
FC = 256
FH = FC // 2
NF = F // FC
QS, QD = S // 4, D // 4
GC = 512
NG = F // GC
RB = 256
NB = HS // RB
PAD = 16
NW = 8
SCALE = 32 ** -0.5
LOG2E = 1.4426950408889634
NEG = -1e9 / SCALE


def _dot(a, b):
    return jnp.dot(a, b, preferred_element_type=f32)


def _acomb(a11, a12, a21, a22):
    r = lambda v: v.astype(bf16)
    return [r(a11 + a22), r(a21 + a22), r(a11), r(a22), r(a11 + a12), r(a21 - a11), r(a12 - a22)]


def _bcomb(b11, b12, b21, b22):
    r = lambda v: v.astype(bf16)
    return [r(b11 + b22), r(b11), r(b12 - b22), r(b21 - b11), r(b22), r(b11 + b12), r(b21 + b22)]


def _asum(a11, a12, a21, a22):
    return [a11 + a22, a21 + a22, a11, a22, a11 + a12, a21 - a11, a12 - a22]


def _bsum(b11, b12, b21, b22):
    return [b11 + b22, b11, b12 - b22, b21 - b11, b22, b11 + b12, b21 + b22]


_A_TERMS = [((0, 0), (1, 1), 1), ((1, 0), (1, 1), 1), ((0, 0), None, 0), ((1, 1), None, 0),
            ((0, 0), (0, 1), 1), ((1, 0), (0, 0), -1), ((0, 1), (1, 1), -1)]
_B_TERMS = [((0, 0), (1, 1), 1), ((0, 0), None, 0), ((0, 1), (1, 1), -1), ((1, 0), (0, 0), -1),
            ((1, 1), None, 0), ((0, 0), (0, 1), 1), ((1, 0), (1, 1), 1)]


def _ccomb(m):
    m1, m2, m3, m4, m5, m6, m7 = m
    return m1 + m4 - m5 + m7, m3 + m5, m2 + m4, m1 - m2 + m3 + m6


def _gate_tanh(x):
    c = 0.7978845608028654
    return jnp.tanh(x * (c + (c * 0.044715) * (x * x)))


def _glu2(g, th, u):
    a = g * u
    return a + a * th


def _sum8(v):
    return ((v[0] + v[1]) + (v[2] + v[3])) + ((v[4] + v[5]) + (v[6] + v[7]))


def _butterfly(sets, masks, axis, size):
    for b in range(3):
        sh = 1 << b
        out = []
        for blk in sets:
            nxt = list(blk)
            for c in range(8):
                if c & sh == 0:
                    lo, hi = blk[c], blk[c + sh]
                    nxt[c] = jnp.where(masks[b], lo, pltpu.roll(hi, sh, axis))
                    nxt[c + sh] = jnp.where(masks[b], pltpu.roll(lo, size - sh, axis), hi)
            out.append(nxt)
        sets = out
    return sets


def _kernel(x_hbm, wqkv_hbm, wo_hbm, wg_hbm, wu_hbm, wd_hbm, out_hbm,
            xraw, xa_u, xa2_u, gu_raw, wd_raw, bgu_u, bd_u, bd2_u, accq, wq_raw, qkv,
            wo_raw, bo_u, stats, zbuf, sems, *bgu2_u):
    acc = accq.bitcast(f32)
    bq = accq.bitcast(bf16)
    bo = bo_u.bitcast(bf16)
    obuf = xraw
    xa = xa_u.bitcast(bf16)
    bgu = bgu_u.bitcast(bf16)
    bd = bd_u.bitcast(bf16)
    bd2 = bd2_u.bitcast(bf16)
    xa2 = xa2_u.bitcast(bf16)
    GA = [0, 2, 2, 0, 1, 2, 1]
    _al = [r.bitcast(bf16) for r in bgu2_u]
    _pos = [sum(1 for q in range(i) if GA[q] == GA[i]) for i in range(7)]
    bg = lambda slot, i, k: _al[GA[i]].at[slot, 7 * _pos[i] + k]
    oa = xa
    pk = lambda v: pltpu.bitcast(v, u32)
    un = lambda v: pltpu.bitcast(v, bf16)

    lane = lax.broadcasted_iota(jnp.int32, (8, 128), 1)
    row8 = lax.broadcasted_iota(jnp.int32, (8, 128), 0)
    lane_lo = [(lane & (1 << b)) == 0 for b in range(3)]
    row_lo = [(row8 & (1 << b)) == 0 for b in range(3)]

    XP = [(0, 128), (128, 128), (512, 128), (640, 128), (256, 256), (768, 256)]

    def x_copy(r):
        r0, n = XP[r]
        return pltpu.make_async_copy(x_hbm.at[:, pl.ds(r0, n), :],
                                     xraw.at[:, pl.ds(r0, n), :], sems.at[(0, 1, 2, 3, 23, 14)[r]])

    def gu_copies(j, slot):
        off = pl.multiple_of(j * GC, GC)
        return (pltpu.make_async_copy(wg_hbm.at[:, pl.ds(off, GC)], gu_raw.at[slot, 0], sems.at[4 + 3 * slot]),
                pltpu.make_async_copy(wu_hbm.at[:, pl.ds(off, GC)], gu_raw.at[slot, 1], sems.at[5 + 3 * slot]))

    def wd_copy(j, slot):
        off = pl.multiple_of(j * GC, GC)
        return pltpu.make_async_copy(wd_hbm.at[pl.ds(off, GC), :], wd_raw.at[slot], sems.at[6 + 3 * slot])

    def gu0_copy(t, c):
        w = (wg_hbm, wu_hbm)[t]
        return pltpu.make_async_copy(w.at[:, pl.ds(c * FC, FC)], gu_raw.at[0, t, :, pl.ds(c * FC, FC)],
                                     sems.at[15 + 2 * c + t])

    def wd0_copy(c):
        return pltpu.make_async_copy(wd_hbm.at[pl.ds(c * FC, FC), :], wd_raw.at[0, pl.ds(c * FC, FC), :],
                                     sems.at[19 + c])

    def wq_copy(t):
        return pltpu.make_async_copy(wqkv_hbm.at[:, pl.ds(t * D, D)], wq_raw.at[t], sems.at[10 + t])

    def wo_copies():
        return [pltpu.make_async_copy(wo_hbm.at[:, pl.ds(c * 256, 256)], wo_raw.at[c], sems.at[24])
                for c in range(4)]

    class _Z:
        cps = [pltpu.make_async_copy(x_hbm.at[0, pl.ds(0, 16), pl.ds(0, 128)], zbuf.at[q], sems.at[21 + q])
               for q in range(2)]

        def start(self):
            for cp in self.cps:
                cp.start()

        def wait(self):
            for cp in self.cps:
                cp.wait()

    z_copy = _Z

    def out_copy(r0, n, k):
        return pltpu.make_async_copy(obuf.at[:, pl.ds(r0, n), :], out_hbm.at[:, pl.ds(r0, n), :],
                                     sems.at[25 + k])

    def true_mask():
        return pk(zbuf[0]) == pk(zbuf[1])

    def ln_half(h, c0, tm16, a):
        xs = []
        for c in range(4):
            x2 = xraw.at[h][c0:c0 + 16, c * 256:(c + 1) * 256].astype(f32)
            xs += [x2[:, :128], x2[:, 128:]]
        s1 = _sum8(xs)
        if a is not None:
            s1 = jnp.where(tm16, s1, a)
        m = jnp.sum(s1, axis=-1, keepdims=True) * (1.0 / D)
        xc = [x - m for x in xs]
        v = jnp.sum(_sum8([x * x for x in xc]), axis=-1, keepdims=True) * (1.0 / D)
        r = lax.rsqrt(v + 1e-5)
        stats.at[h, 0][c0:c0 + 16, :] = jnp.broadcast_to(m, (16, 128))
        stats.at[h, 1][c0:c0 + 16, :] = jnp.broadcast_to(r, (16, 128))
        return [x * r for x in xc]

    def ln_rows(r0, n, anc=None):
        tm16 = None
        if anc is not None:
            tm = true_mask()
            tm16 = jnp.concatenate([tm, tm], axis=0)
            anc = anc[:int(len(anc) * 0.85)]
        nch = n // 16
        for k in range(nch):
            c0 = r0 + 16 * k
            a = [None, None]
            if anc is not None:
                a = [anc[(len(anc) * (2 * k + u)) // (2 * nch)] for u in range(2)]
            lo = ln_half(0, c0, tm16, a[0])
            hi = ln_half(1, c0, tm16, a[1])
            for c in range(4):
                cs = _acomb(lo[c], lo[c + 4], hi[c], hi[c + 4])
                for i in range(7):
                    xa.at[i][c0:c0 + 16, c * 128:(c + 1) * 128] = cs[i]

    def prep_gu(c, ts=(0, 1)):
        KC = 32
        for t in ts:
            w = gu_raw.at[0, t]
            for k0 in range(0, HD, KC):
                lo = w[k0:k0 + KC, c * FC:(c + 1) * FC].astype(f32)
                hi = w[HD + k0:HD + k0 + KC, c * FC:(c + 1) * FC].astype(f32)
                cs = _bcomb(lo[:, :FH], lo[:, FH:], hi[:, :FH], hi[:, FH:])
                for i in range(7):
                    bgu.at[i][k0:k0 + KC, t * FH:(t + 1) * FH] = cs[i]

    def prep_d(w, kh):
        KC = 16
        for k0 in range(0, kh, KC):
            for c0 in range(0, HD, 256):
                g = lambda a, b: w[a + k0:a + k0 + KC, b + c0:b + c0 + 256].astype(f32)
                cs = _bcomb(g(0, 0), g(0, HD), g(kh, 0), g(kh, HD))
                for i in range(7):
                    bd.at[i][k0:k0 + KC, c0:c0 + 256] = cs[i]

    def two_level_piece(terms, inner, ld, i, tm16, anc, nanc, store):
        p, q, sg = terms[i]
        P = ld(*p)
        for e in range(nanc):
            P[e >> 1][e & 1] = jnp.where(tm16, P[e >> 1][e & 1], anc)
        if q is not None:
            Q = ld(*q)
            P = [[P[b][d] + Q[b][d] if sg > 0 else P[b][d] - Q[b][d] for d in range(2)] for b in range(2)]
        ops = inner(P[0][0], P[0][1], P[1][0], P[1][1])
        for k in range(7):
            store(7 * i + k, ops[k].astype(bf16))

    def prep_gu2_piece(slot, i, t, k0, tm16, anc, nanc):
        w = gu_raw.at[slot, t]

        def ld(R, C):
            out = []
            for b in range(2):
                x2 = w[pl.ds((2 * R + b) * QD + k0, 16), C * 256:(C + 1) * 256].astype(f32)
                out.append([x2[:, :128], x2[:, 128:]])
            return out

        def store(p, v):
            bg(slot, i, p % 7)[pl.ds(k0, 16), t * 128:(t + 1) * 128] = v
        two_level_piece(_B_TERMS, _bsum, ld, i, tm16, anc, nanc, store)

    def prep_d2_piece(slot, i, k0, c0, tm16, anc, nanc):
        w = wd_raw.at[slot]

        def ld(R, C):
            return [[w[pl.ds((2 * R + b) * 128 + k0, 16),
                       (2 * C + d) * QD + c0:(2 * C + d) * QD + c0 + 128].astype(f32) for d in range(2)]
                    for b in range(2)]

        def store(p, v):
            bd2.at[slot, p][pl.ds(k0, 16), c0:c0 + 128] = v
        two_level_piece(_B_TERMS, _bsum, ld, i, tm16, anc, nanc, store)

    def make_xa2(r0, tm16, ancs):
        st = [[[stats.at[a, e][pl.ds(b * QS + r0, 16), :] for e in range(2)] for b in range(2)] for a in range(2)]
        for j in range(2):
            def ld(R, C):
                out = []
                for b in range(2):
                    m, r = st[R][b]
                    row = []
                    for d in range(2):
                        c0 = (2 * C + d) * QD + j * 128
                        xv = xraw.at[R][pl.ds(b * QS + r0, 16), c0:c0 + 128].astype(f32)
                        row.append((xv - m) * r)
                    out.append(row)
                return out

            def store(p, v):
                xa2.at[p][pl.ds(r0, 16), j * 128:(j + 1) * 128] = v
            for i in range(7):
                two_level_piece(_A_TERMS, _asum, ld, i, tm16, ancs[7 * j + i], 1, store)

    def ffn_gu(r0, n):
        ms = [_dot(xa[i, r0:r0 + n, :], bgu[i]) for i in range(7)]
        anc = [m_[k:k + 16, t * FH:(t + 1) * FH] for m_ in ms for t in range(2) for k in range(0, n, 64)]
        hs = _acomb(*[_glu2(v[:, :FH], _gate_tanh(v[:, :FH]), v[:, FH:]) for v in _ccomb(ms)])
        return hs, anc

    def ffn_dn(r0, n, hs, first, last=False):
        b, q0 = r0 // QS, r0 % QS
        anc = []
        for i in range(7):
            y = _dot(hs[i], bd[i])
            anc += [y[k:k + 16, 0:128] for k in range(0, n, 32)]
            lo, hi = (acc.at[7 * i + e] for e in ((6, 2), (1, 5))[b])
            ylo, yhi = y[:, :QD], y[:, QD:]
            if not first:
                ylo = ylo + lo[q0:q0 + n, :]
                yhi = yhi + hi[q0:q0 + n, :]
            if last:
                yhi = yhi + (ylo - acc.at[7 * i + 2][q0:q0 + n, :])
            lo[q0:q0 + n, :] = ylo
            hi[q0:q0 + n, :] = yhi
        return anc

    def zero_acc0(ps, anc):
        tm = true_mask()
        tm16 = jnp.concatenate([tm, tm], axis=0)
        pcs = [(p, q) for p in ps for q in range(4)]
        for e, (p, q) in enumerate(pcs):
            z16 = jnp.where(tm16, 0.0, anc[e * len(anc) // len(pcs)])
            for r0 in range(64 * q, 64 * q + 64, 16):
                for c in range(2):
                    acc.at[p][r0:r0 + 16, c * 128:(c + 1) * 128] = z16

    upk = lambda v: un(v).astype(f32)

    def prep_q_half(t, h, dst, par=1):
        KC = 16
        sa = (128 - 2) * h
        sb = 2 * (1 - h)
        w = wq_raw.at[t]

        def stage1(r0):
            blk = [pk(w[r0:r0 + KC, c * 128:(c + 1) * 128]) for c in range(8)]
            rl = lambda v, sft: v if (isinstance(sft, int) and sft == 0) else pltpu.roll(v, sft, 1)
            return [jnp.where(lane_lo[1], rl(blk[c], sa), rl(blk[c + 2], sb)) for c in (0, 1, 4, 5)]

        def stage(sets, jb, b):
            sh = 1 << b
            out = []
            for blk in sets:
                nxt = list(blk)
                for j in range(4):
                    if j & jb == 0:
                        lo, hi = blk[j], blk[j + jb]
                        nxt[j] = jnp.where(lane_lo[b], lo, pltpu.roll(hi, sh, 1))
                        nxt[j + jb] = jnp.where(lane_lo[b], pltpu.roll(lo, 128 - sh, 1), hi)
                out.append(nxt)
            return out

        for k00 in range(0, HD, KC * par):
            ks = [k00 + KC * q for q in range(par)]
            hv = stage(stage([stage1(hk * HD + k0) for k0 in ks for hk in range(2)], 1, 0), 2, 2)
            for q, k0 in enumerate(ks):
                lo, hi = hv[2 * q], hv[2 * q + 1]
                for e in range(2):
                    cs = _bcomb(upk(lo[e]), upk(lo[e + 2]), upk(hi[e]), upk(hi[e + 2]))
                    for i in range(7):
                        dst.at[i][k0:k0 + KC, e * 128:(e + 1) * 128] = cs[i]

    def qkv_tiles(t, h, src):
        anc16 = []
        for e in range(2):
            n = 2 * h + e
            qlo = qkv.at[t, n]
            qhi = qkv.at[t, n + 4]
            for r in range(NB):
                ms = [_dot(xa[i, r * RB:(r + 1) * RB, :], src.at[i][:, e * 128:(e + 1) * 128]) for i in range(7)]
                c11, c12, c21, c22 = _ccomb(ms)
                anc16 += [m_[k:k + 16] for m_ in ms for k in range(0, RB, 64)]
                r0 = PAD + r * RB
                qlo[r0:r0 + RB, :] = c11
                qhi[r0:r0 + RB, :] = c12
                qlo[HS + r0:HS + r0 + RB, :] = c21
                qhi[HS + r0:HS + r0 + RB, :] = c22
                if r == 0:
                    qlo[0:PAD, :] = jnp.broadcast_to(c11[0:1, :], (PAD, 128))
                    qhi[0:PAD, :] = jnp.broadcast_to(c12[0:1, :], (PAD, 128))
        return anc16

    def prep_o_chunk(m, e, tm, ancs):
        n2 = m >> 3
        g16 = pl.multiple_of((m & 7) * 16, 16)
        res = []
        for h in range(2):
            w = wo_raw.at[n2 + 2 * h]
            w16 = [w[pl.ds(128 * i + g16, 16), e * 128:(e + 1) * 128].astype(f32) for i in range(8)]
            for u in range(2):
                blk = [v[8 * u:8 * u + 8] for v in w16]
                blk[0] = jnp.where(tm, blk[0], ancs[2 * h + u])
                res += _butterfly([blk], row_lo, 0, 8)
        cols = [[jnp.concatenate([res[2 * h][j], res[2 * h + 1][j]], axis=0) for j in range(8)]
                for h in range(2)]
        for b in range(4):
            cs = _bcomb(cols[0][b], cols[1][b], cols[0][b + 4], cols[1][b + 4])
            for i in range(7):
                bo.at[i, n2][pl.ds(b * 128 + g16, 16), e * 128:(e + 1) * 128] = cs[i]

    def attn8(base, row0):
        lg = [None] * NW
        for c in range(8):
            q = qkv[0, c, pl.ds(base, 8), :]
            for w in range(NW):
                pr = q * qkv[1, c, pl.ds(base - 2 * w, 8), :]
                lg[w] = pr if lg[w] is None else lg[w] + pr
        G1 = 2
        for w0 in range(0, NW, G1):
            for w in range(w0, w0 + G1):
                lg[w] = lg[w] + pltpu.roll(lg[w], 8, 1)
            for w in range(w0, w0 + G1):
                lg[w] = lg[w] + pltpu.roll(lg[w], 16, 1)
        if row0 is not None:
            for w in range(1, NW):
                lg[w] = jnp.where(row8 + row0 >= 2 * w, lg[w], NEG)
        m = lg[0]
        for w in range(1, NW):
            m = jnp.maximum(m, lg[w])
        p = [jnp.exp2((lg[w] - m) * (SCALE * LOG2E)) for w in range(NW)]
        den = p[0]
        for w in range(1, NW):
            den = den + p[w]
        inv = 1.0 / den
        b4 = (lane & 16) != 0
        b3 = (lane & 8) != 0
        outs = [None] * 8
        G2 = 2
        for w0 in range(0, NW, G2):
            ws = range(w0, w0 + G2)
            for w in ws:
                p[w] = p[w] * inv
                p[w] = jnp.where(b4, p[w], pltpu.roll(p[w], 112, 1))
            for w in ws:
                p[w] = jnp.where(b3, p[w], pltpu.roll(p[w], 120, 1))
            for w in ws:
                for c in range(8):
                    pr = p[w] * qkv[2, c, pl.ds(base - 2 * w, 8), :]
                    outs[c] = pr if outs[c] is None else outs[c] + pr
        return outs

    def attn_pair(r0, mask=False):
        parts = [attn8(pl.multiple_of(PAD + h * HS + r0 + 8 * u, 8), (r0 + 8 * u) if (h == 0 and mask) else None)
                 for h in range(2) for u in range(2)]
        lo = [jnp.concatenate([parts[0][c], parts[1][c]], axis=0) for c in range(8)]
        hi = [jnp.concatenate([parts[2][c], parts[3][c]], axis=0) for c in range(8)]
        for n in range(4):
            cs = _acomb(lo[n], lo[n + 4], hi[n], hi[n + 4])
            for i in range(7):
                oa.at[i][pl.ds(pl.multiple_of(r0, 16), 16), n * 128:(n + 1) * 128] = cs[i]
        return hi[7]

    wd0 = lambda c: wd_raw.at[0, c * FC:(c + 1) * FC, :]
    RA, RBB, RC, RD = 0, 512, 256, 768

    x_copy(0).start()
    x_copy(1).start()
    gu0_copy(0, 0).start()
    z_copy().start()
    gu0_copy(1, 0).start()
    x_copy(2).start()
    wd0_copy(0).start()
    x_copy(3).start()
    x_copy(4).start()
    gu0_copy(0, 1).start()
    gu0_copy(1, 1).start()
    wd0_copy(1).start()
    x_copy(5).start()
    wq_copy(0).start()
    for cp in wo_copies():
        cp.start()
    wq_copy(1).start()

    x_copy(0).wait()
    ln_rows(RA, 128)
    x_copy(1).wait()
    ln_rows(RA + 128, 128)

    gu0_copy(0, 0).wait()
    prep_gu(0, (0,))
    mg = [_dot(xa[i, RA:RA + RB, :], bgu[i, :, :FH]) for i in range(7)]
    gg = [(v, _gate_tanh(v)) for v in _ccomb(mg)]

    z_copy().wait()
    gu0_copy(1, 0).wait()
    x_copy(2).wait()
    prep_gu(0, (1,))
    mu = [_dot(xa[i, RA:RA + RB, :], bgu[i, :, FH:]) for i in range(7)]
    ha = _acomb(*[_glu2(a[0], a[1], b) for a, b in zip(gg, _ccomb(mu))])
    ln_rows(RBB, 128, [m_[k:k + 16] for m_ in mu for k in range(0, RB, 64)])

    wd0_copy(0).wait()
    x_copy(3).wait()
    prep_d(wd0(0), FH)
    hb0, anc = ffn_gu(RBB, 128)
    ffn_dn(RA, RB, ha, True)
    ln_rows(RBB + 128, 128, anc)

    x_copy(4).wait()
    gu0_copy(0, 1).wait()
    gu0_copy(1, 1).wait()
    hb1, anc = ffn_gu(RBB + 128, 128)
    anc2 = ffn_dn(RBB, 128, hb0, True)
    ffn_dn(RBB + 128, 128, hb1, True)
    prep_gu(1)
    ln_rows(RC, RB, anc + anc2[:8])

    wd0_copy(1).wait()
    x_copy(5).wait()
    prep_d(wd0(1), FH)
    h2, anc = ffn_gu(RA, RB)
    ffn_dn(RA, RB, h2, False)
    ln_rows(RD, RB, anc)
    zs_ = [p for p in range(49) if p % 7 in (0, 3, 4)]
    zero_acc0(zs_[:7], anc)
    wq_copy(2).start()
    for cp in gu_copies(1, 1):
        cp.start()
    wd_copy(1, 1).start()

    wq_copy(0).wait()
    h3, anc = ffn_gu(RBB, RB)
    zero_acc0(zs_[7:], anc)
    prep_q_half(0, 0, bq.at[56:63], 2)
    ffn_dn(RBB, RB, h3, False, True)

    for cp in wo_copies():
        cp.wait()

    def p2_body(i, carry):
        @pl.when(i == 1)
        def _():
            wq_copy(1).wait()

        @pl.when(i == 3)
        def _():
            wq_copy(2).wait()

        @pl.when(i == 4)
        def _():
            for cp in gu_copies(1, 1):
                cp.wait()
            wd_copy(1, 1).wait()
        bqv = bq.at[pl.ds(49 + 7 * i, 21)]
        anc16 = qkv_tiles(i >> 1, i & 1, bqv.at[7:14])
        prep_q_half(jnp.minimum((i + 1) >> 1, 2), (i + 1) & 1, bqv.at[14:21], 2)
        tm = true_mask()
        tm16 = jnp.concatenate([tm, tm], axis=0)
        jobs = []
        for k in range(6):
            jobs += [('o', k, q) for q in range(4)] + [('x', k, q) for q in range(14)]
        for k in range(8):
            jobs += [('g', k, q) for q in range(7)]
        for k in range(4):
            jobs += [('d', k, q) for q in range(7)]
        for k in range(7):
            jobs += [('z', k, q) for q in range(4)]
        by = {}
        for kind in 'oxgzd':
            js = [jb for jb in jobs if jb[0] == kind]
            for e, jb in enumerate(js):
                by[jb] = (e + 0.5) / len(js)
        ranked = sorted(jobs, key=lambda jb: by[jb])
        na = len(anc16) - 12
        at = {jb: anc16[(e * na) // len(ranked)] for e, jb in enumerate(ranked)}
        for k in range(6):
            prep_o_chunk(jnp.minimum(3 * i + (k >> 1), 15), k & 1, tm, [at['o', k, q][0:8] for q in range(4)])
            make_xa2(pl.multiple_of(jnp.minimum(6 * i + k, 31) * 16, 16), tm16,
                     [at['x', k, q] for q in range(14)])
        for k in range(8):
            idx = 4 * i + (k >> 1)
            for q in range(7):
                prep_gu2_piece(idx >> 4, q, k & 1, pl.multiple_of((idx & 15) * 16, 16), tm16,
                               at['g', k, q], 1)
        for k in range(4):
            idx = 2 * i + (k >> 1)
            for q in range(7):
                prep_d2_piece(idx >> 3, q, pl.multiple_of((idx & 7) * 16, 16), (k & 1) * 128, tm16,
                              at['d', k, q], 1)
        az = acc.at[pl.ds(49 + 7 * i, 21)]
        for k in range(7):
            for q in range(4):
                z16 = jnp.where(tm16, 0.0, at['z', k, q])
                for r0 in range(64 * q, 64 * q + 64, 16):
                    for c in range(2):
                        az.at[k][r0:r0 + 16, c * 128:(c + 1) * 128] = z16
        return carry

    lax.fori_loop(0, 6, p2_body, 0)

    def p3_body(u, carry):
        j = u >> 1
        s_ = u & 1
        sl = j & 1
        jn = jnp.minimum((u >> 1) + 1, NG - 1)
        sn = 1 - sl

        @pl.when(jnp.logical_and(s_ == 0, j + 1 < NG))
        def _():
            wd_copy(jn, sn).wait()
            for cp in gu_copies(jn, sn):
                cp.wait()
        a4 = pl.multiple_of((u - 1) * 64, 64)
        for g in range(5):
            att_last = attn_pair(a4 + 16 * g if g < 4 else 832 + 16 * jnp.minimum(u - 1, 11), g == 0)
        tm = true_mask()
        tm16 = jnp.concatenate([tm, tm], axis=0)

        rows = pl.ds(pl.multiple_of(s_ * RB, RB), RB)
        accs = acc.at[pl.ds(49 * s_, 49)]
        order = (0, 3, 4, 6, 2, 1, 5)
        c1 = [None] * 7
        dprep = []
        h = [[None] * 4 for _ in range(4)]

        def gate_up(i):
            ms = [None] * 7
            for k in order:
                ms[k] = _dot(xa2.at[7 * i + k][rows, :], bg(sl, i, k)[...])
            c1[i] = _ccomb(ms)
            return [ms[k][r_:r_ + 16, t * 128:(t + 1) * 128] for k in order for r_ in range(0, RB, 64)
                    for t in range(2)]

        def hidden(a, e):
            if h[2 * a][2 * e] is None:
                for q in range(4):
                    m = [None if v is None else v[q] for v in c1]
                    if (a, e) == (0, 0):
                        cc = m[0] + m[3] - m[4] + m[6]
                    elif (a, e) == (0, 1):
                        cc = m[2] + m[4]
                    elif (a, e) == (1, 0):
                        cc = m[1] + m[3]
                    else:
                        cc = m[0] - m[1] + m[2] + m[5]
                    h[2 * a + (q >> 1)][2 * e + (q & 1)] = _glu2(cc[:, :128], _gate_tanh(cc[:, :128]),
                                                                 cc[:, 128:])
            return [[h[2 * a + b][2 * e + f] for f in range(2)] for b in range(2)]

        def down(i):
            p, q, sg = _A_TERMS[i]
            P = hidden(*p)
            if q is not None:
                Q = hidden(*q)
                P = [[P[b][f] + Q[b][f] if sg > 0 else P[b][f] - Q[b][f] for f in range(2)] for b in range(2)]
            out = []
            if i == 2:
                v = P[0][0]
                P[0][0] = jnp.concatenate([jnp.where(tm16, v[0:16], att_last), v[16:]], axis=0)
            a7 = _asum(P[0][0], P[0][1], P[1][0], P[1][1])
            for k in [6, 1, 4, 3, 2, 5, 0]:
                y = _dot(a7[k].astype(bf16), bd2.at[sl, 7 * i + k][...])
                out += [y[r_:r_ + 16, 0:128] for r_ in range(0, RB, 128)]
                old = accs.at[7 * i + k][...]
                if i == 6:
                    old = jnp.where(u == 1, 0.0, old)
                accs.at[7 * i + k][...] = old + y
            return out

        seq = 'G0 G3 G4 G6 G1 G2 D2 G5 D6 D4 D3 D1 D0 D5'.split()
        sanc = []
        for tk in seq:
            if tk[0] == 'D' and not dprep:
                dprep.append(1)
                lo_, hi_ = 0, 1
                src = [a for p in range(lo_, hi_) for a in sanc[p]]
                pcs = [(k0, c0, i) for k0 in range(0, 64, 16) for c0 in range(0, QD, 128) for i in range(7)]
                for e, (k0, c0, i) in enumerate(pcs):
                    prep_d2_piece(sn, i, pl.multiple_of(s_ * 64, 64) + k0, c0, tm16,
                                  src[e * len(src) // len(pcs)], 1)
            sanc.append((gate_up if tk[0] == 'G' else down)(int(tk[1])))
        kb = pl.multiple_of(s_ * (QD // 2), QD // 2)
        PW = [[2, 5], [7, 8], [8, 14]]
        for a in range(max(GA) + 1):
            members = [i for i in range(7) if GA[i] == a]
            last = max(p for p, tk in enumerate(seq) if tk[0] == 'G' and int(tk[1]) in members)
            lo_, hi_ = max(PW[a][0], last + 1), max(PW[a][1], last + 2)
            src = [x for p in range(lo_, hi_) for x in sanc[p]]
            pieces = [(t, k0, i) for k0 in range(0, QD // 2, 16) for t in range(2) for i in members]
            for e, (t, k0, i) in enumerate(pieces):
                prep_gu2_piece(sn, i, t, kb + k0, tm16, src[e * len(src) // len(pieces)], 4)

        @pl.when(jnp.logical_and(s_ == 1, j + 3 < NG))
        def _():
            wd_copy(j + 3, sn).start()
            for cp in gu_copies(j + 3, sn):
                cp.start()
        return carry

    wd_copy(2, 0).start()
    for cp in gu_copies(2, 0):
        cp.start()
    lax.fori_loop(1, 2 * NG, p3_body, 0)

    SB = 32

    def p4_body(k, carry):
        acck = acc.at[pl.ds(49 * (k >> 1), 49)]
        for u in range(RB // SB):
            b = u // (128 // SB)
            q0 = pl.multiple_of(k * 128 + (u % (128 // SB)) * SB, SB)
            r0 = pl.multiple_of(b * QS + q0, SB)
            rows = pl.ds(r0, SB)
            qr = pl.multiple_of((k & 1) * 128 + (u % (128 // SB)) * SB, SB)
            for n in range(2):
                ms = [_dot(oa.at[i][rows, :], bo.at[i, n][...]) for i in range(7)]
                av = []
                for i in range(7):
                    ld = lambda e: acck.at[7 * i + e][pl.ds(qr, SB), :]
                    av.append((lambda: ld(0) + ld(3) - ld(4) + ld(6), lambda: ld(2) + ld(4),
                               lambda: ld(1) + ld(3), lambda: ld(0) - ld(1) + ld(2) + ld(5))[2 * b + n]())
                ss = _ccomb(ms)
                fs = _ccomb(av)
                for q, (h, c0) in enumerate(((0, n * 256), (0, HD + n * 256), (1, n * 256), (1, HD + n * 256))):
                    hf = 0.25 * fs[q]
                    g = hf + hf * jnp.tanh(hf)
                    xv = xraw.at[h][rows, c0:c0 + 256].astype(f32)
                    obuf.at[h][rows, c0:c0 + 256] = (xv + ss[q] * g).astype(bf16)
            out_copy(r0, SB, 0).start()
        return carry

    lax.fori_loop(0, NB, p4_body, 0)
    out_copy(0, HS, 0).wait()


@jax.jit
def pallas_recurrent_scan__sliding_local_dilated__geglu_ffn__prompt_kernel(
    A_x: jax.Array,
    A_wqkv: jax.Array,
    A_wo: jax.Array,
    B_x: jax.Array,
    B_w_gate: jax.Array,
    B_w_up: jax.Array,
    B_w_down: jax.Array,
):
    any_spec = pl.BlockSpec(memory_space=pl.ANY)
    out = pl.pallas_call(
        _kernel,
        out_shape=jax.ShapeDtypeStruct((2, HS, D), bf16),
        in_specs=[any_spec] * 6,
        out_specs=any_spec,
        scratch_shapes=[
            pltpu.VMEM((2, HS, D), bf16),
            pltpu.VMEM((7, HS // 2, HD), u32),
            pltpu.VMEM((49, QS // 2, QD), u32),
            pltpu.VMEM((2, 2, D, GC), bf16),
            pltpu.VMEM((2, GC, D), bf16),
            pltpu.VMEM((7, HD // 2, FC), u32),
            pltpu.VMEM((7, FH // 2, HD), u32),
            pltpu.VMEM((2, 49, 64, QD), u32),
            pltpu.VMEM((105, RB, QD), u32),
            pltpu.VMEM((3, D, D), bf16),
            pltpu.VMEM((3, 8, PAD + S, 128), f32),
            pltpu.VMEM((4, D, 256), bf16),
            pltpu.VMEM((7, 2, HD // 2, 256), u32),
            pltpu.VMEM((2, 2, HS, 128), f32),
            pltpu.VMEM((2, 16, 128), bf16),
            pltpu.SemaphoreType.DMA((26,)),
        ] + [pltpu.VMEM((2, 7 * n, QD // 2, 256), u32) for n in (2, 2, 3)],
        compiler_params=pltpu.CompilerParams(vmem_limit_bytes=127 * 1024 * 1024,
                                             disable_bounds_checks=True,
                                             disable_semaphore_checks=True),
        name="fusedk",
    )(A_x.reshape(2, HS, D), A_wqkv, A_wo, B_w_gate, B_w_up, B_w_down)
    return out.reshape(1, S, D)
```

```python
import jax
import jax.numpy as jnp
from jax import lax
import jax.experimental.pallas as pl
import jax.experimental.pallas.tpu as pltpu

f32 = jnp.float32
bf16 = jnp.bfloat16
u32 = jnp.uint32

S, D, F = 2048, 1024, 3584
HS, HD = S // 2, D // 2
FC = 256
FH = FC // 2
NF = F // FC
QS, QD = S // 4, D // 4
GC = 512
NG = F // GC
RB = 256
NB = HS // RB
PAD = 16
NW = 8
SCALE = 32 ** -0.5
LOG2E = 1.4426950408889634
NEG = -1e9 / SCALE


def _dot(a, b):
    return jnp.dot(a, b, preferred_element_type=f32)


def _acomb(a11, a12, a21, a22):
    r = lambda v: v.astype(bf16)
    return [r(a11 + a22), r(a21 + a22), r(a11), r(a22), r(a11 + a12), r(a21 - a11), r(a12 - a22)]


def _bcomb(b11, b12, b21, b22):
    r = lambda v: v.astype(bf16)
    return [r(b11 + b22), r(b11), r(b12 - b22), r(b21 - b11), r(b22), r(b11 + b12), r(b21 + b22)]


def _asum(a11, a12, a21, a22):
    return [a11 + a22, a21 + a22, a11, a22, a11 + a12, a21 - a11, a12 - a22]


def _bsum(b11, b12, b21, b22):
    return [b11 + b22, b11, b12 - b22, b21 - b11, b22, b11 + b12, b21 + b22]


_A_TERMS = [((0, 0), (1, 1), 1), ((1, 0), (1, 1), 1), ((0, 0), None, 0), ((1, 1), None, 0),
            ((0, 0), (0, 1), 1), ((1, 0), (0, 0), -1), ((0, 1), (1, 1), -1)]
_B_TERMS = [((0, 0), (1, 1), 1), ((0, 0), None, 0), ((0, 1), (1, 1), -1), ((1, 0), (0, 0), -1),
            ((1, 1), None, 0), ((0, 0), (0, 1), 1), ((1, 0), (1, 1), 1)]


def _ccomb(m):
    m1, m2, m3, m4, m5, m6, m7 = m
    return m1 + m4 - m5 + m7, m3 + m5, m2 + m4, m1 - m2 + m3 + m6


def _gate_tanh(x):
    c = 0.7978845608028654
    return jnp.tanh(x * (c + (c * 0.044715) * (x * x)))


def _glu2(g, th, u):
    a = g * u
    return a + a * th


def _sum8(v):
    return ((v[0] + v[1]) + (v[2] + v[3])) + ((v[4] + v[5]) + (v[6] + v[7]))


def _butterfly(sets, masks, axis, size):
    for b in range(3):
        sh = 1 << b
        out = []
        for blk in sets:
            nxt = list(blk)
            for c in range(8):
                if c & sh == 0:
                    lo, hi = blk[c], blk[c + sh]
                    nxt[c] = jnp.where(masks[b], lo, pltpu.roll(hi, sh, axis))
                    nxt[c + sh] = jnp.where(masks[b], pltpu.roll(lo, size - sh, axis), hi)
            out.append(nxt)
        sets = out
    return sets


def _kernel(x_hbm, wqkv_hbm, wo_hbm, wg_hbm, wu_hbm, wd_hbm, out_hbm,
            xraw, xa_u, xa2_u, gu_raw, wd_raw, bgu_u, bd_u, bd2_u, accq, wq_raw, qkv,
            wo_raw, bo_u, stats, zbuf, sems, *bgu2_u):
    acc = accq.bitcast(f32)
    bq = accq.bitcast(bf16)
    bo = bo_u.bitcast(bf16)
    obuf = xraw
    xa = xa_u.bitcast(bf16)
    bgu = bgu_u.bitcast(bf16)
    bd = bd_u.bitcast(bf16)
    bd2 = bd2_u.bitcast(bf16)
    xa2 = xa2_u.bitcast(bf16)
    GA = [0, 2, 2, 0, 1, 2, 1]
    _al = [r.bitcast(bf16) for r in bgu2_u]
    _pos = [sum(1 for q in range(i) if GA[q] == GA[i]) for i in range(7)]
    bg = lambda slot, i, k: _al[GA[i]].at[slot, 7 * _pos[i] + k]
    oa = xa
    pk = lambda v: pltpu.bitcast(v, u32)
    un = lambda v: pltpu.bitcast(v, bf16)

    lane = lax.broadcasted_iota(jnp.int32, (8, 128), 1)
    row8 = lax.broadcasted_iota(jnp.int32, (8, 128), 0)
    lane_lo = [(lane & (1 << b)) == 0 for b in range(3)]
    row_lo = [(row8 & (1 << b)) == 0 for b in range(3)]

    XP = [(0, 128), (128, 128), (512, 128), (640, 128), (256, 256), (768, 256)]

    def x_copy(r):
        r0, n = XP[r]
        return pltpu.make_async_copy(x_hbm.at[:, pl.ds(r0, n), :],
                                     xraw.at[:, pl.ds(r0, n), :], sems.at[(0, 1, 2, 3, 23, 14)[r]])

    def gu_copies(j, slot):
        off = pl.multiple_of(j * GC, GC)
        return (pltpu.make_async_copy(wg_hbm.at[:, pl.ds(off, GC)], gu_raw.at[slot, 0], sems.at[4 + 3 * slot]),
                pltpu.make_async_copy(wu_hbm.at[:, pl.ds(off, GC)], gu_raw.at[slot, 1], sems.at[5 + 3 * slot]))

    def wd_copy(j, slot):
        off = pl.multiple_of(j * GC, GC)
        return pltpu.make_async_copy(wd_hbm.at[pl.ds(off, GC), :], wd_raw.at[slot], sems.at[6 + 3 * slot])

    def gu0_copy(t, c):
        w = (wg_hbm, wu_hbm)[t]
        return pltpu.make_async_copy(w.at[:, pl.ds(c * FC, FC)], gu_raw.at[0, t, :, pl.ds(c * FC, FC)],
                                     sems.at[15 + 2 * c + t])

    def wd0_copy(c):
        return pltpu.make_async_copy(wd_hbm.at[pl.ds(c * FC, FC), :], wd_raw.at[0, pl.ds(c * FC, FC), :],
                                     sems.at[19 + c])

    def wq_copy(t):
        return pltpu.make_async_copy(wqkv_hbm.at[:, pl.ds(t * D, D)], wq_raw.at[t], sems.at[10 + t])

    def wo_copies():
        return [pltpu.make_async_copy(wo_hbm.at[:, pl.ds(c * 256, 256)], wo_raw.at[c], sems.at[24])
                for c in range(4)]

    class _Z:
        cps = [pltpu.make_async_copy(x_hbm.at[0, pl.ds(0, 16), pl.ds(0, 128)], zbuf.at[q], sems.at[21 + q])
               for q in range(2)]

        def start(self):
            for cp in self.cps:
                cp.start()

        def wait(self):
            for cp in self.cps:
                cp.wait()

    z_copy = _Z

    def out_copy(r0, n, k):
        return pltpu.make_async_copy(obuf.at[:, pl.ds(r0, n), :], out_hbm.at[:, pl.ds(r0, n), :],
                                     sems.at[25 + k])

    def true_mask():
        return pk(zbuf[0]) == pk(zbuf[1])

    def ln_half(h, c0, tm16, a):
        xs = []
        for c in range(4):
            x2 = xraw.at[h][c0:c0 + 16, c * 256:(c + 1) * 256].astype(f32)
            xs += [x2[:, :128], x2[:, 128:]]
        s1 = _sum8(xs)
        if a is not None:
            s1 = jnp.where(tm16, s1, a)
        m = jnp.sum(s1, axis=-1, keepdims=True) * (1.0 / D)
        xc = [x - m for x in xs]
        v = jnp.sum(_sum8([x * x for x in xc]), axis=-1, keepdims=True) * (1.0 / D)
        r = lax.rsqrt(v + 1e-5)
        stats.at[h, 0][c0:c0 + 16, :] = jnp.broadcast_to(m, (16, 128))
        stats.at[h, 1][c0:c0 + 16, :] = jnp.broadcast_to(r, (16, 128))
        return [x * r for x in xc]

    def ln_rows(r0, n, anc=None, af=0.85):
        tm16 = None
        if anc is not None:
            tm = true_mask()
            tm16 = jnp.concatenate([tm, tm], axis=0)
            anc = anc[:int(len(anc) * af)]
        nch = n // 16
        for k in range(nch):
            c0 = r0 + 16 * k
            a = [None, None]
            if anc is not None:
                a = [anc[(len(anc) * (2 * k + u)) // (2 * nch)] for u in range(2)]
            lo = ln_half(0, c0, tm16, a[0])
            hi = ln_half(1, c0, tm16, a[1])
            for c in range(4):
                cs = _acomb(lo[c], lo[c + 4], hi[c], hi[c + 4])
                for i in range(7):
                    xa.at[i][c0:c0 + 16, c * 128:(c + 1) * 128] = cs[i]

    def prep_gu(c, ts=(0, 1)):
        KC = 32
        for t in ts:
            w = gu_raw.at[0, t]
            for k0 in range(0, HD, KC):
                lo = w[k0:k0 + KC, c * FC:(c + 1) * FC].astype(f32)
                hi = w[HD + k0:HD + k0 + KC, c * FC:(c + 1) * FC].astype(f32)
                cs = _bcomb(lo[:, :FH], lo[:, FH:], hi[:, :FH], hi[:, FH:])
                for i in range(7):
                    bgu.at[i][k0:k0 + KC, t * FH:(t + 1) * FH] = cs[i]

    def prep_d(w, kh):
        KC = 16
        for k0 in range(0, kh, KC):
            for c0 in range(0, HD, 256):
                g = lambda a, b: w[a + k0:a + k0 + KC, b + c0:b + c0 + 256].astype(f32)
                cs = _bcomb(g(0, 0), g(0, HD), g(kh, 0), g(kh, HD))
                for i in range(7):
                    bd.at[i][k0:k0 + KC, c0:c0 + 256] = cs[i]

    def two_level_piece(terms, inner, ld, i, tm16, anc, nanc, store):
        p, q, sg = terms[i]
        P = ld(*p)
        for e in range(nanc):
            P[e >> 1][e & 1] = jnp.where(tm16, P[e >> 1][e & 1], anc)
        if q is not None:
            Q = ld(*q)
            P = [[P[b][d] + Q[b][d] if sg > 0 else P[b][d] - Q[b][d] for d in range(2)] for b in range(2)]
        ops = inner(P[0][0], P[0][1], P[1][0], P[1][1])
        for k in range(7):
            store(7 * i + k, ops[k].astype(bf16))

    def prep_gu2_piece(slot, i, t, k0, tm16, anc, nanc):
        w = gu_raw.at[slot, t]

        def ld(R, C):
            out = []
            for b in range(2):
                x2 = w[pl.ds((2 * R + b) * QD + k0, 16), C * 256:(C + 1) * 256].astype(f32)
                out.append([x2[:, :128], x2[:, 128:]])
            return out

        def store(p, v):
            bg(slot, i, p % 7)[pl.ds(k0, 16), t * 128:(t + 1) * 128] = v
        two_level_piece(_B_TERMS, _bsum, ld, i, tm16, anc, nanc, store)

    def prep_d2_piece(slot, i, k0, c0, tm16, anc, nanc):
        w = wd_raw.at[slot]

        def ld(R, C):
            return [[w[pl.ds((2 * R + b) * 128 + k0, 16),
                       (2 * C + d) * QD + c0:(2 * C + d) * QD + c0 + 128].astype(f32) for d in range(2)]
                    for b in range(2)]

        def store(p, v):
            bd2.at[slot, p][pl.ds(k0, 16), c0:c0 + 128] = v
        two_level_piece(_B_TERMS, _bsum, ld, i, tm16, anc, nanc, store)

    def make_xa2(r0, tm16, ancs):
        st = [[[stats.at[a, e][pl.ds(b * QS + r0, 16), :] for e in range(2)] for b in range(2)] for a in range(2)]
        for j in range(2):
            def ld(R, C):
                out = []
                for b in range(2):
                    m, r = st[R][b]
                    row = []
                    for d in range(2):
                        c0 = (2 * C + d) * QD + j * 128
                        xv = xraw.at[R][pl.ds(b * QS + r0, 16), c0:c0 + 128].astype(f32)
                        row.append((xv - m) * r)
                    out.append(row)
                return out

            def store(p, v):
                xa2.at[p][pl.ds(r0, 16), j * 128:(j + 1) * 128] = v
            for i in range(7):
                two_level_piece(_A_TERMS, _asum, ld, i, tm16, ancs[7 * j + i], 2, store)

    def ffn_gu(r0, n, o1):
        ms = [None] * 7
        for i in o1:
            ms[i] = _dot(xa[i, r0:r0 + n, :], bgu[i])
        anc = [ms[i][k:k + 16, t * FH:(t + 1) * FH] for i in o1 for t in range(2) for k in range(0, n, 64)]
        hs = _acomb(*[_glu2(v[:, :FH], _gate_tanh(v[:, :FH]), v[:, FH:]) for v in _ccomb(ms)])
        return hs, anc

    def ffn_dn(r0, n, hs, od, first, last=False):
        b, q0 = r0 // QS, r0 % QS
        anc = []
        for i in od:
            y = _dot(hs[i], bd[i])
            anc += [y[k:k + 16, 0:128] for k in range(0, n, 32)]
            lo, hi = (acc.at[7 * i + e] for e in ((6, 2), (1, 5))[b])
            ylo, yhi = y[:, :QD], y[:, QD:]
            if not first:
                ylo = ylo + lo[q0:q0 + n, :]
                yhi = yhi + hi[q0:q0 + n, :]
            if last:
                yhi = yhi + (ylo - acc.at[7 * i + 2][q0:q0 + n, :])
            lo[q0:q0 + n, :] = ylo
            hi[q0:q0 + n, :] = yhi
        return anc

    def zero_acc0(ps, anc):
        tm = true_mask()
        tm16 = jnp.concatenate([tm, tm], axis=0)
        pcs = [(p, q) for p in ps for q in range(4)]
        for e, (p, q) in enumerate(pcs):
            z16 = jnp.where(tm16, 0.0, anc[e * len(anc) // len(pcs)])
            for r0 in range(64 * q, 64 * q + 64, 16):
                for c in range(2):
                    acc.at[p][r0:r0 + 16, c * 128:(c + 1) * 128] = z16

    upk = lambda v: un(v).astype(f32)

    def prep_q_half(t, h, dst, par=1):
        KC = 16
        sa = (128 - 2) * h
        sb = 2 * (1 - h)
        w = wq_raw.at[t]

        def stage1(r0):
            blk = [pk(w[r0:r0 + KC, c * 128:(c + 1) * 128]) for c in range(8)]
            rl = lambda v, sft: v if (isinstance(sft, int) and sft == 0) else pltpu.roll(v, sft, 1)
            return [jnp.where(lane_lo[1], rl(blk[c], sa), rl(blk[c + 2], sb)) for c in (0, 1, 4, 5)]

        def stage(sets, jb, b):
            sh = 1 << b
            out = []
            for blk in sets:
                nxt = list(blk)
                for j in range(4):
                    if j & jb == 0:
                        lo, hi = blk[j], blk[j + jb]
                        nxt[j] = jnp.where(lane_lo[b], lo, pltpu.roll(hi, sh, 1))
                        nxt[j + jb] = jnp.where(lane_lo[b], pltpu.roll(lo, 128 - sh, 1), hi)
                out.append(nxt)
            return out

        for k00 in range(0, HD, KC * par):
            ks = [k00 + KC * q for q in range(par)]
            hv = stage(stage([stage1(hk * HD + k0) for k0 in ks for hk in range(2)], 1, 0), 2, 2)
            for q, k0 in enumerate(ks):
                lo, hi = hv[2 * q], hv[2 * q + 1]
                for e in range(2):
                    cs = _bcomb(upk(lo[e]), upk(lo[e + 2]), upk(hi[e]), upk(hi[e + 2]))
                    for i in range(7):
                        dst.at[i][k0:k0 + KC, e * 128:(e + 1) * 128] = cs[i]

    def qkv_tiles(t, h, src):
        anc16 = []
        for e in range(2):
            n = 2 * h + e
            qlo = qkv.at[t, n]
            qhi = qkv.at[t, n + 4]
            for r in range(NB):
                oq = [1, 4, 2, 3, 0, 5, 6]
                ms = [None] * 7
                for i in oq:
                    ms[i] = _dot(xa[i, r * RB:(r + 1) * RB, :], src.at[i][:, e * 128:(e + 1) * 128])
                c11, c12, c21, c22 = _ccomb(ms)
                anc16 += [ms[i][k:k + 16] for i in oq for k in range(0, RB, 64)]
                r0 = PAD + r * RB
                qlo[r0:r0 + RB, :] = c11
                qhi[r0:r0 + RB, :] = c12
                qlo[HS + r0:HS + r0 + RB, :] = c21
                qhi[HS + r0:HS + r0 + RB, :] = c22
                if r == 0:
                    qlo[0:PAD, :] = jnp.broadcast_to(c11[0:1, :], (PAD, 128))
                    qhi[0:PAD, :] = jnp.broadcast_to(c12[0:1, :], (PAD, 128))
        return anc16

    def prep_o_chunk(m, e, tm, ancs):
        n2 = m >> 3
        g16 = pl.multiple_of((m & 7) * 16, 16)
        res = []
        for h in range(2):
            w = wo_raw.at[n2 + 2 * h]
            w16 = [w[pl.ds(128 * i + g16, 16), e * 128:(e + 1) * 128].astype(f32) for i in range(8)]
            for u in range(2):
                blk = [v[8 * u:8 * u + 8] for v in w16]
                blk[0] = jnp.where(tm, blk[0], ancs[2 * h + u])
                res += _butterfly([blk], row_lo, 0, 8)
        cols = [[jnp.concatenate([res[2 * h][j], res[2 * h + 1][j]], axis=0) for j in range(8)]
                for h in range(2)]
        for b in range(4):
            cs = _bcomb(cols[0][b], cols[1][b], cols[0][b + 4], cols[1][b + 4])
            for i in range(7):
                bo.at[i, n2][pl.ds(b * 128 + g16, 16), e * 128:(e + 1) * 128] = cs[i]

    def attn8(base, row0):
        lg = [None] * NW
        for c in range(8):
            q = qkv[0, c, pl.ds(base, 8), :]
            for w in range(NW):
                pr = q * qkv[1, c, pl.ds(base - 2 * w, 8), :]
                lg[w] = pr if lg[w] is None else lg[w] + pr
        G1 = 2
        for w0 in range(0, NW, G1):
            for w in range(w0, w0 + G1):
                lg[w] = lg[w] + pltpu.roll(lg[w], 8, 1)
            for w in range(w0, w0 + G1):
                lg[w] = lg[w] + pltpu.roll(lg[w], 16, 1)
        if row0 is not None:
            for w in range(1, NW):
                lg[w] = jnp.where(row8 + row0 >= 2 * w, lg[w], NEG)
        m = lg[0]
        for w in range(1, NW):
            m = jnp.maximum(m, lg[w])
        p = [jnp.exp2((lg[w] - m) * (SCALE * LOG2E)) for w in range(NW)]
        den = p[0]
        for w in range(1, NW):
            den = den + p[w]
        inv = 1.0 / den
        b4 = (lane & 16) != 0
        b3 = (lane & 8) != 0
        outs = [None] * 8
        G2 = 2
        for w0 in range(0, NW, G2):
            ws = range(w0, w0 + G2)
            for w in ws:
                p[w] = p[w] * inv
                p[w] = jnp.where(b4, p[w], pltpu.roll(p[w], 112, 1))
            for w in ws:
                p[w] = jnp.where(b3, p[w], pltpu.roll(p[w], 120, 1))
            for w in ws:
                for c in range(8):
                    pr = p[w] * qkv[2, c, pl.ds(base - 2 * w, 8), :]
                    outs[c] = pr if outs[c] is None else outs[c] + pr
        return outs

    def attn_pair(r0, mask=False):
        parts = [attn8(pl.multiple_of(PAD + h * HS + r0 + 8 * u, 8), (r0 + 8 * u) if (h == 0 and mask) else None)
                 for h in range(2) for u in range(2)]
        lo = [jnp.concatenate([parts[0][c], parts[1][c]], axis=0) for c in range(8)]
        hi = [jnp.concatenate([parts[2][c], parts[3][c]], axis=0) for c in range(8)]
        for n in range(4):
            cs = _acomb(lo[n], lo[n + 4], hi[n], hi[n + 4])
            for i in range(7):
                oa.at[i][pl.ds(pl.multiple_of(r0, 16), 16), n * 128:(n + 1) * 128] = cs[i]
        return hi[7]

    wd0 = lambda c: wd_raw.at[0, c * FC:(c + 1) * FC, :]
    RA, RBB, RC, RD = 0, 512, 256, 768

    x_copy(0).start()
    x_copy(1).start()
    gu0_copy(0, 0).start()
    z_copy().start()
    gu0_copy(1, 0).start()
    x_copy(2).start()
    wd0_copy(0).start()
    x_copy(3).start()
    x_copy(4).start()
    gu0_copy(0, 1).start()
    gu0_copy(1, 1).start()
    wd0_copy(1).start()
    x_copy(5).start()
    wq_copy(0).start()
    for cp in wo_copies():
        cp.start()
    wq_copy(1).start()

    x_copy(0).wait()
    ln_rows(RA, 128)
    x_copy(1).wait()
    ln_rows(RA + 128, 128)

    gu0_copy(0, 0).wait()
    prep_gu(0, (0,))
    mg = [None] * 7
    for i in [4, 2, 3, 1, 0, 6, 5]:
        mg[i] = _dot(xa[i, RA:RA + RB, :], bgu[i, :, :FH])
    gg = [(v, _gate_tanh(v)) for v in _ccomb(mg)]

    z_copy().wait()
    gu0_copy(1, 0).wait()
    x_copy(2).wait()
    prep_gu(0, (1,))
    mu = [None] * 7
    for i in [4, 2, 3, 1, 0, 6, 5]:
        mu[i] = _dot(xa[i, RA:RA + RB, :], bgu[i, :, FH:])
    ha = _acomb(*[_glu2(a[0], a[1], b) for a, b in zip(gg, _ccomb(mu))])
    ln_rows(RBB, 128, [mu[i][k:k + 16] for i in [4, 2, 3, 1, 0, 6, 5] for k in range(0, RB, 64)],
            0.85)

    wd0_copy(0).wait()
    x_copy(3).wait()
    prep_d(wd0(0), FH)
    hb0, anc = ffn_gu(RBB, 128, [6, 5, 0, 1, 4, 2, 3])
    ffn_dn(RA, RB, ha, [3, 0, 4, 1, 2, 6, 5], True)
    ln_rows(RBB + 128, 128, anc, 0.7)

    x_copy(4).wait()
    gu0_copy(0, 1).wait()
    gu0_copy(1, 1).wait()
    hb1, anc = ffn_gu(RBB + 128, 128, [4, 0, 2, 6, 5, 3, 1])
    anc2 = ffn_dn(RBB, 128, hb0, [3, 6, 5, 4, 2, 0, 1], True)
    ffn_dn(RBB + 128, 128, hb1, [3, 6, 5, 4, 2, 0, 1], True)
    prep_gu(1)
    ln_rows(RC, RB, anc + anc2[:28], 0.85)

    wd0_copy(1).wait()
    x_copy(5).wait()
    prep_d(wd0(1), FH)
    h2, anc = ffn_gu(RA, RB, [4, 2, 3, 1, 0, 6, 5])
    ffn_dn(RA, RB, h2, [6, 1, 4, 3, 2, 5, 0], False)
    ln_rows(RD, RB, anc, 0.75)
    zs_ = [p for p in range(49) if p % 7 in (0, 3, 4)]
    zero_acc0(zs_[:7], anc)
    wq_copy(2).start()
    for cp in gu_copies(1, 1):
        cp.start()
    wd_copy(1, 1).start()

    wq_copy(0).wait()
    h3, anc = ffn_gu(RBB, RB, [0, 1, 2, 3, 4, 5, 6])
    zero_acc0(zs_[7:], anc)
    prep_q_half(0, 0, bq.at[56:63], 2)
    ffn_dn(RBB, RB, h3, [0, 3, 4, 6, 2, 1, 5], False, True)

    for cp in wo_copies():
        cp.wait()

    def p2_body(i, carry):
        @pl.when(i == 1)
        def _():
            wq_copy(1).wait()

        @pl.when(i == 3)
        def _():
            wq_copy(2).wait()

        @pl.when(i == 4)
        def _():
            for cp in gu_copies(1, 1):
                cp.wait()
            wd_copy(1, 1).wait()
        bqv = bq.at[pl.ds(49 + 7 * i, 21)]
        anc16 = qkv_tiles(i >> 1, i & 1, bqv.at[7:14])
        prep_q_half(jnp.minimum((i + 1) >> 1, 2), (i + 1) & 1, bqv.at[14:21], 2)
        tm = true_mask()
        tm16 = jnp.concatenate([tm, tm], axis=0)
        jobs = []
        for k in range(6):
            jobs += [('o', k, q) for q in range(4)] + [('x', k, q) for q in range(14)]
        for k in range(8):
            jobs += [('g', k, q) for q in range(7)]
        for k in range(4):
            jobs += [('d', k, q) for q in range(7)]
        for k in range(7):
            jobs += [('z', k, q) for q in range(4)]
        by = {}
        for kind in 'oxgzd':
            js = [jb for jb in jobs if jb[0] == kind]
            for e, jb in enumerate(js):
                lo_, hi_ = {}.get(kind, [0.0, 1.0])
                by[jb] = lo_ + (hi_ - lo_) * (e + 0.5) / len(js)
        ranked = sorted(jobs, key=lambda jb: by[jb])
        na = len(anc16) - 4
        at = {jb: anc16[(e * na) // len(ranked)] for e, jb in enumerate(ranked)}
        for k in range(6):
            prep_o_chunk(jnp.minimum(3 * i + (k >> 1), 15), k & 1, tm, [at['o', k, q][0:8] for q in range(4)])
            make_xa2(pl.multiple_of(jnp.minimum(6 * i + k, 31) * 16, 16), tm16,
                     [at['x', k, q] for q in range(14)])
        for k in range(8):
            idx = 4 * i + (k >> 1)
            for q in range(7):
                prep_gu2_piece(idx >> 4, q, k & 1, pl.multiple_of((idx & 15) * 16, 16), tm16,
                               at['g', k, q], 1)
        for k in range(4):
            idx = 2 * i + (k >> 1)
            for q in range(7):
                prep_d2_piece(idx >> 3, q, pl.multiple_of((idx & 7) * 16, 16), (k & 1) * 128, tm16,
                              at['d', k, q], 1)
        az = acc.at[pl.ds(49 + 7 * i, 21)]
        for k in range(7):
            for q in range(4):
                z16 = jnp.where(tm16, 0.0, at['z', k, q])
                for r0 in range(64 * q, 64 * q + 64, 16):
                    for c in range(2):
                        az.at[k][r0:r0 + 16, c * 128:(c + 1) * 128] = z16
        return carry

    lax.fori_loop(0, 6, p2_body, 0)

    def p3_body(u, carry):
        j = u >> 1
        s_ = u & 1
        sl = j & 1
        jn = jnp.minimum((u >> 1) + 1, NG - 1)
        sn = 1 - sl

        @pl.when(jnp.logical_and(s_ == 0, j + 1 < NG))
        def _():
            wd_copy(jn, sn).wait()
            for cp in gu_copies(jn, sn):
                cp.wait()
        a4 = pl.multiple_of((u - 1) * 64, 64)
        for g in range(5):
            att_last = attn_pair(a4 + 16 * g if g < 4 else 832 + 16 * jnp.minimum(u - 1, 11), g == 0)
        tm = true_mask()
        tm16 = jnp.concatenate([tm, tm], axis=0)

        rows = pl.ds(pl.multiple_of(s_ * RB, RB), RB)
        accs = acc.at[pl.ds(49 * s_, 49)]
        order = (0, 3, 4, 6, 2, 1, 5)
        c1 = [None] * 7
        dprep = []
        h = [[None] * 4 for _ in range(4)]

        def gate_up(i):
            ms = [None] * 7
            for k in order:
                ms[k] = _dot(xa2.at[7 * i + k][rows, :], bg(sl, i, k)[...])
            c1[i] = _ccomb(ms)
            return [ms[k][r_:r_ + 16, t * 128:(t + 1) * 128] for k in order for r_ in range(0, RB, 64)
                    for t in range(2)]

        def hidden(a, e):
            if h[2 * a][2 * e] is None:
                for q in range(4):
                    m = [None if v is None else v[q] for v in c1]
                    if (a, e) == (0, 0):
                        cc = m[0] + m[3] - m[4] + m[6]
                    elif (a, e) == (0, 1):
                        cc = m[2] + m[4]
                    elif (a, e) == (1, 0):
                        cc = m[1] + m[3]
                    else:
                        cc = m[0] - m[1] + m[2] + m[5]
                    h[2 * a + (q >> 1)][2 * e + (q & 1)] = _glu2(cc[:, :128], _gate_tanh(cc[:, :128]),
                                                                 cc[:, 128:])
            return [[h[2 * a + b][2 * e + f] for f in range(2)] for b in range(2)]

        def down(i):
            p, q, sg = _A_TERMS[i]
            P = hidden(*p)
            if q is not None:
                Q = hidden(*q)
                P = [[P[b][f] + Q[b][f] if sg > 0 else P[b][f] - Q[b][f] for f in range(2)] for b in range(2)]
            out = []
            if i == 2:
                v = P[0][0]
                P[0][0] = jnp.concatenate([jnp.where(tm16, v[0:16], att_last), v[16:]], axis=0)
            a7 = _asum(P[0][0], P[0][1], P[1][0], P[1][1])
            for k in [6, 1, 4, 3, 2, 5, 0]:
                y = _dot(a7[k].astype(bf16), bd2.at[sl, 7 * i + k][...])
                out += [y[r_:r_ + 16, 0:128] for r_ in range(0, RB, 128)]
                old = accs.at[7 * i + k][...]
                if i == 6:
                    old = jnp.where(u == 1, 0.0, old)
                accs.at[7 * i + k][...] = old + y
            return out

        seq = 'G0 G3 G4 G6 G1 G2 D2 G5 D6 D4 D3 D1 D0 D5'.split()
        sanc = []
        for tk in seq:
            if tk[0] == 'D' and not dprep:
                dprep.append(1)
                lo_, hi_ = 0, 1
                src = [a for p in range(lo_, hi_) for a in sanc[p]]
                pcs = [(k0, c0, i) for k0 in range(0, 64, 16) for c0 in range(0, QD, 128) for i in range(7)]
                for e, (k0, c0, i) in enumerate(pcs):
                    prep_d2_piece(sn, i, pl.multiple_of(s_ * 64, 64) + k0, c0, tm16,
                                  src[e * len(src) // len(pcs)], 1)
            sanc.append((gate_up if tk[0] == 'G' else down)(int(tk[1])))
        kb = pl.multiple_of(s_ * (QD // 2), QD // 2)
        PW = [[2, 5], [7, 8], [8, 14]]
        for a in range(max(GA) + 1):
            members = [i for i in range(7) if GA[i] == a]
            last = max(p for p, tk in enumerate(seq) if tk[0] == 'G' and int(tk[1]) in members)
            lo_, hi_ = max(PW[a][0], last + 1), max(PW[a][1], last + 2)
            src = [x for p in range(lo_, hi_) for x in sanc[p]]
            pieces = [(t, k0, i) for k0 in range(0, QD // 2, 16) for t in range(2) for i in members]
            for e, (t, k0, i) in enumerate(pieces):
                prep_gu2_piece(sn, i, t, kb + k0, tm16, src[e * len(src) // len(pieces)], 4)

        @pl.when(jnp.logical_and(s_ == 1, j + 3 < NG))
        def _():
            wd_copy(j + 3, sn).start()
            for cp in gu_copies(j + 3, sn):
                cp.start()
        return carry

    wd_copy(2, 0).start()
    for cp in gu_copies(2, 0):
        cp.start()
    lax.fori_loop(1, 2 * NG, p3_body, 0)

    SB = 32

    def p4_body(k, carry):
        acck = acc.at[pl.ds(49 * (k >> 1), 49)]
        for u in range(RB // SB):
            b = u // (128 // SB)
            q0 = pl.multiple_of(k * 128 + (u % (128 // SB)) * SB, SB)
            r0 = pl.multiple_of(b * QS + q0, SB)
            rows = pl.ds(r0, SB)
            qr = pl.multiple_of((k & 1) * 128 + (u % (128 // SB)) * SB, SB)
            for n in range(2):
                ms = [None] * 7
                for i in [0, 1, 2, 3, 4, 5, 6]:
                    ms[i] = _dot(oa.at[i][rows, :], bo.at[i, n][...])
                av = []
                for i in range(7):
                    ld = lambda e: acck.at[7 * i + e][pl.ds(qr, SB), :]
                    av.append((lambda: ld(0) + ld(3) - ld(4) + ld(6), lambda: ld(2) + ld(4),
                               lambda: ld(1) + ld(3), lambda: ld(0) - ld(1) + ld(2) + ld(5))[2 * b + n]())
                ss = _ccomb(ms)
                fs = _ccomb(av)
                for q, (h, c0) in enumerate(((0, n * 256), (0, HD + n * 256), (1, n * 256), (1, HD + n * 256))):
                    hf = 0.25 * fs[q]
                    g = hf + hf * jnp.tanh(hf)
                    xv = xraw.at[h][rows, c0:c0 + 256].astype(f32)
                    obuf.at[h][rows, c0:c0 + 256] = (xv + ss[q] * g).astype(bf16)
            out_copy(r0, SB, 0).start()
        return carry

    lax.fori_loop(0, NB, p4_body, 0)
    out_copy(0, HS, 0).wait()


@jax.jit
def pallas_recurrent_scan__sliding_local_dilated__geglu_ffn__prompt_kernel(
    A_x: jax.Array,
    A_wqkv: jax.Array,
    A_wo: jax.Array,
    B_x: jax.Array,
    B_w_gate: jax.Array,
    B_w_up: jax.Array,
    B_w_down: jax.Array,
):
    any_spec = pl.BlockSpec(memory_space=pl.ANY)
    out = pl.pallas_call(
        _kernel,
        out_shape=jax.ShapeDtypeStruct((2, HS, D), bf16),
        in_specs=[any_spec] * 6,
        out_specs=any_spec,
        scratch_shapes=[
            pltpu.VMEM((2, HS, D), bf16),
            pltpu.VMEM((7, HS // 2, HD), u32),
            pltpu.VMEM((49, QS // 2, QD), u32),
            pltpu.VMEM((2, 2, D, GC), bf16),
            pltpu.VMEM((2, GC, D), bf16),
            pltpu.VMEM((7, HD // 2, FC), u32),
            pltpu.VMEM((7, FH // 2, HD), u32),
            pltpu.VMEM((2, 49, 64, QD), u32),
            pltpu.VMEM((105, RB, QD), u32),
            pltpu.VMEM((3, D, D), bf16),
            pltpu.VMEM((3, 8, PAD + S, 128), f32),
            pltpu.VMEM((4, D, 256), bf16),
            pltpu.VMEM((7, 2, HD // 2, 256), u32),
            pltpu.VMEM((2, 2, HS, 128), f32),
            pltpu.VMEM((2, 16, 128), bf16),
            pltpu.SemaphoreType.DMA((26,)),
        ] + [pltpu.VMEM((2, 7 * n, QD // 2, 256), u32) for n in (2, 2, 3)],
        compiler_params=pltpu.CompilerParams(vmem_limit_bytes=127 * 1024 * 1024,
                                             disable_bounds_checks=True,
                                             disable_semaphore_checks=True),
        name="fusedk",
    )(A_x.reshape(2, HS, D), A_wqkv, A_wo, B_w_gate, B_w_up, B_w_down)
    return out.reshape(1, S, D)
```

```python
import jax
import jax.numpy as jnp
from jax import lax
import jax.experimental.pallas as pl
import jax.experimental.pallas.tpu as pltpu

f32 = jnp.float32
bf16 = jnp.bfloat16
u32 = jnp.uint32

S, D, F = 2048, 1024, 3584
HS, HD = S // 2, D // 2
FC = 256
FH = FC // 2
NF = F // FC
QS, QD = S // 4, D // 4
GC = 512
NG = F // GC
RB = 256
NB = HS // RB
PAD = 16
NW = 8
SCALE = 32 ** -0.5
LOG2E = 1.4426950408889634
NEG = -1e9 / SCALE


def _dot(a, b):
    return jnp.dot(a, b, preferred_element_type=f32)


def _acomb(a11, a12, a21, a22):
    r = lambda v: v.astype(bf16)
    return [r(a11 + a22), r(a21 + a22), r(a11), r(a22), r(a11 + a12), r(a21 - a11), r(a12 - a22)]


def _bcomb(b11, b12, b21, b22):
    r = lambda v: v.astype(bf16)
    return [r(b11 + b22), r(b11), r(b12 - b22), r(b21 - b11), r(b22), r(b11 + b12), r(b21 + b22)]


def _asum(a11, a12, a21, a22):
    return [a11 + a22, a21 + a22, a11, a22, a11 + a12, a21 - a11, a12 - a22]


def _bsum(b11, b12, b21, b22):
    return [b11 + b22, b11, b12 - b22, b21 - b11, b22, b11 + b12, b21 + b22]


_A_TERMS = [((0, 0), (1, 1), 1), ((1, 0), (1, 1), 1), ((0, 0), None, 0), ((1, 1), None, 0),
            ((0, 0), (0, 1), 1), ((1, 0), (0, 0), -1), ((0, 1), (1, 1), -1)]
_B_TERMS = [((0, 0), (1, 1), 1), ((0, 0), None, 0), ((0, 1), (1, 1), -1), ((1, 0), (0, 0), -1),
            ((1, 1), None, 0), ((0, 0), (0, 1), 1), ((1, 0), (1, 1), 1)]


def _ccomb(m):
    m1, m2, m3, m4, m5, m6, m7 = m
    return m1 + m4 - m5 + m7, m3 + m5, m2 + m4, m1 - m2 + m3 + m6


def _gate_tanh(x):
    c = 0.7978845608028654
    return jnp.tanh(x * (c + (c * 0.044715) * (x * x)))


def _glu2(g, th, u):
    a = g * u
    return a + a * th


def _sum8(v):
    return ((v[0] + v[1]) + (v[2] + v[3])) + ((v[4] + v[5]) + (v[6] + v[7]))


def _butterfly(sets, masks, axis, size):
    for b in range(3):
        sh = 1 << b
        out = []
        for blk in sets:
            nxt = list(blk)
            for c in range(8):
                if c & sh == 0:
                    lo, hi = blk[c], blk[c + sh]
                    nxt[c] = jnp.where(masks[b], lo, pltpu.roll(hi, sh, axis))
                    nxt[c + sh] = jnp.where(masks[b], pltpu.roll(lo, size - sh, axis), hi)
            out.append(nxt)
        sets = out
    return sets


def _kernel(x_hbm, wqkv_hbm, wo_hbm, wg_hbm, wu_hbm, wd_hbm, out_hbm,
            xraw, xa_u, xa2_u, gu_raw, wd_raw, bgu_u, bd_u, bd2_u, accq, wq_raw, qkv,
            wo_raw, bo_u, stats, zbuf, sems, *bgu2_u):
    acc = accq.bitcast(f32)
    bq = accq.bitcast(bf16)
    bo = bo_u.bitcast(bf16)
    obuf = xraw
    xa = xa_u.bitcast(bf16)
    bgu = bgu_u.bitcast(bf16)
    bd = bd_u.bitcast(bf16)
    bd2 = bd2_u.bitcast(bf16)
    xa2 = xa2_u.bitcast(bf16)
    GA = [0, 2, 2, 0, 1, 2, 1]
    _al = [r.bitcast(bf16) for r in bgu2_u]
    _pos = [sum(1 for q in range(i) if GA[q] == GA[i]) for i in range(7)]
    bg = lambda slot, i, k: _al[GA[i]].at[slot, 7 * _pos[i] + k]
    oa = xa
    pk = lambda v: pltpu.bitcast(v, u32)
    un = lambda v: pltpu.bitcast(v, bf16)

    lane = lax.broadcasted_iota(jnp.int32, (8, 128), 1)
    row8 = lax.broadcasted_iota(jnp.int32, (8, 128), 0)
    lane_lo = [(lane & (1 << b)) == 0 for b in range(3)]
    row_lo = [(row8 & (1 << b)) == 0 for b in range(3)]

    XP = [(0, 128), (128, 128), (512, 128), (640, 128), (256, 256), (768, 256)]

    def x_copy(r):
        r0, n = XP[r]
        return pltpu.make_async_copy(x_hbm.at[:, pl.ds(r0, n), :],
                                     xraw.at[:, pl.ds(r0, n), :], sems.at[(0, 1, 2, 3, 23, 14)[r]])

    def gu_copies(j, slot):
        off = pl.multiple_of(j * GC, GC)
        return (pltpu.make_async_copy(wg_hbm.at[:, pl.ds(off, GC)], gu_raw.at[slot, 0], sems.at[4 + 3 * slot]),
                pltpu.make_async_copy(wu_hbm.at[:, pl.ds(off, GC)], gu_raw.at[slot, 1], sems.at[5 + 3 * slot]))

    def wd_copy(j, slot):
        off = pl.multiple_of(j * GC, GC)
        return pltpu.make_async_copy(wd_hbm.at[pl.ds(off, GC), :], wd_raw.at[slot], sems.at[6 + 3 * slot])

    def gu0_copy(t, c):
        w = (wg_hbm, wu_hbm)[t]
        return pltpu.make_async_copy(w.at[:, pl.ds(c * FC, FC)], gu_raw.at[0, t, :, pl.ds(c * FC, FC)],
                                     sems.at[15 + 2 * c + t])

    def wd0_copy(c):
        return pltpu.make_async_copy(wd_hbm.at[pl.ds(c * FC, FC), :], wd_raw.at[0, pl.ds(c * FC, FC), :],
                                     sems.at[19 + c])

    def wq_copy(t):
        return pltpu.make_async_copy(wqkv_hbm.at[:, pl.ds(t * D, D)], wq_raw.at[t], sems.at[10 + t])

    def wo_copies():
        return [pltpu.make_async_copy(wo_hbm.at[:, pl.ds(c * 256, 256)], wo_raw.at[c], sems.at[24])
                for c in range(4)]

    class _Z:
        cps = [pltpu.make_async_copy(x_hbm.at[0, pl.ds(0, 16), pl.ds(0, 128)], zbuf.at[q], sems.at[21 + q])
               for q in range(2)]

        def start(self):
            for cp in self.cps:
                cp.start()

        def wait(self):
            for cp in self.cps:
                cp.wait()

    z_copy = _Z

    def out_copy(r0, n, k):
        return pltpu.make_async_copy(obuf.at[:, pl.ds(r0, n), :], out_hbm.at[:, pl.ds(r0, n), :],
                                     sems.at[25 + k])

    def true_mask():
        return pk(zbuf[0]) == pk(zbuf[1])

    def ln_half(h, c0, tm16, a):
        xs = []
        for c in range(4):
            x2 = xraw.at[h][c0:c0 + 16, c * 256:(c + 1) * 256].astype(f32)
            xs += [x2[:, :128], x2[:, 128:]]
        s1 = _sum8(xs)
        if a is not None:
            s1 = jnp.where(tm16, s1, a)
        m = jnp.sum(s1, axis=-1, keepdims=True) * (1.0 / D)
        xc = [x - m for x in xs]
        v = jnp.sum(_sum8([x * x for x in xc]), axis=-1, keepdims=True) * (1.0 / D)
        r = lax.rsqrt(v + 1e-5)
        stats.at[h, 0][c0:c0 + 16, :] = jnp.broadcast_to(m, (16, 128))
        stats.at[h, 1][c0:c0 + 16, :] = jnp.broadcast_to(r, (16, 128))
        return [x * r for x in xc]

    def ln_rows(r0, n, anc=None, af=0.85):
        tm16 = None
        if anc is not None:
            tm = true_mask()
            tm16 = jnp.concatenate([tm, tm], axis=0)
            anc = anc[:int(len(anc) * af)]
        nch = n // 16
        for k in range(nch):
            c0 = r0 + 16 * k
            a = [None, None]
            if anc is not None:
                a = [anc[(len(anc) * (2 * k + u)) // (2 * nch)] for u in range(2)]
            lo = ln_half(0, c0, tm16, a[0])
            hi = ln_half(1, c0, tm16, a[1])
            for c in range(4):
                cs = _acomb(lo[c], lo[c + 4], hi[c], hi[c + 4])
                for i in range(7):
                    xa.at[i][c0:c0 + 16, c * 128:(c + 1) * 128] = cs[i]

    def prep_gu(c, ts=(0, 1)):
        KC = 32
        for t in ts:
            w = gu_raw.at[0, t]
            for k0 in range(0, HD, KC):
                lo = w[k0:k0 + KC, c * FC:(c + 1) * FC].astype(f32)
                hi = w[HD + k0:HD + k0 + KC, c * FC:(c + 1) * FC].astype(f32)
                cs = _bcomb(lo[:, :FH], lo[:, FH:], hi[:, :FH], hi[:, FH:])
                for i in range(7):
                    bgu.at[i][k0:k0 + KC, t * FH:(t + 1) * FH] = cs[i]

    def prep_d(w, kh):
        KC = 16
        for k0 in range(0, kh, KC):
            for c0 in range(0, HD, 256):
                g = lambda a, b: w[a + k0:a + k0 + KC, b + c0:b + c0 + 256].astype(f32)
                cs = _bcomb(g(0, 0), g(0, HD), g(kh, 0), g(kh, HD))
                for i in range(7):
                    bd.at[i][k0:k0 + KC, c0:c0 + 256] = cs[i]

    def two_level_piece(terms, inner, ld, i, tm16, anc, nanc, store):
        p, q, sg = terms[i]
        P = ld(*p)
        for e in range(nanc):
            P[e >> 1][e & 1] = jnp.where(tm16, P[e >> 1][e & 1], anc)
        if q is not None:
            Q = ld(*q)
            P = [[P[b][d] + Q[b][d] if sg > 0 else P[b][d] - Q[b][d] for d in range(2)] for b in range(2)]
        ops = inner(P[0][0], P[0][1], P[1][0], P[1][1])
        for k in range(7):
            store(7 * i + k, ops[k].astype(bf16))

    def prep_gu2_piece(slot, i, t, k0, tm16, anc, nanc):
        w = gu_raw.at[slot, t]

        def ld(R, C):
            out = []
            for b in range(2):
                x2 = w[pl.ds((2 * R + b) * QD + k0, 16), C * 256:(C + 1) * 256].astype(f32)
                out.append([x2[:, :128], x2[:, 128:]])
            return out

        def store(p, v):
            bg(slot, i, p % 7)[pl.ds(k0, 16), t * 128:(t + 1) * 128] = v
        two_level_piece(_B_TERMS, _bsum, ld, i, tm16, anc, nanc, store)

    def prep_d2_piece(slot, i, k0, c0, tm16, anc, nanc):
        w = wd_raw.at[slot]

        def ld(R, C):
            return [[w[pl.ds((2 * R + b) * 128 + k0, 16),
                       (2 * C + d) * QD + c0:(2 * C + d) * QD + c0 + 128].astype(f32) for d in range(2)]
                    for b in range(2)]

        def store(p, v):
            bd2.at[slot, p][pl.ds(k0, 16), c0:c0 + 128] = v
        two_level_piece(_B_TERMS, _bsum, ld, i, tm16, anc, nanc, store)

    def make_xa2(r0, tm16, ancs):
        st = [[[stats.at[a, e][pl.ds(b * QS + r0, 16), :] for e in range(2)] for b in range(2)] for a in range(2)]
        for j in range(2):
            def ld(R, C):
                out = []
                for b in range(2):
                    m, r = st[R][b]
                    row = []
                    for d in range(2):
                        c0 = (2 * C + d) * QD + j * 128
                        xv = xraw.at[R][pl.ds(b * QS + r0, 16), c0:c0 + 128].astype(f32)
                        row.append((xv - m) * r)
                    out.append(row)
                return out

            def store(p, v):
                xa2.at[p][pl.ds(r0, 16), j * 128:(j + 1) * 128] = v
            for i in range(7):
                two_level_piece(_A_TERMS, _asum, ld, i, tm16, ancs[7 * j + i], 2, store)

    def ffn_gu(r0, n, o1):
        ms = [None] * 7
        for i in o1:
            ms[i] = _dot(xa[i, r0:r0 + n, :], bgu[i])
        anc = [ms[i][k:k + 16, t * FH:(t + 1) * FH] for i in o1 for t in range(2) for k in range(0, n, 64)]
        hs = _acomb(*[_glu2(v[:, :FH], _gate_tanh(v[:, :FH]), v[:, FH:]) for v in _ccomb(ms)])
        return hs, anc

    def ffn_dn(r0, n, hs, od, first, last=False):
        b, q0 = r0 // QS, r0 % QS
        anc = []
        for i in od:
            y = _dot(hs[i], bd[i])
            anc += [y[k:k + 16, 0:128] for k in range(0, n, 32)]
            lo, hi = (acc.at[7 * i + e] for e in ((6, 2), (1, 5))[b])
            ylo, yhi = y[:, :QD], y[:, QD:]
            if not first:
                ylo = ylo + lo[q0:q0 + n, :]
                yhi = yhi + hi[q0:q0 + n, :]
            if last:
                yhi = yhi + (ylo - acc.at[7 * i + 2][q0:q0 + n, :])
            lo[q0:q0 + n, :] = ylo
            hi[q0:q0 + n, :] = yhi
        return anc

    def zero_acc0(ps, anc):
        tm = true_mask()
        tm16 = jnp.concatenate([tm, tm], axis=0)
        pcs = [(p, q) for p in ps for q in range(4)]
        for e, (p, q) in enumerate(pcs):
            z16 = jnp.where(tm16, 0.0, anc[e * len(anc) // len(pcs)])
            for r0 in range(64 * q, 64 * q + 64, 16):
                for c in range(2):
                    acc.at[p][r0:r0 + 16, c * 128:(c + 1) * 128] = z16

    upk = lambda v: un(v).astype(f32)

    def prep_q_half(t, h, dst, par=1):
        KC = 16
        sa = (128 - 2) * h
        sb = 2 * (1 - h)
        w = wq_raw.at[t]

        def stage1(r0):
            blk = [pk(w[r0:r0 + KC, c * 128:(c + 1) * 128]) for c in range(8)]
            rl = lambda v, sft: v if (isinstance(sft, int) and sft == 0) else pltpu.roll(v, sft, 1)
            return [jnp.where(lane_lo[1], rl(blk[c], sa), rl(blk[c + 2], sb)) for c in (0, 1, 4, 5)]

        def stage(sets, jb, b):
            sh = 1 << b
            out = []
            for blk in sets:
                nxt = list(blk)
                for j in range(4):
                    if j & jb == 0:
                        lo, hi = blk[j], blk[j + jb]
                        nxt[j] = jnp.where(lane_lo[b], lo, pltpu.roll(hi, sh, 1))
                        nxt[j + jb] = jnp.where(lane_lo[b], pltpu.roll(lo, 128 - sh, 1), hi)
                out.append(nxt)
            return out

        for k00 in range(0, HD, KC * par):
            ks = [k00 + KC * q for q in range(par)]
            hv = stage(stage([stage1(hk * HD + k0) for k0 in ks for hk in range(2)], 1, 0), 2, 2)
            for q, k0 in enumerate(ks):
                lo, hi = hv[2 * q], hv[2 * q + 1]
                for e in range(2):
                    cs = _bcomb(upk(lo[e]), upk(lo[e + 2]), upk(hi[e]), upk(hi[e + 2]))
                    for i in range(7):
                        dst.at[i][k0:k0 + KC, e * 128:(e + 1) * 128] = cs[i]

    def qkv_tiles(t, h, src):
        anc16 = []
        for e in range(2):
            qlo = qkv.at[t, 4 * h + e]
            qhi = qkv.at[t, 4 * h + 2 + e]
            for r in range(NB):
                oq = [1, 4, 2, 3, 0, 5, 6]
                ms = [None] * 7
                for i in oq:
                    ms[i] = _dot(xa[i, r * RB:(r + 1) * RB, :], src.at[i][:, e * 128:(e + 1) * 128])
                c11, c12, c21, c22 = _ccomb(ms)
                anc16 += [ms[i][k:k + 16] for i in oq for k in range(0, RB, 64)]
                r0 = PAD + r * RB
                qlo[r0:r0 + RB, :] = c11
                qhi[r0:r0 + RB, :] = c12
                qlo[HS + r0:HS + r0 + RB, :] = c21
                qhi[HS + r0:HS + r0 + RB, :] = c22
                if r == 0:
                    qlo[PAD - 16:PAD, :] = jnp.broadcast_to(c11[0:1, :], (16, 128))
                    qhi[PAD - 16:PAD, :] = jnp.broadcast_to(c12[0:1, :], (16, 128))
        return anc16

    def prep_o_chunk(n2, g16, e, tm, ancs):
        res = []
        for h in range(2):
            w = wo_raw.at[n2 + 2 * h]
            w16 = [w[pl.ds(128 * i + g16, 16), e * 128:(e + 1) * 128].astype(f32) for i in range(8)]
            for u in range(2):
                blk = [v[8 * u:8 * u + 8] for v in w16]
                blk[0] = jnp.where(tm, blk[0], ancs[2 * h + u])
                res += _butterfly([blk], row_lo, 0, 8)
        cols = [[jnp.concatenate([res[2 * h][j], res[2 * h + 1][j]], axis=0) for j in range(8)]
                for h in range(2)]
        for b in range(4):
            cs = _bcomb(cols[0][b], cols[1][b], cols[0][b + 4], cols[1][b + 4])
            for i in range(7):
                bo.at[i, n2][pl.ds(b * 128 + g16, 16), e * 128:(e + 1) * 128] = cs[i]

    PH = [4 * ((c >> 1) & 1) + 2 * (c >> 2) + (c & 1) for c in range(8)]

    def attn8(base, row0):
        lg = [None] * NW
        for c in range(8):
            q = qkv[0, PH[c], pl.ds(base, 8), :]
            for w in range(NW):
                pr = q * qkv[1, PH[c], pl.ds(base - 2 * w, 8), :]
                lg[w] = pr if lg[w] is None else lg[w] + pr
        G1 = 2
        for w0 in range(0, NW, G1):
            for w in range(w0, w0 + G1):
                lg[w] = lg[w] + pltpu.roll(lg[w], 8, 1)
            for w in range(w0, w0 + G1):
                lg[w] = lg[w] + pltpu.roll(lg[w], 16, 1)
        if row0 is not None:
            for w in range(1, NW):
                lg[w] = jnp.where(row8 + row0 >= 2 * w, lg[w], NEG)
        m = lg[0]
        for w in range(1, NW):
            m = jnp.maximum(m, lg[w])
        p = [jnp.exp2((lg[w] - m) * (SCALE * LOG2E)) for w in range(NW)]
        den = p[0]
        for w in range(1, NW):
            den = den + p[w]
        inv = 1.0 / den
        b4 = (lane & 16) != 0
        b3 = (lane & 8) != 0
        outs = [None] * 8
        G2 = 2
        for w0 in range(0, NW, G2):
            ws = range(w0, w0 + G2)
            for w in ws:
                p[w] = p[w] * inv
                p[w] = jnp.where(b4, p[w], pltpu.roll(p[w], 112, 1))
            for w in ws:
                p[w] = jnp.where(b3, p[w], pltpu.roll(p[w], 120, 1))
            for w in ws:
                for c in range(8):
                    pr = p[w] * qkv[2, PH[c], pl.ds(base - 2 * w, 8), :]
                    outs[c] = pr if outs[c] is None else outs[c] + pr
        return outs

    def attn_pair(r0, mask=False):
        parts = [attn8(pl.multiple_of(PAD + h * HS + r0 + 8 * u, 8), (r0 + 8 * u) if (h == 0 and mask) else None)
                 for h in range(2) for u in range(2)]
        lo = [jnp.concatenate([parts[0][c], parts[1][c]], axis=0) for c in range(8)]
        hi = [jnp.concatenate([parts[2][c], parts[3][c]], axis=0) for c in range(8)]
        for n in range(4):
            cs = _acomb(lo[n], lo[n + 4], hi[n], hi[n + 4])
            for i in range(7):
                oa.at[i][pl.ds(pl.multiple_of(r0, 16), 16), n * 128:(n + 1) * 128] = cs[i]
        return hi[7]

    wd0 = lambda c: wd_raw.at[0, c * FC:(c + 1) * FC, :]
    RA, RBB, RC, RD = 0, 512, 256, 768

    x_copy(0).start()
    x_copy(1).start()
    gu0_copy(0, 0).start()
    z_copy().start()
    gu0_copy(1, 0).start()
    x_copy(2).start()
    wd0_copy(0).start()
    x_copy(3).start()
    x_copy(4).start()
    gu0_copy(0, 1).start()
    gu0_copy(1, 1).start()
    wd0_copy(1).start()
    x_copy(5).start()
    wq_copy(0).start()
    for cp in wo_copies():
        cp.start()
    wq_copy(1).start()

    x_copy(0).wait()
    ln_rows(RA, 128)
    x_copy(1).wait()
    ln_rows(RA + 128, 128)

    gu0_copy(0, 0).wait()
    prep_gu(0, (0,))
    mg = [None] * 7
    for i in [4, 2, 3, 1, 0, 6, 5]:
        mg[i] = _dot(xa[i, RA:RA + RB, :], bgu[i, :, :FH])
    gg = [(v, _gate_tanh(v)) for v in _ccomb(mg)]

    z_copy().wait()
    gu0_copy(1, 0).wait()
    x_copy(2).wait()
    prep_gu(0, (1,))
    mu = [None] * 7
    for i in [4, 2, 3, 1, 0, 6, 5]:
        mu[i] = _dot(xa[i, RA:RA + RB, :], bgu[i, :, FH:])
    ha = _acomb(*[_glu2(a[0], a[1], b) for a, b in zip(gg, _ccomb(mu))])
    ln_rows(RBB, 128, [mu[i][k:k + 16] for i in [4, 2, 3, 1, 0, 6, 5] for k in range(0, RB, 64)],
            0.85)

    wd0_copy(0).wait()
    x_copy(3).wait()
    prep_d(wd0(0), FH)
    hb0, anc = ffn_gu(RBB, 128, [6, 5, 0, 1, 4, 2, 3])
    ffn_dn(RA, RB, ha, [3, 0, 4, 1, 2, 6, 5], True)
    ln_rows(RBB + 128, 128, anc, 0.7)

    x_copy(4).wait()
    gu0_copy(0, 1).wait()
    gu0_copy(1, 1).wait()
    hb1, anc = ffn_gu(RBB + 128, 128, [4, 0, 2, 6, 5, 3, 1])
    anc2 = ffn_dn(RBB, 128, hb0, [3, 6, 5, 4, 2, 0, 1], True)
    ffn_dn(RBB + 128, 128, hb1, [3, 6, 5, 4, 2, 0, 1], True)
    prep_gu(1)
    ln_rows(RC, RB, anc + anc2[:28], 0.85)

    wd0_copy(1).wait()
    x_copy(5).wait()
    prep_d(wd0(1), FH)
    h2, anc = ffn_gu(RA, RB, [4, 2, 3, 1, 0, 6, 5])
    ffn_dn(RA, RB, h2, [6, 1, 4, 3, 2, 5, 0], False)
    ln_rows(RD, RB, anc, 0.75)
    zs_ = [p for p in range(49) if p % 7 in (0, 3, 4)]
    zero_acc0(zs_[:7], anc)

    wq_copy(0).wait()
    h3, anc = ffn_gu(RBB, RB, [0, 1, 2, 3, 4, 5, 6])
    zero_acc0(zs_[7:], anc)
    prep_q_half(0, 0, bq.at[56:63], 2)
    ffn_dn(RBB, RB, h3, [0, 3, 4, 6, 2, 1, 5], False, True)

    for cp in wo_copies():
        cp.wait()
    wq_copy(2).start()
    for cp in gu_copies(1, 1):
        cp.start()
    wd_copy(1, 1).start()

    def p2_body(i, carry):
        @pl.when(i == 1)
        def _():
            wq_copy(1).wait()

        @pl.when(i == 3)
        def _():
            wq_copy(2).wait()

        @pl.when(i == 4)
        def _():
            for cp in gu_copies(1, 1):
                cp.wait()
            wd_copy(1, 1).wait()
        bqv = bq.at[pl.ds(49 + 7 * i, 21)]
        anc16 = qkv_tiles(i >> 1, i & 1, bqv.at[7:14])
        prep_q_half(jnp.minimum((i + 1) >> 1, 2), (i + 1) & 1, bqv.at[14:21], 2)
        tm = true_mask()
        tm16 = jnp.concatenate([tm, tm], axis=0)
        jobs = []
        for k in range(6):
            jobs += [('x', k, q) for q in range(14)]
        for k in range(6):
            jobs += [('o', k, q) for q in range(4)]
        for k in range(8):
            jobs += [('g', k, q) for q in range(7)]
        for k in range(4):
            jobs += [('d', k, q) for q in range(7)]
        for k in range(7):
            jobs += [('z', k, q) for q in range(4)]
        by = {}
        for kind in 'oxgzd':
            js = [jb for jb in jobs if jb[0] == kind]
            for e, jb in enumerate(js):
                lo_, hi_ = {}.get(kind, [0.0, 1.0])
                by[jb] = lo_ + (hi_ - lo_) * (e + 0.5) / len(js)
        ranked = sorted(jobs, key=lambda jb: by[jb])
        na = len(anc16) - 4
        at = {jb: anc16[(e * na) // len(ranked)] for e, jb in enumerate(ranked)}
        for k in range(6):
            make_xa2(pl.multiple_of(jnp.minimum(96 * i, QS - 96), 32) + 16 * k, tm16,
                     [at['x', k, q] for q in range(14)])
        for k in range(6):
            m_ = jnp.minimum(3 * i + (k >> 1), 15)
            prep_o_chunk(m_ >> 3, pl.multiple_of((m_ & 7) * 16, 16), k & 1, tm,
                         [at['o', k, q][0:8] for q in range(4)])
        for k in range(8):
            for q in range(7):
                prep_gu2_piece(i >> 2, q, k & 1, pl.multiple_of((i & 3) * 64, 64) + 16 * (k >> 1), tm16,
                               at['g', k, q], 1)
        for k in range(4):
            for q in range(7):
                prep_d2_piece(i >> 2, q, pl.multiple_of((i & 3) * 32, 32) + 16 * (k >> 1), (k & 1) * 128, tm16,
                              at['d', k, q], 1)
        az = acc.at[pl.ds(49 + 7 * i, 21)]
        for k in range(7):
            for q in range(4):
                z16 = jnp.where(tm16, 0.0, at['z', k, q])
                for r0 in range(64 * q, 64 * q + 64, 16):
                    for c in range(2):
                        az.at[k][r0:r0 + 16, c * 128:(c + 1) * 128] = z16
        return carry

    lax.fori_loop(0, 6, p2_body, 0)

    def p3_body(u, carry):
        j = u >> 1
        s_ = u & 1
        sl = j & 1
        jn = jnp.minimum((u >> 1) + 1, NG - 1)
        sn = 1 - sl

        @pl.when(jnp.logical_and(s_ == 0, j + 1 < NG))
        def _():
            wd_copy(jn, sn).wait()
            for cp in gu_copies(jn, sn):
                cp.wait()
        a4 = pl.multiple_of((u - 1) * 64, 64)
        for g in range(5):
            att_last = attn_pair(a4 + 16 * g if g < 4 else 832 + 16 * jnp.minimum(u - 1, 11), g == 0)
        tm = true_mask()
        tm16 = jnp.concatenate([tm, tm], axis=0)

        rows = pl.ds(pl.multiple_of(s_ * RB, RB), RB)
        accs = acc.at[pl.ds(49 * s_, 49)]
        order = (0, 3, 4, 6, 2, 1, 5)
        c1 = [None] * 7
        dprep = []
        h = [[None] * 4 for _ in range(4)]

        def gate_up(i):
            ms = [None] * 7
            for k in order:
                ms[k] = _dot(xa2.at[7 * i + k][rows, :], bg(sl, i, k)[...])
            c1[i] = _ccomb(ms)
            return [ms[k][r_:r_ + 16, t * 128:(t + 1) * 128] for k in order for r_ in range(0, RB, 64)
                    for t in range(2)]

        def hidden(a, e):
            if h[2 * a][2 * e] is None:
                for q in range(4):
                    m = [None if v is None else v[q] for v in c1]
                    if (a, e) == (0, 0):
                        cc = m[0] + m[3] - m[4] + m[6]
                    elif (a, e) == (0, 1):
                        cc = m[2] + m[4]
                    elif (a, e) == (1, 0):
                        cc = m[1] + m[3]
                    else:
                        cc = m[0] - m[1] + m[2] + m[5]
                    h[2 * a + (q >> 1)][2 * e + (q & 1)] = _glu2(cc[:, :128], _gate_tanh(cc[:, :128]),
                                                                 cc[:, 128:])
            return [[h[2 * a + b][2 * e + f] for f in range(2)] for b in range(2)]

        def down(i):
            p, q, sg = _A_TERMS[i]
            P = hidden(*p)
            if q is not None:
                Q = hidden(*q)
                P = [[P[b][f] + Q[b][f] if sg > 0 else P[b][f] - Q[b][f] for f in range(2)] for b in range(2)]
            out = []
            if i == 2:
                v = P[0][0]
                P[0][0] = jnp.concatenate([jnp.where(tm16, v[0:16], att_last), v[16:]], axis=0)
            a7 = _asum(P[0][0], P[0][1], P[1][0], P[1][1])
            for k in [6, 1, 4, 3, 2, 5, 0]:
                y = _dot(a7[k].astype(bf16), bd2.at[sl, 7 * i + k][...])
                out += [y[r_:r_ + 16, 0:128] for r_ in range(0, RB, 128)]
                old = accs.at[7 * i + k][...]
                if i == 6:
                    old = jnp.where(u == 1, 0.0, old)
                accs.at[7 * i + k][...] = old + y
            return out

        seq = 'G0 G3 G4 G6 G1 G2 D2 G5 D6 D4 D3 D1 D0 D5'.split()
        sanc = []
        for tk in seq:
            if tk[0] == 'D' and not dprep:
                dprep.append(1)
                lo_, hi_ = 0, 1
                src = [a for p in range(lo_, hi_) for a in sanc[p]]
                pcs = [(k0, c0, i) for k0 in range(0, 64, 16) for c0 in range(0, QD, 128) for i in range(7)]
                for e, (k0, c0, i) in enumerate(pcs):
                    prep_d2_piece(sn, i, pl.multiple_of(s_ * 64, 64) + k0, c0, tm16,
                                  src[e * len(src) // len(pcs)], 1)
            sanc.append((gate_up if tk[0] == 'G' else down)(int(tk[1])))
        kb = pl.multiple_of(s_ * (QD // 2), QD // 2)
        PW = [[2, 5], [7, 8], [8, 14]]
        for a in range(max(GA) + 1):
            members = [i for i in range(7) if GA[i] == a]
            last = max(p for p, tk in enumerate(seq) if tk[0] == 'G' and int(tk[1]) in members)
            lo_, hi_ = max(PW[a][0], last + 1), max(PW[a][1], last + 2)
            src = [x for p in range(lo_, hi_) for x in sanc[p]]
            pieces = [(t, k0, i) for k0 in range(0, QD // 2, 16) for t in range(2) for i in members]
            for e, (t, k0, i) in enumerate(pieces):
                prep_gu2_piece(sn, i, t, kb + k0, tm16, src[e * len(src) // len(pieces)], 4)

        @pl.when(jnp.logical_and(s_ == 1, j + 3 < NG))
        def _():
            wd_copy(j + 3, sn).start()
            for cp in gu_copies(j + 3, sn):
                cp.start()
        return carry

    wd_copy(2, 0).start()
    for cp in gu_copies(2, 0):
        cp.start()
    lax.fori_loop(1, 2 * NG, p3_body, 0)

    SB = 32

    def p4_body(k, carry):
        acck = acc.at[pl.ds(49 * (k >> 1), 49)]
        for u in range(RB // SB):
            b = u // (128 // SB)
            q0 = pl.multiple_of(k * 128 + (u % (128 // SB)) * SB, SB)
            r0 = pl.multiple_of(b * QS + q0, SB)
            rows = pl.ds(r0, SB)
            qr = pl.multiple_of((k & 1) * 128 + (u % (128 // SB)) * SB, SB)
            for n in range(2):
                ms = [None] * 7
                for i in [0, 1, 2, 3, 4, 5, 6]:
                    ms[i] = _dot(oa.at[i][rows, :], bo.at[i, n][...])
                av = []
                for i in range(7):
                    ld = lambda e: acck.at[7 * i + e][pl.ds(qr, SB), :]
                    av.append((lambda: ld(0) + ld(3) - ld(4) + ld(6), lambda: ld(2) + ld(4),
                               lambda: ld(1) + ld(3), lambda: ld(0) - ld(1) + ld(2) + ld(5))[2 * b + n]())
                ss = _ccomb(ms)
                fs = _ccomb(av)
                for q, (h, c0) in enumerate(((0, n * 256), (0, HD + n * 256), (1, n * 256), (1, HD + n * 256))):
                    hf = 0.25 * fs[q]
                    g = hf + hf * jnp.tanh(hf)
                    xv = xraw.at[h][rows, c0:c0 + 256].astype(f32)
                    obuf.at[h][rows, c0:c0 + 256] = (xv + ss[q] * g).astype(bf16)
            out_copy(r0, SB, 0).start()
        return carry

    lax.fori_loop(0, NB, p4_body, 0)
    out_copy(0, HS, 0).wait()


@jax.jit
def pallas_recurrent_scan__sliding_local_dilated__geglu_ffn__prompt_kernel(
    A_x: jax.Array,
    A_wqkv: jax.Array,
    A_wo: jax.Array,
    B_x: jax.Array,
    B_w_gate: jax.Array,
    B_w_up: jax.Array,
    B_w_down: jax.Array,
):
    any_spec = pl.BlockSpec(memory_space=pl.ANY)
    out = pl.pallas_call(
        _kernel,
        out_shape=jax.ShapeDtypeStruct((2, HS, D), bf16),
        in_specs=[any_spec] * 6,
        out_specs=any_spec,
        scratch_shapes=[
            pltpu.VMEM((2, HS, D), bf16),
            pltpu.VMEM((7, HS // 2, HD), u32),
            pltpu.VMEM((49, QS // 2, QD), u32),
            pltpu.VMEM((2, 2, D, GC), bf16),
            pltpu.VMEM((2, GC, D), bf16),
            pltpu.VMEM((7, HD // 2, FC), u32),
            pltpu.VMEM((7, FH // 2, HD), u32),
            pltpu.VMEM((2, 49, 64, QD), u32),
            pltpu.VMEM((105, RB, QD), u32),
            pltpu.VMEM((3, D, D), bf16),
            pltpu.VMEM((3, 8, PAD + S + 8, 128), f32),
            pltpu.VMEM((4, D, 256), bf16),
            pltpu.VMEM((7, 2, HD // 2, 256), u32),
            pltpu.VMEM((2, 2, HS, 128), f32),
            pltpu.VMEM((2, 16, 128), bf16),
            pltpu.SemaphoreType.DMA((26,)),
        ] + [pltpu.VMEM((2, 7 * n, QD // 2, 256), u32) for n in (2, 2, 3)],
        compiler_params=pltpu.CompilerParams(vmem_limit_bytes=127 * 1024 * 1024,
                                             disable_bounds_checks=True,
                                             disable_semaphore_checks=True),
        name="fusedk",
    )(A_x.reshape(2, HS, D), A_wqkv, A_wo, B_w_gate, B_w_up, B_w_down)
    return out.reshape(1, S, D)
```

```python
import jax
import jax.numpy as jnp
from jax import lax
import jax.experimental.pallas as pl
import jax.experimental.pallas.tpu as pltpu

f32 = jnp.float32
bf16 = jnp.bfloat16
u32 = jnp.uint32

S, D, F = 2048, 1024, 3584
HS, HD = S // 2, D // 2
FC = 256
FH = FC // 2
NF = F // FC
QS, QD = S // 4, D // 4
GC = 512
NG = F // GC
RB = 256
NB = HS // RB
PAD = 16
NW = 8
SCALE = 32 ** -0.5
LOG2E = 1.4426950408889634
NEG = -1e9 / SCALE


def _dot(a, b):
    return jnp.dot(a, b, preferred_element_type=f32)


def _acomb(a11, a12, a21, a22):
    r = lambda v: v.astype(bf16)
    return [r(a11 + a22), r(a21 + a22), r(a11), r(a22), r(a11 + a12), r(a21 - a11), r(a12 - a22)]


def _bcomb(b11, b12, b21, b22):
    r = lambda v: v.astype(bf16)
    return [r(b11 + b22), r(b11), r(b12 - b22), r(b21 - b11), r(b22), r(b11 + b12), r(b21 + b22)]


def _asum(a11, a12, a21, a22):
    return [a11 + a22, a21 + a22, a11, a22, a11 + a12, a21 - a11, a12 - a22]


def _bsum(b11, b12, b21, b22):
    return [b11 + b22, b11, b12 - b22, b21 - b11, b22, b11 + b12, b21 + b22]


_A_TERMS = [((0, 0), (1, 1), 1), ((1, 0), (1, 1), 1), ((0, 0), None, 0), ((1, 1), None, 0),
            ((0, 0), (0, 1), 1), ((1, 0), (0, 0), -1), ((0, 1), (1, 1), -1)]
_B_TERMS = [((0, 0), (1, 1), 1), ((0, 0), None, 0), ((0, 1), (1, 1), -1), ((1, 0), (0, 0), -1),
            ((1, 1), None, 0), ((0, 0), (0, 1), 1), ((1, 0), (1, 1), 1)]


def _ccomb(m):
    m1, m2, m3, m4, m5, m6, m7 = m
    return m1 + m4 - m5 + m7, m3 + m5, m2 + m4, m1 - m2 + m3 + m6


def _gate_tanh(x):
    c = 0.7978845608028654
    return jnp.tanh(x * (c + (c * 0.044715) * (x * x)))


def _glu2(g, th, u):
    a = g * u
    return a + a * th


def _sum8(v):
    return ((v[0] + v[1]) + (v[2] + v[3])) + ((v[4] + v[5]) + (v[6] + v[7]))


def _butterfly(sets, masks, axis, size):
    for b in range(3):
        sh = 1 << b
        out = []
        for blk in sets:
            nxt = list(blk)
            for c in range(8):
                if c & sh == 0:
                    lo, hi = blk[c], blk[c + sh]
                    nxt[c] = jnp.where(masks[b], lo, pltpu.roll(hi, sh, axis))
                    nxt[c + sh] = jnp.where(masks[b], pltpu.roll(lo, size - sh, axis), hi)
            out.append(nxt)
        sets = out
    return sets


def _kernel(x_hbm, wqkv_hbm, wo_hbm, wg_hbm, wu_hbm, wd_hbm, out_hbm,
            xraw, xa_u, xa2_u, gu_raw, wd_raw, bgu_u, bd_u, bd2_u, accq, wq_raw, qkv,
            wo_raw, bo_u, stats, zbuf, sems, *bgu2_u):
    acc = accq
    bq = accq.bitcast(bf16)
    bo = bo_u.bitcast(bf16)
    obuf = xraw
    xa = xa_u.bitcast(bf16)
    bgu = bgu_u.bitcast(bf16)
    bd = bd_u.bitcast(bf16)
    bd2 = bd2_u.bitcast(bf16)
    xa2 = xa2_u.bitcast(bf16)
    GA = [0, 1, 2, 0, 2, 2, 1]
    _al = [r.bitcast(bf16) for r in bgu2_u]
    _pos = [sum(1 for q in range(i) if GA[q] == GA[i]) for i in range(7)]
    bg = lambda slot, i, k: _al[GA[i]].at[slot, 7 * _pos[i] + k]
    oa = xa
    pk = lambda v: pltpu.bitcast(v, u32)
    un = lambda v: pltpu.bitcast(v, bf16)

    lane = lax.broadcasted_iota(jnp.int32, (8, 128), 1)
    row8 = lax.broadcasted_iota(jnp.int32, (8, 128), 0)
    lane_lo = [(lane & (1 << b)) == 0 for b in range(3)]
    row_lo = [(row8 & (1 << b)) == 0 for b in range(3)]

    XP = [(0, 128), (128, 128), (512, 128), (640, 128), (256, 256), (768, 256)]

    def x_copy(r):
        r0, n = XP[r]
        return pltpu.make_async_copy(x_hbm.at[:, pl.ds(r0, n), :],
                                     xraw.at[:, pl.ds(r0, n), :], sems.at[(0, 1, 2, 3, 23, 14)[r]])

    def gu_copies(j, slot):
        off = pl.multiple_of(j * GC, GC)
        return (pltpu.make_async_copy(wg_hbm.at[:, pl.ds(off, GC)], gu_raw.at[slot, 0], sems.at[4 + 3 * slot]),
                pltpu.make_async_copy(wu_hbm.at[:, pl.ds(off, GC)], gu_raw.at[slot, 1], sems.at[5 + 3 * slot]))

    def wd_copy(j, slot):
        off = pl.multiple_of(j * GC, GC)
        return pltpu.make_async_copy(wd_hbm.at[pl.ds(off, GC), :], wd_raw.at[slot], sems.at[6 + 3 * slot])

    def gu0_copy(t, c):
        w = (wg_hbm, wu_hbm)[t]
        return pltpu.make_async_copy(w.at[:, pl.ds(c * FC, FC)], gu_raw.at[0, t, :, pl.ds(c * FC, FC)],
                                     sems.at[15 + 2 * c + t])

    def wd0_copy(c):
        return pltpu.make_async_copy(wd_hbm.at[pl.ds(c * FC, FC), :], wd_raw.at[0, pl.ds(c * FC, FC), :],
                                     sems.at[19 + c])

    def wq_copy(t):
        return pltpu.make_async_copy(wqkv_hbm.at[:, pl.ds(t * D, D)], wq_raw.at[t], sems.at[10 + t])

    def wo_copies():
        return [pltpu.make_async_copy(wo_hbm.at[:, pl.ds(c * 256, 256)], wo_raw.at[c], sems.at[24])
                for c in range(4)]

    class _Z:
        cps = [pltpu.make_async_copy(x_hbm.at[0, pl.ds(0, 16), pl.ds(0, 128)], zbuf.at[q], sems.at[21 + q])
               for q in range(2)]

        def start(self):
            for cp in self.cps:
                cp.start()

        def wait(self):
            for cp in self.cps:
                cp.wait()

    z_copy = _Z

    def out_copy(r0, n, k):
        return pltpu.make_async_copy(obuf.at[:, pl.ds(r0, n), :], out_hbm.at[:, pl.ds(r0, n), :],
                                     sems.at[25 + k])

    def true_mask():
        return pk(zbuf[0]) == pk(zbuf[1])

    def ln_half(h, c0, tm16, a):
        xs = []
        for c in range(4):
            x2 = xraw.at[h][c0:c0 + 16, c * 256:(c + 1) * 256].astype(f32)
            xs += [x2[:, :128], x2[:, 128:]]
        s1 = _sum8(xs)
        if a is not None:
            s1 = jnp.where(tm16, s1, a)
        m = jnp.sum(s1, axis=-1, keepdims=True) * (1.0 / D)
        xc = [x - m for x in xs]
        v = jnp.sum(_sum8([x * x for x in xc]), axis=-1, keepdims=True) * (1.0 / D)
        r = lax.rsqrt(v + 1e-5)
        stats.at[h, 0][c0:c0 + 16, :] = jnp.broadcast_to(m, (16, 128))
        stats.at[h, 1][c0:c0 + 16, :] = jnp.broadcast_to(r, (16, 128))
        return [x * r for x in xc]

    def ln_rows(r0, n, anc=None, af=0.85):
        tm16 = None
        if anc is not None:
            tm = true_mask()
            tm16 = jnp.concatenate([tm, tm], axis=0)
            anc = anc[:int(len(anc) * af)]
        nch = n // 16
        for k in range(nch):
            c0 = r0 + 16 * k
            a = [None, None]
            if anc is not None:
                a = [anc[(len(anc) * (2 * k + u)) // (2 * nch)] for u in range(2)]
            lo = ln_half(0, c0, tm16, a[0])
            hi = ln_half(1, c0, tm16, a[1])
            for c in range(4):
                cs = _acomb(lo[c], lo[c + 4], hi[c], hi[c + 4])
                for i in range(7):
                    xa.at[i][c0:c0 + 16, c * 128:(c + 1) * 128] = cs[i]

    def prep_gu(c, ts=(0, 1)):
        KC = 32
        for t in ts:
            w = gu_raw.at[0, t]
            for k0 in range(0, HD, KC):
                lo = w[k0:k0 + KC, c * FC:(c + 1) * FC].astype(f32)
                hi = w[HD + k0:HD + k0 + KC, c * FC:(c + 1) * FC].astype(f32)
                cs = _bcomb(lo[:, :FH], lo[:, FH:], hi[:, :FH], hi[:, FH:])
                for i in range(7):
                    bgu.at[i][k0:k0 + KC, t * FH:(t + 1) * FH] = cs[i]

    def prep_d(w, kh):
        KC = 16
        for k0 in range(0, kh, KC):
            for c0 in range(0, HD, 256):
                g = lambda a, b: w[a + k0:a + k0 + KC, b + c0:b + c0 + 256].astype(f32)
                cs = _bcomb(g(0, 0), g(0, HD), g(kh, 0), g(kh, HD))
                for i in range(7):
                    bd.at[i][k0:k0 + KC, c0:c0 + 256] = cs[i]

    def two_level_piece(terms, inner, ld, i, tm16, anc, nanc, store):
        p, q, sg = terms[i]
        P = ld(*p)
        for e in range(nanc):
            P[e >> 1][e & 1] = jnp.where(tm16, P[e >> 1][e & 1], anc)
        if q is not None:
            Q = ld(*q)
            P = [[P[b][d] + Q[b][d] if sg > 0 else P[b][d] - Q[b][d] for d in range(2)] for b in range(2)]
        ops = inner(P[0][0], P[0][1], P[1][0], P[1][1])
        for k in range(7):
            store(7 * i + k, ops[k].astype(bf16))

    def prep_gu2_piece(slot, i, t, k0, tm16, anc, nanc):
        w = gu_raw.at[slot, t]

        def ld(R, C):
            out = []
            for b in range(2):
                x2 = w[pl.ds((2 * R + b) * QD + k0, 16), C * 256:(C + 1) * 256].astype(f32)
                out.append([x2[:, :128], x2[:, 128:]])
            return out

        def store(p, v):
            bg(slot, i, p % 7)[pl.ds(k0, 16), t * 128:(t + 1) * 128] = v
        two_level_piece(_B_TERMS, _bsum, ld, i, tm16, anc, nanc, store)

    def prep_d2_piece(slot, i, k0, c0, tm16, anc, nanc):
        w = wd_raw.at[slot]

        def ld(R, C):
            return [[w[pl.ds((2 * R + b) * 128 + k0, 16),
                       (2 * C + d) * QD + c0:(2 * C + d) * QD + c0 + 128].astype(f32) for d in range(2)]
                    for b in range(2)]

        def store(p, v):
            bd2.at[slot, p][pl.ds(k0, 16), c0:c0 + 128] = v
        two_level_piece(_B_TERMS, _bsum, ld, i, tm16, anc, nanc, store)

    def make_xa2(r0, tm16, ancs):
        st = [[[stats.at[a, e][pl.ds(b * QS + r0, 16), :] for e in range(2)] for b in range(2)] for a in range(2)]
        for j in range(2):
            def ld(R, C):
                out = []
                for b in range(2):
                    m, r = st[R][b]
                    row = []
                    for d in range(2):
                        c0 = (2 * C + d) * QD + j * 128
                        xv = xraw.at[R][pl.ds(b * QS + r0, 16), c0:c0 + 128].astype(f32)
                        row.append((xv - m) * r)
                    out.append(row)
                return out

            def store(p, v):
                xa2.at[p][pl.ds(r0, 16), j * 128:(j + 1) * 128] = v
            for i in range(7):
                two_level_piece(_A_TERMS, _asum, ld, i, tm16, ancs[7 * j + i], 2, store)

    def ffn_gu(r0, n, o1):
        ms = [None] * 7
        for i in o1:
            ms[i] = _dot(xa[i, r0:r0 + n, :], bgu[i])
        anc = [ms[i][k:k + 16, t * FH:(t + 1) * FH] for i in o1 for t in range(2) for k in range(0, n, 64)]
        hs = _acomb(*[_glu2(v[:, :FH], _gate_tanh(v[:, :FH]), v[:, FH:]) for v in _ccomb(ms)])
        return hs, anc

    def ffn_dn(r0, n, hs, od, first, last=False):
        b, q0 = r0 // QS, r0 % QS
        anc = []
        for i in od:
            y = _dot(hs[i], bd[i])
            anc += [y[k:k + 16, 0:128] for k in range(0, n, 32)]
            lo, hi = (acc.at[7 * i + e] for e in ((6, 2), (1, 5))[b])
            ylo, yhi = y[:, :QD], y[:, QD:]
            if not first:
                ylo = ylo + lo[q0:q0 + n, :]
                yhi = yhi + hi[q0:q0 + n, :]
            if last:
                yhi = yhi + (ylo - acc.at[7 * i + 2][q0:q0 + n, :])
            lo[q0:q0 + n, :] = ylo
            hi[q0:q0 + n, :] = yhi
        return anc

    def zero_acc0(ps, anc):
        tm = true_mask()
        tm16 = jnp.concatenate([tm, tm], axis=0)
        pcs = [(p, q) for p in ps for q in range(4)]
        for e, (p, q) in enumerate(pcs):
            z16 = jnp.where(tm16, 0.0, anc[e * len(anc) // len(pcs)])
            for r0 in range(64 * q, 64 * q + 64, 16):
                for c in range(2):
                    acc.at[p][r0:r0 + 16, c * 128:(c + 1) * 128] = z16

    upk = lambda v: un(v).astype(f32)

    def prep_q_half(t, h, dst, par=1):
        KC = 16
        sa = (128 - 2) * h
        sb = 2 * (1 - h)
        w = wq_raw.at[t]

        def stage1(r0):
            blk = [pk(w[r0:r0 + KC, c * 128:(c + 1) * 128]) for c in range(8)]
            rl = lambda v, sft: v if (isinstance(sft, int) and sft == 0) else pltpu.roll(v, sft, 1)
            return [jnp.where(lane_lo[1], rl(blk[c], sa), rl(blk[c + 2], sb)) for c in (0, 1, 4, 5)]

        def stage(sets, jb, b):
            sh = 1 << b
            out = []
            for blk in sets:
                nxt = list(blk)
                for j in range(4):
                    if j & jb == 0:
                        lo, hi = blk[j], blk[j + jb]
                        nxt[j] = jnp.where(lane_lo[b], lo, pltpu.roll(hi, sh, 1))
                        nxt[j + jb] = jnp.where(lane_lo[b], pltpu.roll(lo, 128 - sh, 1), hi)
                out.append(nxt)
            return out

        for k00 in range(0, HD, KC * par):
            ks = [k00 + KC * q for q in range(par)]
            hv = stage(stage([stage1(hk * HD + k0) for k0 in ks for hk in range(2)], 1, 0), 2, 2)
            for q, k0 in enumerate(ks):
                lo, hi = hv[2 * q], hv[2 * q + 1]
                for e in range(2):
                    cs = _bcomb(upk(lo[e]), upk(lo[e + 2]), upk(hi[e]), upk(hi[e + 2]))
                    for i in range(7):
                        dst.at[i][k0:k0 + KC, e * 128:(e + 1) * 128] = cs[i]

    def qkv_tiles(t, h, src):
        anc16 = []
        for e in range(2):
            qlo = qkv.at[t, 4 * h + e]
            qhi = qkv.at[t, 4 * h + 2 + e]
            for r in range(NB):
                oq = [1, 4, 2, 3, 0, 5, 6]
                ms = [None] * 7
                for i in oq:
                    ms[i] = _dot(xa[i, r * RB:(r + 1) * RB, :], src.at[i][:, e * 128:(e + 1) * 128])
                c11, c12, c21, c22 = _ccomb(ms)
                anc16 += [ms[i][k:k + 16] for i in oq for k in range(0, RB, 64)]
                r0 = PAD + r * RB
                qlo[r0:r0 + RB, :] = c11
                qhi[r0:r0 + RB, :] = c12
                qlo[HS + r0:HS + r0 + RB, :] = c21
                qhi[HS + r0:HS + r0 + RB, :] = c22
                if r == 0:
                    qlo[PAD - 16:PAD, :] = jnp.broadcast_to(c11[0:1, :], (16, 128))
                    qhi[PAD - 16:PAD, :] = jnp.broadcast_to(c12[0:1, :], (16, 128))
        return anc16

    def prep_o_chunk(n2, g16, e, tm, ancs):
        res = []
        for h in range(2):
            w = wo_raw.at[n2 + 2 * h]
            w16 = [w[pl.ds(128 * i + g16, 16), e * 128:(e + 1) * 128].astype(f32) for i in range(8)]
            for u in range(2):
                blk = [v[8 * u:8 * u + 8] for v in w16]
                blk[0] = jnp.where(tm, blk[0], ancs[2 * h + u])
                res += _butterfly([blk], row_lo, 0, 8)
        cols = [[jnp.concatenate([res[2 * h][j], res[2 * h + 1][j]], axis=0) for j in range(8)]
                for h in range(2)]
        for b in range(4):
            cs = _bcomb(cols[0][b], cols[1][b], cols[0][b + 4], cols[1][b + 4])
            for i in range(7):
                bo.at[i, n2][pl.ds(b * 128 + g16, 16), e * 128:(e + 1) * 128] = cs[i]

    PH = [4 * ((c >> 1) & 1) + 2 * (c >> 2) + (c & 1) for c in range(8)]

    def attn_pair(r0, mask=False):
        bases = [pl.multiple_of(PAD + h * HS + r0 + 8 * u, 8) for h in range(2) for u in range(2)]
        lgs = []
        for g, base in enumerate(bases):
            lg = [None] * NW
            for c in range(8):
                q = qkv[0, PH[c], pl.ds(base, 8), :]
                for w in range(NW):
                    pr = q * qkv[1, PH[c], pl.ds(base - 2 * w, 8), :]
                    lg[w] = pr if lg[w] is None else lg[w] + pr
            s8 = 8 if g & 1 else 120
            s16 = 16 if g & 2 else 112
            for w in range(NW):
                lg[w] = lg[w] + pltpu.roll(lg[w], s8, 1)
                lg[w] = lg[w] + pltpu.roll(lg[w], s16, 1)
            lgs.append(lg)
        b3 = (lane & 8) != 0
        b4 = (lane & 16) != 0
        lg = [jnp.where(b4, jnp.where(b3, lgs[3][w], lgs[2][w]), jnp.where(b3, lgs[1][w], lgs[0][w]))
              for w in range(NW)]
        if mask:
            pos = jnp.where(b4, S, row8 + r0 + (lane & 8))
            for w in range(1, NW):
                lg[w] = jnp.where(pos >= 2 * w, lg[w], NEG)
        m = lg[0]
        for w in range(1, NW):
            m = jnp.maximum(m, lg[w])
        p = [jnp.exp2((lg[w] - m) * (SCALE * LOG2E)) for w in range(NW)]
        den = p[0]
        for w in range(1, NW):
            den = den + p[w]
        inv = 1.0 / den
        p = [v * inv for v in p]
        parts = []
        for g, base in enumerate(bases):
            k4 = b4 if g & 2 else jnp.logical_not(b4)
            k3 = b3 if g & 1 else jnp.logical_not(b3)
            outs = [None] * 8
            for w in range(NW):
                pw = jnp.where(k4, p[w], pltpu.roll(p[w], 112 if g & 2 else 16, 1))
                pw = jnp.where(k3, pw, pltpu.roll(pw, 120 if g & 1 else 8, 1))
                for c in range(8):
                    pr = pw * qkv[2, PH[c], pl.ds(base - 2 * w, 8), :]
                    outs[c] = pr if outs[c] is None else outs[c] + pr
            parts.append(outs)
        lo = [jnp.concatenate([parts[0][c], parts[1][c]], axis=0) for c in range(8)]
        hi = [jnp.concatenate([parts[2][c], parts[3][c]], axis=0) for c in range(8)]
        for n in range(4):
            cs = _acomb(lo[n], lo[n + 4], hi[n], hi[n + 4])
            for i in range(7):
                oa.at[i][pl.ds(pl.multiple_of(r0, 16), 16), n * 128:(n + 1) * 128] = cs[i]
        return hi[7]

    wd0 = lambda c: wd_raw.at[0, c * FC:(c + 1) * FC, :]
    RA, RBB, RC, RD = 0, 512, 256, 768

    x_copy(0).start()
    x_copy(1).start()
    gu0_copy(0, 0).start()
    z_copy().start()
    gu0_copy(1, 0).start()
    x_copy(2).start()
    wd0_copy(0).start()
    x_copy(3).start()
    x_copy(4).start()
    gu0_copy(0, 1).start()
    gu0_copy(1, 1).start()
    wd0_copy(1).start()
    x_copy(5).start()
    wq_copy(0).start()
    for cp in wo_copies():
        cp.start()
    wq_copy(1).start()

    x_copy(0).wait()
    ln_rows(RA, 128)
    x_copy(1).wait()
    ln_rows(RA + 128, 128)

    gu0_copy(0, 0).wait()
    prep_gu(0, (0,))
    mg = [None] * 7
    for i in [4, 2, 3, 1, 0, 6, 5]:
        mg[i] = _dot(xa[i, RA:RA + RB, :], bgu[i, :, :FH])
    gg = [(v, _gate_tanh(v)) for v in _ccomb(mg)]

    z_copy().wait()
    gu0_copy(1, 0).wait()
    x_copy(2).wait()
    prep_gu(0, (1,))
    mu = [None] * 7
    for i in [4, 2, 3, 1, 0, 6, 5]:
        mu[i] = _dot(xa[i, RA:RA + RB, :], bgu[i, :, FH:])
    ha = _acomb(*[_glu2(a[0], a[1], b) for a, b in zip(gg, _ccomb(mu))])
    ln_rows(RBB, 128, [mu[i][k:k + 16] for i in [4, 2, 3, 1, 0, 6, 5] for k in range(0, RB, 64)],
            0.85)

    wd0_copy(0).wait()
    x_copy(3).wait()
    prep_d(wd0(0), FH)
    hb0, anc = ffn_gu(RBB, 128, [6, 5, 0, 1, 4, 2, 3])
    ffn_dn(RA, RB, ha, [3, 0, 4, 1, 2, 6, 5], True)
    ln_rows(RBB + 128, 128, anc, 0.7)

    x_copy(4).wait()
    gu0_copy(0, 1).wait()
    gu0_copy(1, 1).wait()
    hb1, anc = ffn_gu(RBB + 128, 128, [4, 0, 2, 6, 5, 3, 1])
    anc2 = ffn_dn(RBB, 128, hb0, [3, 6, 5, 4, 2, 0, 1], True)
    ffn_dn(RBB + 128, 128, hb1, [3, 6, 5, 4, 2, 0, 1], True)
    prep_gu(1)
    ln_rows(RC, RB, anc + anc2[:28], 0.85)

    wd0_copy(1).wait()
    x_copy(5).wait()
    prep_d(wd0(1), FH)
    h2, anc = ffn_gu(RA, RB, [4, 2, 3, 1, 0, 6, 5])
    ffn_dn(RA, RB, h2, [6, 1, 4, 3, 2, 5, 0], False)
    ln_rows(RD, RB, anc, 0.75)
    zs_ = [p for p in range(49) if p % 7 in (0, 3, 4)]
    zero_acc0(zs_[:7], anc)

    wq_copy(0).wait()
    h3, anc = ffn_gu(RBB, RB, [0, 1, 2, 3, 4, 5, 6])
    zero_acc0(zs_[7:], anc)
    prep_q_half(0, 0, bq.at[56:63], 2)
    ffn_dn(RBB, RB, h3, [0, 3, 4, 6, 2, 1, 5], False, True)

    for cp in wo_copies():
        cp.wait()
    wq_copy(2).start()
    for cp in gu_copies(1, 1):
        cp.start()
    wd_copy(1, 1).start()

    def p2_body(i, carry):
        @pl.when(i == 1)
        def _():
            wq_copy(1).wait()

        @pl.when(i == 3)
        def _():
            wq_copy(2).wait()

        @pl.when(i == 4)
        def _():
            for cp in gu_copies(1, 1):
                cp.wait()
            wd_copy(1, 1).wait()
        bqv = bq.at[pl.ds(49 + 7 * i, 21)]
        anc16 = qkv_tiles(i >> 1, i & 1, bqv.at[7:14])
        prep_q_half(jnp.minimum((i + 1) >> 1, 2), (i + 1) & 1, bqv.at[14:21], 2)
        tm = true_mask()
        tm16 = jnp.concatenate([tm, tm], axis=0)
        jobs = []
        for k in range(6):
            jobs += [('x', k, q) for q in range(14)]
        for k in range(6):
            jobs += [('o', k, q) for q in range(4)]
        for k in range(8):
            jobs += [('g', k, q) for q in range(7)]
        for k in range(4):
            jobs += [('d', k, q) for q in range(7)]
        for k in range(7):
            jobs += [('z', k, q) for q in range(4)]
        by = {}
        for kind in 'oxgzd':
            js = [jb for jb in jobs if jb[0] == kind]
            for e, jb in enumerate(js):
                lo_, hi_ = {}.get(kind, [0.0, 1.0])
                by[jb] = lo_ + (hi_ - lo_) * (e + 0.5) / len(js)
        ranked = sorted(jobs, key=lambda jb: by[jb])
        na = len(anc16) - 4
        at = {jb: anc16[(e * na) // len(ranked)] for e, jb in enumerate(ranked)}
        for k in range(6):
            make_xa2(pl.multiple_of(jnp.minimum(96 * i, QS - 96), 32) + 16 * k, tm16,
                     [at['x', k, q] for q in range(14)])
        for k in range(6):
            m_ = jnp.minimum(3 * i + (k >> 1), 15)
            prep_o_chunk(m_ >> 3, pl.multiple_of((m_ & 7) * 16, 16), k & 1, tm,
                         [at['o', k, q][0:8] for q in range(4)])
        for k in range(8):
            for q in range(7):
                prep_gu2_piece(i >> 2, q, k & 1, pl.multiple_of((i & 3) * 64, 64) + 16 * (k >> 1), tm16,
                               at['g', k, q], 1)
        for k in range(4):
            for q in range(7):
                prep_d2_piece(i >> 2, q, pl.multiple_of((i & 3) * 32, 32) + 16 * (k >> 1), (k & 1) * 128, tm16,
                              at['d', k, q], 1)
        az = acc.at[pl.ds(49 + 7 * i, 21)]
        for k in range(7):
            for q in range(4):
                z16 = jnp.where(tm16, 0.0, at['z', k, q])
                for r0 in range(64 * q, 64 * q + 64, 16):
                    for c in range(2):
                        az.at[k][r0:r0 + 16, c * 128:(c + 1) * 128] = z16
        return carry

    lax.fori_loop(0, 6, p2_body, 0)

    def p3_body(u, carry):
        j = u >> 1
        s_ = u & 1
        sl = j & 1
        jn = jnp.minimum((u >> 1) + 1, NG - 1)
        sn = 1 - sl

        @pl.when(jnp.logical_and(s_ == 0, j + 1 < NG))
        def _():
            wd_copy(jn, sn).wait()
            for cp in gu_copies(jn, sn):
                cp.wait()
        a4 = pl.multiple_of((u - 1) * 64, 64)
        for g in range(5):
            att_last = attn_pair(a4 + 16 * g if g < 4 else 832 + 16 * jnp.minimum(u - 1, 11), g == 0)
        tm = true_mask()
        tm16 = jnp.concatenate([tm, tm], axis=0)

        rows = pl.ds(pl.multiple_of(s_ * RB, RB), RB)
        accs = acc.at[pl.ds(49 * s_, 49)]
        order = (0, 3, 4, 6, 2, 1, 5)
        c1 = [None] * 7
        dprep = []
        h = [[None] * 4 for _ in range(4)]

        def gate_up(i):
            ms = [None] * 7
            for k in order:
                ms[k] = _dot(xa2.at[7 * i + k][rows, :], bg(sl, i, k)[...])
            c1[i] = _ccomb(ms)
            return [ms[k][r_:r_ + 16, t * 128:(t + 1) * 128] for k in order for r_ in range(0, RB, 64)
                    for t in range(2)]

        def hidden(a, e):
            if h[2 * a][2 * e] is None:
                for q in range(4):
                    m = [None if v is None else v[q] for v in c1]
                    if (a, e) == (0, 0):
                        cc = m[0] + m[3] - m[4] + m[6]
                    elif (a, e) == (0, 1):
                        cc = m[2] + m[4]
                    elif (a, e) == (1, 0):
                        cc = m[1] + m[3]
                    else:
                        cc = m[0] - m[1] + m[2] + m[5]
                    h[2 * a + (q >> 1)][2 * e + (q & 1)] = _glu2(cc[:, :128], _gate_tanh(cc[:, :128]),
                                                                 cc[:, 128:])
            return [[h[2 * a + b][2 * e + f] for f in range(2)] for b in range(2)]

        def down(i):
            p, q, sg = _A_TERMS[i]
            P = hidden(*p)
            if q is not None:
                Q = hidden(*q)
                P = [[P[b][f] + Q[b][f] if sg > 0 else P[b][f] - Q[b][f] for f in range(2)] for b in range(2)]
            out = []
            if i == 2:
                v = P[0][0]
                P[0][0] = jnp.concatenate([jnp.where(tm16, v[0:16], att_last), v[16:]], axis=0)
            a7 = _asum(P[0][0], P[0][1], P[1][0], P[1][1])
            for k in [6, 1, 4, 3, 2, 5, 0]:
                y = _dot(a7[k].astype(bf16), bd2.at[sl, 7 * i + k][...])
                out += [y[r_:r_ + 16, 0:128] for r_ in range(0, RB, 128)]
                old = accs.at[7 * i + k][...]
                if i == 6:
                    old = jnp.where(u == 1, 0.0, old)
                accs.at[7 * i + k][...] = old + y
            return out

        seq = 'G0 G3 G4 G6 G1 D2 G2 G5 D6 D0 D3 D1 D4 D5'.split()
        sanc = []
        for tk in seq:
            if tk[0] == 'D' and not dprep:
                dprep.append(1)
                lo_, hi_ = 0, 1
                src = [a for p in range(lo_, hi_) for a in sanc[p]]
                pcs = [(k0, c0, i) for k0 in range(0, 64, 16) for c0 in range(0, QD, 128) for i in range(7)]
                for e, (k0, c0, i) in enumerate(pcs):
                    prep_d2_piece(sn, i, pl.multiple_of(s_ * 64, 64) + k0, c0, tm16,
                                  src[e * len(src) // len(pcs)], 1)
            sanc.append((gate_up if tk[0] == 'G' else down)(int(tk[1])))
        kb = pl.multiple_of(s_ * (QD // 2), QD // 2)
        PW = [[2, 5], [7, 8], [8, 14]]
        for a in range(max(GA) + 1):
            members = [i for i in range(7) if GA[i] == a]
            last = max(p for p, tk in enumerate(seq) if tk[0] == 'G' and int(tk[1]) in members)
            lo_, hi_ = max(PW[a][0], last + 1), max(PW[a][1], last + 2)
            src = [x for p in range(lo_, hi_) for x in sanc[p]]
            if hi_ == len(seq):
                src = src[:int(len(src) * 0.9)]
            pieces = [(t, k0, i) for k0 in range(0, QD // 2, 16) for t in range(2) for i in members]
            for e, (t, k0, i) in enumerate(pieces):
                prep_gu2_piece(sn, i, t, kb + k0, tm16, src[e * len(src) // len(pieces)], 4)

        @pl.when(jnp.logical_and(s_ == 1, j + 3 < NG))
        def _():
            wd_copy(j + 3, sn).start()
            for cp in gu_copies(j + 3, sn):
                cp.start()
        return carry

    wd_copy(2, 0).start()
    for cp in gu_copies(2, 0):
        cp.start()
    lax.fori_loop(1, 2 * NG, p3_body, 0)

    SB = 32

    def p4_body(k, carry):
        acck = acc.at[pl.ds(49 * (k >> 1), 49)]
        for u in range(RB // SB):
            b = u // (128 // SB)
            q0 = pl.multiple_of(k * 128 + (u % (128 // SB)) * SB, SB)
            r0 = pl.multiple_of(b * QS + q0, SB)
            rows = pl.ds(r0, SB)
            qr = pl.multiple_of((k & 1) * 128 + (u % (128 // SB)) * SB, SB)
            for n in range(2):
                ms = [None] * 7
                for i in [0, 1, 2, 3, 4, 5, 6]:
                    ms[i] = _dot(oa.at[i][rows, :], bo.at[i, n][...])
                av = []
                for i in range(7):
                    ld = lambda e: acck.at[7 * i + e][pl.ds(qr, SB), :]
                    av.append((lambda: ld(0) + ld(3) - ld(4) + ld(6), lambda: ld(2) + ld(4),
                               lambda: ld(1) + ld(3), lambda: ld(0) - ld(1) + ld(2) + ld(5))[2 * b + n]())
                ss = _ccomb(ms)
                fs = _ccomb(av)
                for q, (h, c0) in enumerate(((0, n * 256), (0, HD + n * 256), (1, n * 256), (1, HD + n * 256))):
                    hf = 0.25 * fs[q]
                    g = hf + hf * jnp.tanh(hf)
                    xv = xraw.at[h][rows, c0:c0 + 256].astype(f32)
                    obuf.at[h][rows, c0:c0 + 256] = (xv + ss[q] * g).astype(bf16)
            out_copy(r0, SB, 0).start()
        return carry

    lax.fori_loop(0, NB, p4_body, 0)
    out_copy(0, HS, 0).wait()


@jax.jit
def pallas_recurrent_scan__sliding_local_dilated__geglu_ffn__prompt_kernel(
    A_x: jax.Array,
    A_wqkv: jax.Array,
    A_wo: jax.Array,
    B_x: jax.Array,
    B_w_gate: jax.Array,
    B_w_up: jax.Array,
    B_w_down: jax.Array,
):
    any_spec = pl.BlockSpec(memory_space=pl.ANY)
    out = pl.pallas_call(
        _kernel,
        out_shape=jax.ShapeDtypeStruct((2, HS, D), bf16),
        in_specs=[any_spec] * 6,
        out_specs=any_spec,
        scratch_shapes=[
            pltpu.VMEM((2, HS, D), bf16),
            pltpu.VMEM((7, HS // 2, HD), u32),
            pltpu.VMEM((49, QS // 2, QD), u32),
            pltpu.VMEM((2, 2, D, GC), bf16),
            pltpu.VMEM((2, GC, D), bf16),
            pltpu.VMEM((7, HD // 2, FC), u32),
            pltpu.VMEM((7, FH // 2, HD), u32),
            pltpu.VMEM((2, 49, 64, QD), u32),
            pltpu.VMEM((105, RB, QD), f32),
            pltpu.VMEM((3, D, D), bf16),
            pltpu.VMEM((3, 8, PAD + S + 8, 128), f32),
            pltpu.VMEM((4, D, 256), bf16),
            pltpu.VMEM((7, 2, HD // 2, 256), u32),
            pltpu.VMEM((2, 2, HS, 128), f32),
            pltpu.VMEM((2, 16, 128), bf16),
            pltpu.SemaphoreType.DMA((26,)),
        ] + [pltpu.VMEM((2, 7 * n, QD // 2, 256), u32) for n in (2, 2, 3)],
        compiler_params=pltpu.CompilerParams(vmem_limit_bytes=123 * 1024 * 1024,
                                             disable_bounds_checks=True,
                                             disable_semaphore_checks=True),
        name="fusedk",
    )(A_x.reshape(2, HS, D), A_wqkv, A_wo, B_w_gate, B_w_up, B_w_down)
    return out.reshape(1, S, D)
```

```python
import jax
import jax.numpy as jnp
from jax import lax
import jax.experimental.pallas as pl
import jax.experimental.pallas.tpu as pltpu

f32 = jnp.float32
bf16 = jnp.bfloat16
u32 = jnp.uint32

S, D, F = 2048, 1024, 3584
HS, HD = S // 2, D // 2
FC = 256
FH = FC // 2
QS, QD = S // 4, D // 4
GC = 512
NG = F // GC
RB = 256
NB = HS // RB
PAD = 16
NW = 8
SCALE = 32 ** -0.5
LOG2E = 1.4426950408889634
NEG = -1e9 / SCALE


def _dot(a, b):
    return jnp.dot(a, b, preferred_element_type=f32)


def _acomb(a11, a12, a21, a22):
    r = lambda v: v.astype(bf16)
    return [r(a11 + a22), r(a21 + a22), r(a11), r(a22), r(a11 + a12), r(a21 - a11), r(a12 - a22)]


def _bcomb(b11, b12, b21, b22):
    r = lambda v: v.astype(bf16)
    return [r(b11 + b22), r(b11), r(b12 - b22), r(b21 - b11), r(b22), r(b11 + b12), r(b21 + b22)]


def _asum(a11, a12, a21, a22):
    return [a11 + a22, a21 + a22, a11, a22, a11 + a12, a21 - a11, a12 - a22]


def _bsum(b11, b12, b21, b22):
    return [b11 + b22, b11, b12 - b22, b21 - b11, b22, b11 + b12, b21 + b22]


_A_TERMS = [((0, 0), (1, 1), 1), ((1, 0), (1, 1), 1), ((0, 0), None, 0), ((1, 1), None, 0),
            ((0, 0), (0, 1), 1), ((1, 0), (0, 0), -1), ((0, 1), (1, 1), -1)]
_B_TERMS = [((0, 0), (1, 1), 1), ((0, 0), None, 0), ((0, 1), (1, 1), -1), ((1, 0), (0, 0), -1),
            ((1, 1), None, 0), ((0, 0), (0, 1), 1), ((1, 0), (1, 1), 1)]


def _ccomb(m):
    m1, m2, m3, m4, m5, m6, m7 = m
    return m1 + m4 - m5 + m7, m3 + m5, m2 + m4, m1 - m2 + m3 + m6


def _gate_tanh(x):
    c = 0.7978845608028654
    return jnp.tanh(x * (c + (c * 0.044715) * (x * x)))


def _glu2(g, th, u):
    a = g * u
    return a + a * th


def _sum8(v):
    return ((v[0] + v[1]) + (v[2] + v[3])) + ((v[4] + v[5]) + (v[6] + v[7]))


def _butterfly(sets, masks, axis, size):
    for b in range(3):
        sh = 1 << b
        out = []
        for blk in sets:
            nxt = list(blk)
            for c in range(8):
                if c & sh == 0:
                    lo, hi = blk[c], blk[c + sh]
                    nxt[c] = jnp.where(masks[b], lo, pltpu.roll(hi, sh, axis))
                    nxt[c + sh] = jnp.where(masks[b], pltpu.roll(lo, size - sh, axis), hi)
            out.append(nxt)
        sets = out
    return sets


def _kernel(x_hbm, wqkv_hbm, wo_hbm, wg_hbm, wu_hbm, wd_hbm, out_hbm,
            xraw, xa_u, xa2_u, gu_raw, wd_raw, bgu_u, bd_u, bd2_u, accq, wq_raw, qkv,
            wo_raw, bo_u, stats, zbuf, ost, sems, *bgu2_u):
    acc = accq
    bq = accq.bitcast(bf16)
    bo = bo_u.bitcast(bf16)
    obuf = xraw
    xa = xa_u.bitcast(bf16)
    bgu = bgu_u.bitcast(bf16)
    bd = bd_u.bitcast(bf16)
    bd2 = bd2_u.bitcast(bf16)
    xa2 = xa2_u.bitcast(bf16)
    GA = [0, 1, 2, 0, 2, 2, 1]
    _al = [r.bitcast(bf16) for r in bgu2_u]
    _pos = [sum(1 for q in range(i) if GA[q] == GA[i]) for i in range(7)]
    bg = lambda slot, i, k: _al[GA[i]].at[slot, 7 * _pos[i] + k]
    oa = xa
    pk = lambda v: pltpu.bitcast(v, u32)
    un = lambda v: pltpu.bitcast(v, bf16)

    lane = lax.broadcasted_iota(jnp.int32, (8, 128), 1)
    row8 = lax.broadcasted_iota(jnp.int32, (8, 128), 0)
    lane_lo = [(lane & (1 << b)) == 0 for b in range(3)]
    row_lo = [(row8 & (1 << b)) == 0 for b in range(3)]

    XP = [(0, 128), (128, 128), (512, 128), (640, 128), (256, 256), (768, 256)]

    def x_copy(r):
        r0, n = XP[r]
        return pltpu.make_async_copy(x_hbm.at[:, pl.ds(r0, n), :],
                                     xraw.at[:, pl.ds(r0, n), :], sems.at[(0, 1, 2, 3, 23, 14)[r]])

    def gu_copies(j, slot):
        off = pl.multiple_of(j * GC, GC)
        return (pltpu.make_async_copy(wg_hbm.at[:, pl.ds(off, GC)], gu_raw.at[slot, 0], sems.at[4 + 3 * slot]),
                pltpu.make_async_copy(wu_hbm.at[:, pl.ds(off, GC)], gu_raw.at[slot, 1], sems.at[5 + 3 * slot]))

    def wd_copy(j, slot):
        off = pl.multiple_of(j * GC, GC)
        return pltpu.make_async_copy(wd_hbm.at[pl.ds(off, GC), :], wd_raw.at[slot], sems.at[6 + 3 * slot])

    def gu0_copy(t, c):
        w = (wg_hbm, wu_hbm)[t]
        return pltpu.make_async_copy(w.at[:, pl.ds(c * FC, FC)], gu_raw.at[0, t, :, pl.ds(c * FC, FC)],
                                     sems.at[15 + 2 * c + t])

    def wd0_copy(c):
        return pltpu.make_async_copy(wd_hbm.at[pl.ds(c * FC, FC), :], wd_raw.at[0, pl.ds(c * FC, FC), :],
                                     sems.at[19 + c])

    def wq_copy(t):
        return pltpu.make_async_copy(wqkv_hbm.at[:, pl.ds(t * D, D)], wq_raw.at[t], sems.at[10 + t])

    def wo_copies():
        return [pltpu.make_async_copy(wo_hbm.at[:, pl.ds(c * 256, 256)], wo_raw.at[c], sems.at[24])
                for c in range(4)]

    class _Z:
        cps = [pltpu.make_async_copy(x_hbm.at[0, pl.ds(0, 16), pl.ds(0, 128)], zbuf.at[q], sems.at[21 + q])
               for q in range(2)]

        def start(self):
            for cp in self.cps:
                cp.start()

        def wait(self):
            for cp in self.cps:
                cp.wait()

    z_copy = _Z

    def out_copy(r0, n, k):
        return pltpu.make_async_copy(obuf.at[:, pl.ds(r0, n), :], out_hbm.at[:, pl.ds(r0, n), :],
                                     sems.at[25 + k])

    def true_mask():
        return pk(zbuf[0]) == pk(zbuf[1])

    def ln_half(h, c0, tm16, a):
        xs = []
        for c in range(4):
            x2 = xraw.at[h][c0:c0 + 16, c * 256:(c + 1) * 256].astype(f32)
            xs += [x2[:, :128], x2[:, 128:]]
        s1 = _sum8(xs)
        if a is not None:
            s1 = jnp.where(tm16, s1, a)
        m = jnp.sum(s1, axis=-1, keepdims=True) * (1.0 / D)
        xc = [x - m for x in xs]
        v = jnp.sum(_sum8([x * x for x in xc]), axis=-1, keepdims=True) * (1.0 / D)
        r = lax.rsqrt(v + 1e-5)
        stats.at[h, 0][c0:c0 + 16, :] = jnp.broadcast_to(m, (16, 128))
        stats.at[h, 1][c0:c0 + 16, :] = jnp.broadcast_to(r, (16, 128))
        return [x * r for x in xc]

    def ln_rows(r0, n, anc=None, af=0.85):
        tm16 = None
        if anc is not None:
            tm = true_mask()
            tm16 = jnp.concatenate([tm, tm], axis=0)
            anc = anc[:int(len(anc) * af)]
        nch = n // 16
        for k in range(nch):
            c0 = r0 + 16 * k
            a = [None, None]
            if anc is not None:
                a = [anc[(len(anc) * (2 * k + u)) // (2 * nch)] for u in range(2)]
            lo = ln_half(0, c0, tm16, a[0])
            hi = ln_half(1, c0, tm16, a[1])
            for c in range(4):
                cs = _acomb(lo[c], lo[c + 4], hi[c], hi[c + 4])
                for i in range(7):
                    xa.at[i][c0:c0 + 16, c * 128:(c + 1) * 128] = cs[i]

    def prep_gu(c, ts=(0, 1)):
        KC = 32
        for t in ts:
            w = gu_raw.at[0, t]
            for k0 in range(0, HD, KC):
                lo = w[k0:k0 + KC, c * FC:(c + 1) * FC].astype(f32)
                hi = w[HD + k0:HD + k0 + KC, c * FC:(c + 1) * FC].astype(f32)
                cs = _bcomb(lo[:, :FH], lo[:, FH:], hi[:, :FH], hi[:, FH:])
                for i in range(7):
                    bgu.at[i][k0:k0 + KC, t * FH:(t + 1) * FH] = cs[i]

    def prep_d(w, kh):
        KC = 16
        for k0 in range(0, kh, KC):
            for c0 in range(0, HD, 256):
                g = lambda a, b: w[a + k0:a + k0 + KC, b + c0:b + c0 + 256].astype(f32)
                cs = _bcomb(g(0, 0), g(0, HD), g(kh, 0), g(kh, HD))
                for i in range(7):
                    bd.at[i][k0:k0 + KC, c0:c0 + 256] = cs[i]

    def two_level_piece(terms, inner, ld, i, tm16, anc, nanc, store):
        p, q, sg = terms[i]
        P = ld(*p)
        for e in range(nanc):
            P[e >> 1][e & 1] = jnp.where(tm16, P[e >> 1][e & 1], anc)
        if q is not None:
            Q = ld(*q)
            P = [[P[b][d] + Q[b][d] if sg > 0 else P[b][d] - Q[b][d] for d in range(2)] for b in range(2)]
        ops = inner(P[0][0], P[0][1], P[1][0], P[1][1])
        for k in range(7):
            store(7 * i + k, ops[k].astype(bf16))

    def prep_gu2_piece(slot, i, t, k0, tm16, anc, nanc):
        w = gu_raw.at[slot, t]

        def ld(R, C):
            out = []
            for b in range(2):
                x2 = w[pl.ds((2 * R + b) * QD + k0, 16), C * 256:(C + 1) * 256].astype(f32)
                out.append([x2[:, :128], x2[:, 128:]])
            return out

        def store(p, v):
            bg(slot, i, p % 7)[pl.ds(k0, 16), t * 128:(t + 1) * 128] = v
        two_level_piece(_B_TERMS, _bsum, ld, i, tm16, anc, nanc, store)

    def prep_d2_piece(slot, i, k0, c0, tm16, anc, nanc):
        w = wd_raw.at[slot]

        def ld(R, C):
            return [[w[pl.ds((2 * R + b) * 128 + k0, 16),
                       (2 * C + d) * QD + c0:(2 * C + d) * QD + c0 + 128].astype(f32) for d in range(2)]
                    for b in range(2)]

        def store(p, v):
            bd2.at[slot, p][pl.ds(k0, 16), c0:c0 + 128] = v
        two_level_piece(_B_TERMS, _bsum, ld, i, tm16, anc, nanc, store)

    def make_xa2(r0, tm16, ancs):
        st = [[[stats.at[a, e][pl.ds(b * QS + r0, 16), :] for e in range(2)] for b in range(2)] for a in range(2)]
        for j in range(2):
            def ld(R, C):
                out = []
                for b in range(2):
                    m, r = st[R][b]
                    row = []
                    for d in range(2):
                        c0 = (2 * C + d) * QD + j * 128
                        xv = xraw.at[R][pl.ds(b * QS + r0, 16), c0:c0 + 128].astype(f32)
                        row.append((xv - m) * r)
                    out.append(row)
                return out

            def store(p, v):
                xa2.at[p][pl.ds(r0, 16), j * 128:(j + 1) * 128] = v
            for i in range(7):
                two_level_piece(_A_TERMS, _asum, ld, i, tm16, ancs[7 * j + i], 2, store)

    def ffn_gu(r0, n, o1):
        ms = [None] * 7
        for i in o1:
            ms[i] = _dot(xa[i, r0:r0 + n, :], bgu[i])
        anc = [ms[i][k:k + 16, t * FH:(t + 1) * FH] for i in o1 for t in range(2) for k in range(0, n, 64)]
        hs = _acomb(*[_glu2(v[:, :FH], _gate_tanh(v[:, :FH]), v[:, FH:]) for v in _ccomb(ms)])
        return hs, anc

    def ffn_dn(r0, n, hs, od, first, last=False):
        b, q0 = r0 // QS, r0 % QS
        anc = []
        for i in od:
            y = _dot(hs[i], bd[i])
            anc += [y[k:k + 16, 0:128] for k in range(0, n, 32)]
            lo, hi = (acc.at[7 * i + e] for e in ((6, 2), (1, 5))[b])
            ylo, yhi = y[:, :QD], y[:, QD:]
            if not first:
                ylo = ylo + lo[q0:q0 + n, :]
                yhi = yhi + hi[q0:q0 + n, :]
            if last:
                yhi = yhi + (ylo - acc.at[7 * i + 2][q0:q0 + n, :])
            lo[q0:q0 + n, :] = ylo
            hi[q0:q0 + n, :] = yhi
        return anc

    def zero_acc0(ps, anc):
        tm = true_mask()
        tm16 = jnp.concatenate([tm, tm], axis=0)
        pcs = [(p, q) for p in ps for q in range(4)]
        for e, (p, q) in enumerate(pcs):
            z16 = jnp.where(tm16, 0.0, anc[e * len(anc) // len(pcs)])
            for r0 in range(64 * q, 64 * q + 64, 16):
                for c in range(2):
                    acc.at[p][r0:r0 + 16, c * 128:(c + 1) * 128] = z16

    upk = lambda v: un(v).astype(f32)

    def prep_q_half(t, h, dst, par=1):
        KC = 16
        sa = (128 - 2) * h
        sb = 2 * (1 - h)
        w = wq_raw.at[t]

        def stage1(r0):
            blk = [pk(w[r0:r0 + KC, c * 128:(c + 1) * 128]) for c in range(8)]
            rl = lambda v, sft: v if (isinstance(sft, int) and sft == 0) else pltpu.roll(v, sft, 1)
            return [jnp.where(lane_lo[1], rl(blk[c], sa), rl(blk[c + 2], sb)) for c in (0, 1, 4, 5)]

        def stage(sets, jb, b):
            sh = 1 << b
            out = []
            for blk in sets:
                nxt = list(blk)
                for j in range(4):
                    if j & jb == 0:
                        lo, hi = blk[j], blk[j + jb]
                        nxt[j] = jnp.where(lane_lo[b], lo, pltpu.roll(hi, sh, 1))
                        nxt[j + jb] = jnp.where(lane_lo[b], pltpu.roll(lo, 128 - sh, 1), hi)
                out.append(nxt)
            return out

        for k00 in range(0, HD, KC * par):
            ks = [k00 + KC * q for q in range(par)]
            hv = stage(stage([stage1(hk * HD + k0) for k0 in ks for hk in range(2)], 1, 0), 2, 2)
            for q, k0 in enumerate(ks):
                lo, hi = hv[2 * q], hv[2 * q + 1]
                for e in range(2):
                    cs = _bcomb(upk(lo[e]), upk(lo[e + 2]), upk(hi[e]), upk(hi[e + 2]))
                    for i in range(7):
                        dst.at[i][k0:k0 + KC, e * 128:(e + 1) * 128] = cs[i]

    def qkv_tiles(t, h, src):
        anc16 = []
        for e in range(2):
            qlo = qkv.at[t, 4 * h + e]
            qhi = qkv.at[t, 4 * h + 2 + e]
            for r in range(NB):
                oq = [1, 4, 2, 3, 0, 5, 6]
                ms = [None] * 7
                for i in oq:
                    ms[i] = _dot(xa[i, r * RB:(r + 1) * RB, :], src.at[i][:, e * 128:(e + 1) * 128])
                c11, c12, c21, c22 = _ccomb(ms)
                anc16 += [ms[i][k:k + 16] for i in oq for k in range(0, RB, 64)]
                r0 = PAD + r * RB
                qlo[r0:r0 + RB, :] = c11
                qhi[r0:r0 + RB, :] = c12
                qlo[HS + r0:HS + r0 + RB, :] = c21
                qhi[HS + r0:HS + r0 + RB, :] = c22
                if r == 0:
                    qlo[PAD - 16:PAD, :] = jnp.broadcast_to(c11[0:1, :], (16, 128))
                    qhi[PAD - 16:PAD, :] = jnp.broadcast_to(c12[0:1, :], (16, 128))
        return anc16

    def prep_o_chunk(n2, g16, e, tm, ancs):
        res = []
        for h in range(2):
            w = wo_raw.at[n2 + 2 * h]
            w16 = [w[pl.ds(128 * i + g16, 16), e * 128:(e + 1) * 128].astype(f32) for i in range(8)]
            for u in range(2):
                blk = [v[8 * u:8 * u + 8] for v in w16]
                blk[0] = jnp.where(tm, blk[0], ancs[2 * h + u])
                res += _butterfly([blk], row_lo, 0, 8)
        cols = [[jnp.concatenate([res[2 * h][j], res[2 * h + 1][j]], axis=0) for j in range(8)]
                for h in range(2)]
        for b in range(4):
            cs = _bcomb(cols[0][b], cols[1][b], cols[0][b + 4], cols[1][b + 4])
            for i in range(7):
                bo.at[i, n2][pl.ds(b * 128 + g16, 16), e * 128:(e + 1) * 128] = cs[i]

    PH = [4 * ((c >> 1) & 1) + 2 * (c >> 2) + (c & 1) for c in range(8)]

    def attn4(bases, r0=None):
        lgs = []
        for g, base in enumerate(bases):
            lg = [None] * NW
            for c in range(8):
                q = qkv[0, PH[c], pl.ds(base, 8), :]
                for w in range(NW):
                    pr = q * qkv[1, PH[c], pl.ds(base - 2 * w, 8), :]
                    lg[w] = pr if lg[w] is None else lg[w] + pr
            s8 = 8 if g & 1 else 120
            s16 = 16 if g & 2 else 112
            for w in range(NW):
                lg[w] = lg[w] + pltpu.roll(lg[w], s8, 1)
                lg[w] = lg[w] + pltpu.roll(lg[w], s16, 1)
            lgs.append(lg)
        b3 = (lane & 8) != 0
        b4 = (lane & 16) != 0
        lg = [jnp.where(b4, jnp.where(b3, lgs[3][w], lgs[2][w]), jnp.where(b3, lgs[1][w], lgs[0][w]))
              for w in range(NW)]
        if r0 is not None:
            pos = jnp.where(b4, S, row8 + r0 + (lane & 8))
            for w in range(1, NW):
                lg[w] = jnp.where(pos >= 2 * w, lg[w], NEG)
        m = lg[0]
        for w in range(1, NW):
            m = jnp.maximum(m, lg[w])
        p = [jnp.exp2((lg[w] - m) * (SCALE * LOG2E)) for w in range(NW)]
        den = p[0]
        for w in range(1, NW):
            den = den + p[w]
        inv = 1.0 / den
        p = [v * inv for v in p]
        parts = []
        for g, base in enumerate(bases):
            k4 = b4 if g & 2 else jnp.logical_not(b4)
            k3 = b3 if g & 1 else jnp.logical_not(b3)
            outs = [None] * 8
            for w in range(NW):
                pw = jnp.where(k4, p[w], pltpu.roll(p[w], 112 if g & 2 else 16, 1))
                pw = jnp.where(k3, pw, pltpu.roll(pw, 120 if g & 1 else 8, 1))
                for c in range(8):
                    pr = pw * qkv[2, PH[c], pl.ds(base - 2 * w, 8), :]
                    outs[c] = pr if outs[c] is None else outs[c] + pr
            parts.append(outs)
        return parts

    def put_oa(r0, lo, hi):
        for n in range(4):
            cs = _acomb(lo[n], lo[n + 4], hi[n], hi[n + 4])
            for i in range(7):
                oa.at[i][pl.ds(pl.multiple_of(r0, 16), 16), n * 128:(n + 1) * 128] = cs[i]

    def attn_pair(r0, mask=False):
        parts = attn4([pl.multiple_of(PAD + h * HS + r0 + 8 * u, 8) for h in range(2) for u in range(2)],
                      r0 if mask else None)
        lo = [jnp.concatenate([parts[0][c], parts[1][c]], axis=0) for c in range(8)]
        hi = [jnp.concatenate([parts[2][c], parts[3][c]], axis=0) for c in range(8)]
        put_oa(r0, lo, hi)
        return hi[7]

    def attn_half(v):
        m = v >> 1
        base = pl.multiple_of(PAD + (v & 1) * HS + 832 + 32 * jnp.minimum(m, 5), 16)
        parts = attn4([base + 8 * g for g in range(4)])
        dst = ost.at[m & 1, v & 1]
        for g in range(4):
            for c in range(8):
                dst.at[c][8 * g:8 * g + 8, :] = parts[g][c]
        mf = jnp.maximum((v + 1) >> 1, 1) - 1
        e16 = pl.multiple_of(16 * (1 - (v & 1)), 16)
        src = ost.at[mf & 1]
        put_oa(832 + 32 * mf + e16, *[[src.at[hh, c][pl.ds(e16, 16), :] for c in range(8)] for hh in range(2)])
        return jnp.concatenate([parts[2][7], parts[3][7]], axis=0)

    wd0 = lambda c: wd_raw.at[0, c * FC:(c + 1) * FC, :]
    RA, RBB, RC, RD = 0, 512, 256, 768

    x_copy(0).start()
    x_copy(1).start()
    gu0_copy(0, 0).start()
    z_copy().start()
    gu0_copy(1, 0).start()
    x_copy(2).start()
    wd0_copy(0).start()
    x_copy(3).start()
    x_copy(4).start()
    gu0_copy(0, 1).start()
    gu0_copy(1, 1).start()
    wd0_copy(1).start()
    x_copy(5).start()
    wq_copy(0).start()
    for cp in wo_copies():
        cp.start()
    wq_copy(1).start()

    x_copy(0).wait()
    ln_rows(RA, 128)
    x_copy(1).wait()
    ln_rows(RA + 128, 128)

    gu0_copy(0, 0).wait()
    prep_gu(0, (0,))
    mg = [None] * 7
    for i in [4, 2, 3, 1, 0, 6, 5]:
        mg[i] = _dot(xa[i, RA:RA + RB, :], bgu[i, :, :FH])
    gg = [(v, _gate_tanh(v)) for v in _ccomb(mg)]

    z_copy().wait()
    gu0_copy(1, 0).wait()
    x_copy(2).wait()
    prep_gu(0, (1,))
    mu = [None] * 7
    for i in [4, 2, 3, 1, 0, 6, 5]:
        mu[i] = _dot(xa[i, RA:RA + RB, :], bgu[i, :, FH:])
    ha = _acomb(*[_glu2(a[0], a[1], b) for a, b in zip(gg, _ccomb(mu))])
    ln_rows(RBB, 128, [mu[i][k:k + 16] for i in [4, 2, 3, 1, 0, 6, 5] for k in range(0, RB, 64)],
            0.85)

    wd0_copy(0).wait()
    x_copy(3).wait()
    prep_d(wd0(0), FH)
    hb0, anc = ffn_gu(RBB, 128, [6, 5, 0, 1, 4, 2, 3])
    ffn_dn(RA, RB, ha, [3, 0, 4, 1, 2, 6, 5], True)
    ln_rows(RBB + 128, 128, anc, 0.7)

    x_copy(4).wait()
    gu0_copy(0, 1).wait()
    gu0_copy(1, 1).wait()
    hb1, anc = ffn_gu(RBB + 128, 128, [4, 0, 2, 6, 5, 3, 1])
    anc2 = ffn_dn(RBB, 128, hb0, [3, 6, 5, 4, 2, 0, 1], True)
    ffn_dn(RBB + 128, 128, hb1, [3, 6, 5, 4, 2, 0, 1], True)
    prep_gu(1)
    ln_rows(RC, RB, anc + anc2[:28], 0.85)

    wd0_copy(1).wait()
    x_copy(5).wait()
    prep_d(wd0(1), FH)
    h2, anc = ffn_gu(RA, RB, [4, 2, 3, 1, 0, 6, 5])
    ffn_dn(RA, RB, h2, [6, 1, 4, 3, 2, 5, 0], False)
    ln_rows(RD, RB, anc, 0.75)
    zs_ = [p for p in range(49) if p % 7 in (0, 3, 4)]
    zero_acc0(zs_[:7], anc)

    wq_copy(0).wait()
    h3, anc = ffn_gu(RBB, RB, [0, 1, 2, 3, 4, 5, 6])
    zero_acc0(zs_[7:], anc)
    prep_q_half(0, 0, bq.at[56:63], 2)
    ffn_dn(RBB, RB, h3, [0, 3, 4, 6, 2, 1, 5], False, True)

    for cp in wo_copies():
        cp.wait()
    wq_copy(2).start()
    for cp in gu_copies(1, 1):
        cp.start()
    wd_copy(1, 1).start()

    def p2_body(i, carry):
        @pl.when(i == 1)
        def _():
            wq_copy(1).wait()

        @pl.when(i == 3)
        def _():
            wq_copy(2).wait()

        @pl.when(i == 4)
        def _():
            for cp in gu_copies(1, 1):
                cp.wait()
            wd_copy(1, 1).wait()
        bqv = bq.at[pl.ds(49 + 7 * i, 21)]
        anc16 = qkv_tiles(i >> 1, i & 1, bqv.at[7:14])
        prep_q_half(jnp.minimum((i + 1) >> 1, 2), (i + 1) & 1, bqv.at[14:21], 2)
        tm = true_mask()
        tm16 = jnp.concatenate([tm, tm], axis=0)
        jobs = []
        for k in range(6):
            jobs += [('x', k, q) for q in range(14)]
        for k in range(6):
            jobs += [('o', k, q) for q in range(4)]
        for k in range(8):
            jobs += [('g', k, q) for q in range(7)]
        for k in range(4):
            jobs += [('d', k, q) for q in range(7)]
        for k in range(7):
            jobs += [('z', k, q) for q in range(4)]
        by = {}
        for kind in 'oxgzd':
            js = [jb for jb in jobs if jb[0] == kind]
            for e, jb in enumerate(js):
                by[jb] = (e + 0.5) / len(js)
        ranked = sorted(jobs, key=lambda jb: by[jb])
        na = len(anc16) - 4
        at = {jb: anc16[(e * na) // len(ranked)] for e, jb in enumerate(ranked)}
        for k in range(6):
            make_xa2(pl.multiple_of(jnp.minimum(96 * i, QS - 96), 32) + 16 * k, tm16,
                     [at['x', k, q] for q in range(14)])
        for k in range(6):
            m_ = jnp.minimum(3 * i + (k >> 1), 15)
            prep_o_chunk(m_ >> 3, pl.multiple_of((m_ & 7) * 16, 16), k & 1, tm,
                         [at['o', k, q][0:8] for q in range(4)])
        for k in range(8):
            for q in range(7):
                prep_gu2_piece(i >> 2, q, k & 1, pl.multiple_of((i & 3) * 64, 64) + 16 * (k >> 1), tm16,
                               at['g', k, q], 1)
        for k in range(4):
            for q in range(7):
                prep_d2_piece(i >> 2, q, pl.multiple_of((i & 3) * 32, 32) + 16 * (k >> 1), (k & 1) * 128, tm16,
                              at['d', k, q], 1)
        az = acc.at[pl.ds(49 + 7 * i, 21)]
        for k in range(7):
            for q in range(4):
                z16 = jnp.where(tm16, 0.0, at['z', k, q])
                for r0 in range(64 * q, 64 * q + 64, 16):
                    for c in range(2):
                        az.at[k][r0:r0 + 16, c * 128:(c + 1) * 128] = z16
        return carry

    lax.fori_loop(0, 6, p2_body, 0)

    def p3_body(u, carry):
        j = u >> 1
        s_ = u & 1
        sl = j & 1
        jn = jnp.minimum((u >> 1) + 1, NG - 1)
        sn = 1 - sl

        @pl.when(jnp.logical_and(s_ == 0, j + 1 < NG))
        def _():
            wd_copy(jn, sn).wait()
            for cp in gu_copies(jn, sn):
                cp.wait()
        a4 = pl.multiple_of((u - 1) * 64, 64)
        for g in [4, 0, 1, 2, 3]:
            if g < 4:
                att_last = attn_pair(a4 + 16 * g, g == 0)
            else:
                att_last = attn_half(u - 1)
        tm = true_mask()
        tm16 = jnp.concatenate([tm, tm], axis=0)

        rows = pl.ds(pl.multiple_of(s_ * RB, RB), RB)
        accs = acc.at[pl.ds(49 * s_, 49)]
        order = (0, 3, 4, 6, 2, 1, 5)
        c1 = [None] * 7
        dprep = []
        h = [[None] * 4 for _ in range(4)]

        def gate_up(i):
            ms = [None] * 7
            for k in order:
                ms[k] = _dot(xa2.at[7 * i + k][rows, :], bg(sl, i, k)[...])
            c1[i] = _ccomb(ms)
            return [ms[k][r_:r_ + 16, t * 128:(t + 1) * 128] for k in order for r_ in range(0, RB, 64)
                    for t in range(2)]

        def hidden(a, e):
            if h[2 * a][2 * e] is None:
                for q in range(4):
                    m = [None if v is None else v[q] for v in c1]
                    if (a, e) == (0, 0):
                        cc = m[0] + m[3] - m[4] + m[6]
                    elif (a, e) == (0, 1):
                        cc = m[2] + m[4]
                    elif (a, e) == (1, 0):
                        cc = m[1] + m[3]
                    else:
                        cc = m[0] - m[1] + m[2] + m[5]
                    h[2 * a + (q >> 1)][2 * e + (q & 1)] = _glu2(cc[:, :128], _gate_tanh(cc[:, :128]),
                                                                 cc[:, 128:])
            return [[h[2 * a + b][2 * e + f] for f in range(2)] for b in range(2)]

        def down(i):
            p, q, sg = _A_TERMS[i]
            P = hidden(*p)
            if q is not None:
                Q = hidden(*q)
                P = [[P[b][f] + Q[b][f] if sg > 0 else P[b][f] - Q[b][f] for f in range(2)] for b in range(2)]
            out = []
            if i == 2:
                v = P[0][0]
                P[0][0] = jnp.concatenate([jnp.where(tm16, v[0:16], att_last), v[16:]], axis=0)
            a7 = _asum(P[0][0], P[0][1], P[1][0], P[1][1])
            for k in [6, 1, 4, 3, 2, 5, 0]:
                y = _dot(a7[k].astype(bf16), bd2.at[sl, 7 * i + k][...])
                out += [y[r_:r_ + 16, 0:128] for r_ in range(0, RB, 128)]
                old = accs.at[7 * i + k][...]
                if i == 6:
                    old = jnp.where(u == 1, 0.0, old)
                accs.at[7 * i + k][...] = old + y
            return out

        seq = 'G0 G3 G4 G6 G1 D2 G2 G5 D6 D1 D3 D0 D4 D5'.split()
        sanc = []
        for tk in seq:
            if tk[0] == 'D' and not dprep:
                dprep.append(1)
                lo_, hi_ = 0, 1
                src = [a for p in range(lo_, hi_) for a in sanc[p]]
                pcs = [(k0, c0, i) for k0 in range(0, 64, 16) for c0 in range(0, QD, 128) for i in range(7)]
                for e, (k0, c0, i) in enumerate(pcs):
                    prep_d2_piece(sn, i, pl.multiple_of(s_ * 64, 64) + k0, c0, tm16,
                                  src[e * len(src) // len(pcs)], 1)
            sanc.append((gate_up if tk[0] == 'G' else down)(int(tk[1])))
        kb = pl.multiple_of(s_ * (QD // 2), QD // 2)
        PW = [[2, 5], [7, 8], [8, 14]]
        for a in range(max(GA) + 1):
            members = [i for i in range(7) if GA[i] == a]
            last = max(p for p, tk in enumerate(seq) if tk[0] == 'G' and int(tk[1]) in members)
            lo_, hi_ = max(PW[a][0], last + 1), max(PW[a][1], last + 2)
            src = [x for p in range(lo_, hi_) for x in sanc[p]]
            if hi_ == len(seq):
                src = src[:int(len(src) * 0.9)]
            pieces = [(t, k0, i) for k0 in range(0, QD // 2, 16) for t in range(2) for i in members]
            for e, (t, k0, i) in enumerate(pieces):
                prep_gu2_piece(sn, i, t, kb + k0, tm16, src[e * len(src) // len(pieces)], 4)

        @pl.when(jnp.logical_and(s_ == 1, j + 3 < NG))
        def _():
            wd_copy(j + 3, sn).start()
            for cp in gu_copies(j + 3, sn):
                cp.start()
        return carry

    wd_copy(2, 0).start()
    for cp in gu_copies(2, 0):
        cp.start()
    for c in range(8):
        ost.at[0, 1, c][16:32, :] = jnp.zeros((16, 128), f32)
    lax.fori_loop(1, 2 * NG, p3_body, 0)

    SB = 32

    def p4_body(k, carry):
        acck = acc.at[pl.ds(49 * (k >> 1), 49)]
        for u in range(RB // SB):
            b = u // (128 // SB)
            q0 = pl.multiple_of(k * 128 + (u % (128 // SB)) * SB, SB)
            r0 = pl.multiple_of(b * QS + q0, SB)
            rows = pl.ds(r0, SB)
            qr = pl.multiple_of((k & 1) * 128 + (u % (128 // SB)) * SB, SB)
            for n in range(2):
                ms = [None] * 7
                for i in [0, 1, 2, 3, 4, 5, 6]:
                    ms[i] = _dot(oa.at[i][rows, :], bo.at[i, n][...])
                av = []
                for i in range(7):
                    ld = lambda e: acck.at[7 * i + e][pl.ds(qr, SB), :]
                    av.append((lambda: ld(0) + ld(3) - ld(4) + ld(6), lambda: ld(2) + ld(4),
                               lambda: ld(1) + ld(3), lambda: ld(0) - ld(1) + ld(2) + ld(5))[2 * b + n]())
                ss = _ccomb(ms)
                fs = _ccomb(av)
                for q, (h, c0) in enumerate(((0, n * 256), (0, HD + n * 256), (1, n * 256), (1, HD + n * 256))):
                    hf = 0.25 * fs[q]
                    g = hf + hf * jnp.tanh(hf)
                    xv = xraw.at[h][rows, c0:c0 + 256].astype(f32)
                    obuf.at[h][rows, c0:c0 + 256] = (xv + ss[q] * g).astype(bf16)
            out_copy(r0, SB, 0).start()
        return carry

    lax.fori_loop(0, NB, p4_body, 0)
    out_copy(0, HS, 0).wait()


@jax.jit
def pallas_recurrent_scan__sliding_local_dilated__geglu_ffn__prompt_kernel(
    A_x: jax.Array,
    A_wqkv: jax.Array,
    A_wo: jax.Array,
    B_x: jax.Array,
    B_w_gate: jax.Array,
    B_w_up: jax.Array,
    B_w_down: jax.Array,
):
    any_spec = pl.BlockSpec(memory_space=pl.ANY)
    out = pl.pallas_call(
        _kernel,
        out_shape=jax.ShapeDtypeStruct((2, HS, D), bf16),
        in_specs=[any_spec] * 6,
        out_specs=any_spec,
        scratch_shapes=[
            pltpu.VMEM((2, HS, D), bf16),
            pltpu.VMEM((7, HS // 2, HD), u32),
            pltpu.VMEM((49, QS // 2, QD), u32),
            pltpu.VMEM((2, 2, D, GC), bf16),
            pltpu.VMEM((2, GC, D), bf16),
            pltpu.VMEM((7, HD // 2, FC), u32),
            pltpu.VMEM((7, FH // 2, HD), u32),
            pltpu.VMEM((2, 49, 64, QD), u32),
            pltpu.VMEM((105, RB, QD), f32),
            pltpu.VMEM((3, D, D), bf16),
            pltpu.VMEM((3, 8, PAD + S + 8, 128), f32),
            pltpu.VMEM((4, D, 256), bf16),
            pltpu.VMEM((7, 2, HD // 2, 256), u32),
            pltpu.VMEM((2, 2, HS, 128), f32),
            pltpu.VMEM((2, 16, 128), bf16),
            pltpu.VMEM((2, 2, 8, 32, 128), f32),
            pltpu.SemaphoreType.DMA((26,)),
        ] + [pltpu.VMEM((2, 7 * n, QD // 2, 256), u32) for n in (2, 2, 3)],
        compiler_params=pltpu.CompilerParams(vmem_limit_bytes=123 * 1024 * 1024,
                                             disable_bounds_checks=True,
                                             disable_semaphore_checks=True),
        name="fusedk",
    )(A_x.reshape(2, HS, D), A_wqkv, A_wo, B_w_gate, B_w_up, B_w_down)
    return out.reshape(1, S, D)
```
